```python
import jax
import jax.numpy as jnp

def _softmax(x, axis=-1):
    return jax.nn.softmax(x, axis=axis)

def _gelu(x):
    return jax.nn.gelu(x, approximate=True)

def _silu(x):
    return jax.nn.silu(x)

def _sigmoid(x):
    return jax.nn.sigmoid(x)

def _layernorm(x, axis=-1, eps=1e-05):
    m = jnp.mean(x, axis=axis, keepdims=True)
    v = jnp.var(x, axis=axis, keepdims=True)
    return (x - m) / jnp.sqrt(v + eps)

def _scatter_add(tgt, idx, src, axis=0):
    return tgt.at[idx].add(src)

def _segment_sum(src, seg, n):
    return jax.ops.segment_sum(src, seg, n)

class _Rng:

    def __init__(self, key):
        self._k = key

    def _next(self):
        self._k, sub = jax.random.split(self._k)
        return sub

    def normal(self, shape):
        return jax.random.normal(self._next(), shape, dtype=jnp.bfloat16)

    def randint(self, lo, hi, shape):
        return jax.random.randint(self._next(), shape, lo, hi, dtype=jnp.int32)

    def uniform(self, shape, lo=0.0, hi=1.0):
        return jax.random.uniform(self._next(), shape, jnp.bfloat16, lo, hi)

    def permutation(self, n):
        return jax.random.permutation(self._next(), n)
kernel_name = 'adaLN_cond__ssm_conv_h3__glu_gated_swiglu__prompt'

def setup_inputs():
    _rng = _Rng(jax.random.key(int.from_bytes(__import__("os").urandom(4), "little")))
    _w = lambda a: (lambda t: t.astype(jnp.bfloat16) if jnp.issubdtype(t.dtype, jnp.floating) else t)(jnp.asarray(a))

    def _A_setup():
        B, S, D = (1, 2048, 640)
        ks = 4
        return {'q': _w((lambda *s: _rng.normal(s) * 0.05)(B, S, D)), 'k': _w((lambda *s: _rng.normal(s) * 0.05)(B, S, D)), 'v': _w((lambda *s: _rng.normal(s) * 0.05)(B, S, D)), 'shift_k': _w((lambda *s: _rng.normal(s) * 0.05)(D, ks) * 0.5), 'ssm_k': _w((lambda *s: _rng.normal(s) * 0.05)(D, S) * (1.0 / S ** 0.5)), 'ssm_D': _w((lambda *s: _rng.normal(s) * 0.05)(D))}
    _A_in = _A_setup()

    def _B_setup():
        B, S, D, F = (1, 2048, 640, 1536)
        return {'x': _w((lambda *s: _rng.normal(s) * 0.05)(B, S, D)), 'w1': _w((lambda *s: _rng.normal(s) * 0.05)(D, F) * (2.0 / D) ** 0.5), 'w3': _w((lambda *s: _rng.normal(s) * 0.05)(D, F) * (2.0 / D) ** 0.5), 'w2': _w((lambda *s: _rng.normal(s) * 0.05)(F, D) * (2.0 / F) ** 0.5)}
    _B_in = _B_setup()
    return {'A_q': _A_in['q'], 'A_k': _A_in['k'], 'A_v': _A_in['v'], 'A_shift_k': _A_in['shift_k'], 'A_ssm_k': _A_in['ssm_k'], 'A_ssm_D': _A_in['ssm_D'], 'B_x': _B_in['x'], 'B_w1': _B_in['w1'], 'B_w3': _B_in['w3'], 'B_w2': _B_in['w2'], 'c': _w((lambda *s: _rng.normal(s) * 0.05)(1, 640)), 'w_mod': _w((lambda *s: _rng.normal(s) * 0.05)(640, 6 * 640) * 640 ** (-0.5))}

def reference(A_q, A_k, A_v, A_shift_k, A_ssm_k, A_ssm_D, B_x, B_w1, B_w3, B_w2, c, w_mod):

    def _A_ref(q, k, v, shift_k, ssm_k, ssm_D):
        B, S, D = q.shape
        ks = shift_k.shape[-1]
        k_pad = jnp.pad(k, ((0, 0), (ks - 1, 0), (0, 0)))
        k_shift = jnp.zeros_like(k)
        for t in range(ks):
            k_shift = k_shift + k_pad[:, t:t + S, :] * shift_k[:, ks - 1 - t][None, None, :]
        kv = k_shift * v
        L = 2 * S
        kv_pad = jnp.pad(kv, ((0, 0), (0, S), (0, 0)))
        kf_pad = jnp.pad(ssm_k, ((0, 0), (0, S)))
        kv_f = (lambda x, axes=(-2, -1): jnp.fft.rfft2(x.astype(jnp.float32), axes=axes))(kv_pad[:, None, :, :], axes=(1, 2))
        kf_f = (lambda x, axes=(-2, -1): jnp.fft.rfft2(x.astype(jnp.float32), axes=axes))(kf_pad[:, None, :], axes=(1, 2))
        kf_f = (lambda x, *d: x.transpose(*d))(kf_f, 1, 2, 0)
        y_f = kv_f * kf_f[None, :, :, :]
        y = (lambda x, s, axes=(-2, -1): jnp.fft.irfft2(x, s=s, axes=axes).astype(jnp.bfloat16))(y_f, (1, L), axes=(1, 2))[:, 0, :S, :]
        y = y + kv * ssm_D[None, None, :]
        return q * y

    def _B_ref(x, w1, w3, w2):
        gate = jnp.einsum('bsd,df->bsf', x, w1)
        up = jnp.einsum('bsd,df->bsf', x, w3)
        h = _silu(gate) * up
        out = jnp.einsum('bsf,fd->bsd', h, w2)
        return out
    x = A_q
    mod = (_silu(c) @ w_mod).reshape(c.shape[0], 6, 1, -1)
    sa, ca, ga, sb, cb, gb = (mod[:, 0].copy(), mod[:, 1].copy(), mod[:, 2].copy(), mod[:, 3].copy(), mod[:, 4].copy(), mod[:, 5].copy())
    h = _layernorm(x, axis=-1) * (1 + ca) + sa
    x = x + ga * _A_ref(h, A_k, A_v, A_shift_k, A_ssm_k, A_ssm_D)
    h = _layernorm(x, axis=-1) * (1 + cb) + sb
    x = x + gb * _B_ref(h, B_w1, B_w3, B_w2)
    return x
```

```python
import functools
import numpy as np
import jax, jax.numpy as jnp
from jax import lax
from jax.experimental import pallas as pl
from jax.experimental.pallas import tpu as pltpu

S, D, F = 2048, 640, 1536
C = 128
NBLK = S // (2 * C)
NL = D // 128
f32, bf16, u32 = jnp.float32, jnp.bfloat16, jnp.uint32


def _dft_consts():
    f = np.concatenate([np.arange(0, C, 2), np.arange(1, C, 2)])
    zeta = 2 * np.pi * (f + 0.5) / (4 * C)

    def fwd(n):
        ang = zeta[:, None] * n[None, :]
        m = np.stack([np.cos(ang), -np.sin(ang)], 0)
        return m.reshape(2, C // 8, 8, C).transpose(1, 0, 2, 3).reshape(2 * C, C)

    def inv(n):
        ang = n[:, None] * zeta[None, :]
        return np.stack([np.cos(ang), -np.sin(ang)], -1).reshape(C, 2 * C) / (2 * C)

    j = np.arange(C)
    lane = (j // 2) * 2 + (j % 2) * C
    fw = np.concatenate([fwd(2 * j), fwd(2 * j + 1), fwd(lane), fwd(lane + 1)], 0)
    iv = np.concatenate([inv(2 * j), inv(2 * j + 1)], 0)
    return fw.astype(np.float32), iv.astype(np.float32)


def _merge(a, b):
    out, i, j = [], 0, 0
    while i < len(a) or j < len(b):
        if j >= len(b) or (i < len(a) and (i + 0.5) * len(b) <= (j + 0.5) * len(a)):
            out.append(a[i]); i += 1
        else:
            out.append(b[j]); j += 1
    return out


def build(R=256, TF=512, mul3=False, LR=32, do_conv=True, uload=True, skew=4, koff=2, early=True, do_ffn=True):
    NS = S // R
    fwd_np, inv_np = _dft_consts()
    nc = 2
    NT = C // 8
    BS = (2 * nc * NT + skew) * 8
    def addr(a, j, t, c):
        return (j % 2) * BS + ((j // 2) * 2 * skew % 16) * 8 + (a * koff + t * nc + c) * 8

    def kern(q_hbm, k_hbm, v_hbm, shk_ref, ssm_hbm, d_ref, w1_hbm, w3_hbm, w2_hbm, c_ref, wm_hbm,
             fwd_ref, inv_ref, o_hbm,
             qb, kb, vb, sb, w1, w3, w2, wm, xs, ks, kf32, zb, yb, cpar, zero_s, par, x1b, h2b, ob, sem_in, sem_w, sem_o):
        def slab_copies(l):
            cs = pl.ds(l * 128, 128)
            return [
                pltpu.make_async_copy(ssm_hbm.bitcast(u32).at[pl.ds(l * 64, 64)], sb.at[l], sem_in.at[0, l]),
                pltpu.make_async_copy(k_hbm.bitcast(u32).at[:, cs], kb.at[l, pl.ds(8, S // 2)], sem_in.at[1, l]),
                pltpu.make_async_copy(v_hbm.bitcast(u32).at[:, cs], vb.at[l], sem_in.at[2, l]),
            ]
        def out_copy(s):
            r0 = pl.multiple_of(s * R, R) if not isinstance(s, int) else s * R
            return pltpu.make_async_copy(ob.at[pl.ds(r0, R)], o_hbm.at[pl.ds(r0, R)], sem_o.at[s])
        wm_copy = pltpu.make_async_copy(wm_hbm.bitcast(u32), wm, sem_w.at[0])
        q0_copy = pltpu.make_async_copy(q_hbm.at[pl.ds(0, R)], qb.at[pl.ds(0, R)], sem_w.at[5])
        q_copy = pltpu.make_async_copy(q_hbm.at[pl.ds(R, S - R)], qb.at[pl.ds(R, S - R)], sem_w.at[1])
        w1_copy = pltpu.make_async_copy(w1_hbm.bitcast(u32), w1, sem_w.at[2])
        w3_copy = pltpu.make_async_copy(w3_hbm.bitcast(u32), w3, sem_w.at[3])
        w2_copy = pltpu.make_async_copy(w2_hbm.bitcast(u32), w2, sem_w.at[4])

        for l in range(NL):
            for cp in slab_copies(l): cp.start()
        wm_copy.start(); q0_copy.start(); w1_copy.start(); w3_copy.start(); w2_copy.start(); q_copy.start()

        def wload(w, r0, r1, c0, c1):
            return pltpu.bitcast(w[r0 // 2:r1 // 2, c0:c1], bf16)

        shk = shk_ref[...].astype(f32)
        dd = d_ref[...].astype(f32).reshape(1, D)
        for l in range(NL):
            kb[l, 0:8, :] = jnp.zeros((8, 128), u32)
            for j in range(4):
                cpar[l, j] = jnp.broadcast_to(shk[j:j + 1, l * 128:(l + 1) * 128], (8, 128))
            cpar[l, 4] = jnp.broadcast_to(dd[:, l * 128:(l + 1) * 128], (8, 128))

        zero_s[0] = 0
        H = C // 2
        def conv_slab(l, carry):
            for cp in slab_copies(l): cp.wait()
            bc = lambda j, rows: jnp.broadcast_to(cpar[l, j, 0:1, :], (rows, 128))
            kprev = {}
            z0 = pl.multiple_of(zero_s[0] * 1024, 1024)

            unpack = lambda w, i: pltpu.unpack_elementwise(w, index=i, packed_dtype=bf16, unpacked_dtype=f32)
            pack = lambda a, b: pltpu.bitcast(pltpu.pack_elementwise([a, b], packed_dtype=bf16), u32)
            fw = lambda i: fwd_ref[i * 2 * C:(i + 1) * 2 * C, :]

            def xdft(j):
                def f():
                    kw = kb[l, j * C:j * C + C + 8, :]
                    ke, ko = unpack(kw, 0), unpack(kw, 1)
                    kf32[j][0] = ke
                    kf32[j][1] = ko
                    ke1, ko1, ko2 = kf32[j][0, 7:7 + C, :], kf32[j][1, 7:7 + C, :], kf32[j][1, 6:6 + C, :]
                    ke, ko = ke[8:], ko[8:]
                    w0, w1_, w2_, w3_ = (bc(t, C) for t in range(4))
                    se = w0 * ke + w1_ * ko1 + w2_ * ke1 + w3_ * ko2
                    so = w0 * ko + w1_ * ke + w2_ * ko1 + w3_ * ke1
                    vw = vb[l, j * C:(j + 1) * C, :]
                    pe = jnp.dot(fw(0), (se * unpack(vw, 0)).astype(bf16), preferred_element_type=f32)
                    qo = jnp.dot(fw(1), (so * unpack(vw, 1)).astype(bf16), preferred_element_type=f32)
                    a0 = addr(0, j, 0, 0)
                    xs[j // 2][a0:a0 + 2 * C, :] = pe + qo
                    xs[j // 2][a0 + 2 * C:a0 + 4 * C, :] = pe - qo
                return f

            def kdft(j):
                def f():
                    ta = sb[l, :, 2 * j * C:(2 * j + 1) * C]
                    tb = sb[l, :, (2 * j + 1) * C:(2 * j + 2) * C]
                    even = lax.broadcasted_iota(jnp.int32, ta.shape, 1) % 2 == 0
                    te = jnp.where(even, ta, pltpu.roll(tb, 1, 1))
                    to = jnp.where(even, pltpu.roll(ta, C - 1, 1), tb)
                    nt = (((1,), (1,)), ((), ()))
                    pe = lax.dot_general(fw(2), pltpu.bitcast(te, bf16), nt, preferred_element_type=f32)
                    qo = lax.dot_general(fw(3), pltpu.bitcast(to, bf16), nt, preferred_element_type=f32)
                    for t in range(NT):
                        pr_, pi_ = pe[16 * t:16 * t + 8], pe[16 * t + 8:16 * t + 16]
                        qr_, qi_ = qo[16 * t:16 * t + 8], qo[16 * t + 8:16 * t + 16]
                        if j == 0:
                            pr_ = pr_ + bc(4, 8)
                        for hf in range(2):
                            kr, ki = (pr_ + qr_, pi_ + qi_) if hf == 0 else (pr_ - qr_, pi_ - qi_)
                            if j == 0:
                                nr, ni = kr, ki
                            else:
                                pr, pi = kprev[hf, t]
                                nr, ni = (kr - pi, ki + pr) if t < NT // 2 else (kr + pi, ki - pr)
                            kprev[hf, t] = kr, ki
                            for c, val in enumerate([nr, ni]):
                                a0 = addr(1, j, hf * NT + t, c)
                                ks[j // 2][a0:a0 + 8, :] = val
                return f

            def mac(p, t):
                def f():
                    res = []
                    for hf in range(2):
                        tt = hf * NT + t
                        acc = [None, None]
                        xc = {}
                        for m in range(2 * p + 2):
                            kk = [ks[m // 2][pl.ds(z0 + addr(1, m, tt, c), 8), :] for c in range(nc)]
                            for i in range(2):
                                j = 2 * p + i - m
                                if j < 0: continue
                                if j not in xc:
                                    xc[j] = [xs[j // 2][pl.ds(z0 + addr(0, j, tt, c), 8), :] for c in range(nc)]
                                xx = xc[j]
                                term = [kk[0] * xx[0] - kk[1] * xx[1], kk[0] * xx[1] + kk[1] * xx[0]]
                                acc[i] = term if acc[i] is None else [a + b for a, b in zip(acc[i], term)]
                        res.append(acc)
                    for i in range(2):
                        (ar, ai), (br, bi) = res[0][i], res[1][i]
                        zb[2 * p + i, 0, 8 * t:8 * t + 8, :] = pack(ar + br, ai + bi)
                        zb[2 * p + i, 1, 8 * t:8 * t + 8, :] = pack(ar - br, ai - bi)
                return f

            def idft(j):
                def f():
                    ye = jnp.dot(inv_ref[0:C, :], pltpu.bitcast(zb[j, 0], bf16), preferred_element_type=f32)
                    yo = jnp.dot(inv_ref[C:2 * C, :], pltpu.bitcast(zb[j, 1], bf16), preferred_element_type=f32)
                    yb[l, j * C:(j + 1) * C, :] = pack(ye, yo)
                return f

            NP = NBLK // 2
            for f in (xdft(0), kdft(0), xdft(1), kdft(1)): f()
            for p in range(NP):
                other = []
                if p + 1 < NP:
                    other += [xdft(2 * p + 2), kdft(2 * p + 2), xdft(2 * p + 3), kdft(2 * p + 3)]
                if p > 0:
                    other += [idft(2 * p - 2), idft(2 * p - 1)]
                for f in _merge([mac(p, t) for t in range(NT)], other): f()
            idft(NBLK - 2)(); idft(NBLK - 1)()
            return carry
        if do_conv:
            lax.fori_loop(0, NL, conv_slab, 0)
        else:
            for l in range(NL):
                for cp in slab_copies(l): cp.wait()
            yb[...] = jnp.zeros(yb.shape, u32)

        wm_copy.wait()
        cc = c_ref[...].astype(f32)
        sc = jnp.broadcast_to(cc * jax.nn.sigmoid(cc), (16, D)).astype(bf16)
        sa, ca, ga, sb_, cb, gb = [
            jnp.dot(sc, wload(wm, 0, D, j * D, (j + 1) * D), preferred_element_type=f32)[0:8] for j in range(6)]
        par[0] = ga * (1.0 + ca)
        par[1] = ga * sa
        par[2] = 1.0 + cb
        par[3] = sb_
        par[4] = gb
        pb = lambda j, rows: jnp.broadcast_to(par[j, 0:1, :], (rows, D))

        def ln(x):
            mu = jnp.sum(x, axis=-1, keepdims=True) * (1.0 / D)
            xc = x - mu
            var = jnp.sum(xc * xc, axis=-1, keepdims=True) * (1.0 / D)
            return xc * lax.rsqrt(var + 1e-5)

        def pre_pieces(s):
            slot = s % 2 if isinstance(s, int) else lax.rem(s, 2)
            def piece(i):
                def f():
                    r = s * R + i * LR
                    if not isinstance(r, int): r = pl.multiple_of(r, LR)
                    x = qb[pl.ds(r, LR), :].astype(f32)
                    r2 = r // 2 if isinstance(r, int) else pl.multiple_of(s * (R // 2) + i * (LR // 2), LR // 2)
                    y = jnp.concatenate([pltpu.bitcast(yb[l, pl.ds(r2, LR // 2), :], bf16).astype(f32)
                                         for l in range(NL)], axis=1)
                    x1 = x + (ln(x) * pb(0, LR) + pb(1, LR)) * y
                    h2 = ln(x1) * pb(2, LR) + pb(3, LR)
                    x1b[slot, i * LR:(i + 1) * LR, :] = x1
                    h2b[slot, i * LR // 2:(i + 1) * LR // 2, :] = pltpu.bitcast(h2.astype(bf16), u32)
                return f
            return [piece(i) for i in range(R // LR)]

        def ffn_pieces(s, ups_first=False):
            slot = s % 2 if isinstance(s, int) else lax.rem(s, 2)
            r0 = s * R if isinstance(s, int) else pl.multiple_of(s * R, R)
            st = {}
            nt = F // TF
            def gate(t):
                def f():
                    h = pltpu.bitcast(h2b[slot], bf16)
                    st['g', t] = jnp.dot(h, wload(w1, 0, D, t * TF, (t + 1) * TF), preferred_element_type=f32)
                return f
            def up(t):
                def f():
                    h = pltpu.bitcast(h2b[slot], bf16)
                    u = jnp.dot(h, wload(w3, 0, D, t * TF, (t + 1) * TF), preferred_element_type=f32)
                    hg = 0.5 * st['g', t]
                    st['a', t] = ((hg * jnp.tanh(hg) + hg) * u).astype(bf16)
                return f
            def down(t):
                def f():
                    p = jnp.dot(st['a', t], wload(w2, t * TF, (t + 1) * TF, 0, D), preferred_element_type=f32)
                    st['acc'] = p if t == 0 else st['acc'] + p
                return f
            P = [gate(0), up(0)]
            for t in range(nt):
                if t + 1 < nt: P += [gate(t + 1), up(t + 1)]
                P.append(down(t))
            if ups_first:
                P = [f for t in range(nt) for f in (gate(t), up(t))] + [down(t) for t in range(nt)]
            def fin():
                ob[pl.ds(r0, R), :] = (x1b[slot] + pb(4, R) * st['acc']).astype(bf16)
                out_copy(s).start()
            P.append(fin)
            return P

        q0_copy.wait()
        for f in pre_pieces(0): f()
        w1_copy.wait(); w3_copy.wait()
        if do_ffn:
            def body(s, carry):
                fp = ffn_pieces(s)
                for f in _merge(fp[:-1], pre_pieces(s + 1)) + [fp[-1]]: f()
                return carry
            if early:
                fp = ffn_pieces(0, True)
                nup = 2 * (F // TF)
                for f in fp[:nup]: f()
                w2_copy.wait(); q_copy.wait()
                for f in _merge(fp[nup:-1], pre_pieces(1)) + [fp[-1]]: f()
            else:
                w2_copy.wait(); q_copy.wait()
            lax.fori_loop(1 if early else 0, NS - 1, body, 0)
            for f in ffn_pieces(NS - 1): f()
            for s in range(NS):
                out_copy(s).wait()
        else:
            ob[0:R, :] = x1b[0].astype(bf16)
            w2_copy.wait(); q_copy.wait()
            out_copy(0).start(); out_copy(0).wait()

    def f(A_q, A_k, A_v, A_shift_k, A_ssm_k, A_ssm_D, B_x, B_w1, B_w3, B_w2, c, w_mod):
        hbm = pl.BlockSpec(memory_space=pl.ANY)
        vm = pl.BlockSpec(memory_space=pltpu.VMEM)
        out = pl.pallas_call(
            kern,
            in_specs=[hbm, hbm, hbm, vm, hbm, vm, hbm, hbm, hbm, vm, hbm, vm, vm],
            out_specs=hbm,
            out_shape=jax.ShapeDtypeStruct((S, D), bf16),
            scratch_shapes=[
                pltpu.VMEM((S, D), bf16), pltpu.VMEM((NL, S // 2 + 8, 128), u32), pltpu.VMEM((NL, S // 2, 128), u32),
                pltpu.VMEM((NL, 64, S), u32),
                pltpu.VMEM((D // 2, F), u32), pltpu.VMEM((D // 2, F), u32), pltpu.VMEM((F // 2, D), u32),
                pltpu.VMEM((D // 2, 6 * D), u32),
                [pltpu.VMEM((2 * BS + 256, 128), f32) for _ in range(NBLK // 2)],
                [pltpu.VMEM((2 * BS + 256, 128), f32) for _ in range(NBLK // 2)],
                [pltpu.VMEM((2, C + 8, 128), f32) for _ in range(NBLK)],
                pltpu.VMEM((NBLK, 2, C, 128), u32),
                pltpu.VMEM((NL, S // 2, 128), u32),
                pltpu.VMEM((NL, 5, 8, 128), f32), pltpu.SMEM((1,), jnp.int32), pltpu.VMEM((5, 8, D), f32),
                pltpu.VMEM((2, R, D), f32), pltpu.VMEM((2, R // 2, D), u32),
                pltpu.VMEM((S, D), bf16),
                pltpu.SemaphoreType.DMA((3, NL)), pltpu.SemaphoreType.DMA((6,)), pltpu.SemaphoreType.DMA((NS,)),
            ],
            compiler_params=pltpu.CompilerParams(vmem_limit_bytes=100 * 2**20),
        )(A_q.reshape(S, D), A_k.reshape(S, D), A_v.reshape(S, D), A_shift_k.T, A_ssm_k, A_ssm_D,
          B_w1, B_w3, B_w2, c, w_mod, jnp.asarray(fwd_np, bf16), jnp.asarray(inv_np, bf16))
        return out.reshape(1, S, D)
    return f


@jax.jit
def pallas_adaLN_cond__ssm_conv_h3__glu_gated_swiglu__prompt_kernel(
    A_q: jax.Array,
    A_k: jax.Array,
    A_v: jax.Array,
    A_shift_k: jax.Array,
    A_ssm_k: jax.Array,
    A_ssm_D: jax.Array,
    B_x: jax.Array,
    B_w1: jax.Array,
    B_w3: jax.Array,
    B_w2: jax.Array,
    c: jax.Array,
    w_mod: jax.Array,
):
    return build()(A_q, A_k, A_v, A_shift_k, A_ssm_k, A_ssm_D, B_x, B_w1, B_w3, B_w2, c, w_mod)
```

```python
import contextlib
import functools
import numpy as np
import jax, jax.numpy as jnp
from jax import lax
from jax.experimental import pallas as pl
from jax.experimental.pallas import tpu as pltpu

S, D, F = 2048, 640, 1536
C = 128
NBLK = S // (2 * C)
NL = D // 128
f32, bf16, u32 = jnp.float32, jnp.bfloat16, jnp.uint32


def _dft_consts():
    f = np.concatenate([np.arange(0, C, 2), np.arange(1, C, 2)])
    zeta = 2 * np.pi * (f + 0.5) / (4 * C)

    def fwd(n):
        ang = zeta[:, None] * n[None, :]
        m = np.stack([np.cos(ang), -np.sin(ang)], 0)
        return m.reshape(2, C // 8, 8, C).transpose(1, 0, 2, 3).reshape(2 * C, C)

    def inv(n):
        ang = n[:, None] * zeta[None, :]
        return np.stack([np.cos(ang), -np.sin(ang)], -1).reshape(C, 2 * C) / (2 * C)

    j = np.arange(C)
    lane = (j // 2) * 2 + (j % 2) * C
    fw = np.concatenate([fwd(lane), fwd(lane + 1)], 0)
    iv = np.concatenate([inv(2 * j), inv(2 * j + 1)], 0)

    def words(m):
        b = np.asarray(m, np.float32).astype(jnp.bfloat16).view(np.uint16).astype(np.uint32)
        return b[0::2] | (b[1::2] << 16)
    return words(fw), words(iv)


def _merge(a, b):
    out, i, j = [], 0, 0
    while i < len(a) or j < len(b):
        if j >= len(b) or (i < len(a) and (i + 0.5) * len(b) <= (j + 0.5) * len(a)):
            out.append(a[i]); i += 1
        else:
            out.append(b[j]); j += 1
    return out


def build(R=256, TF=512, mul3=False, LR=32, do_conv=True, uload=True, skew=4, koff=2, early=True, do_ffn=True, scopes=False, unroll=1, m0=1, m1=2, nwait=3, wm5_early=True, flags=None, c0=2, PW=512, DW=640, mixud=False, pspan=0.9, dspan=0.9):
    sc_ = lambda n: jax.named_scope(n) if scopes else contextlib.nullcontext()
    NS = S // R
    fwd_np, inv_np = _dft_consts()
    nc = 2
    NT = C // 8
    BS = (2 * nc * NT + skew) * 8
    KO = (NBLK * BS + 511) // 512 * 512
    def addr(a, j, t, c):
        return a * KO + j * BS + (a * koff + t * nc + c) * 8

    def kern(q_hbm, k_hbm, v_hbm, shk_hbm, ssm_hbm, d_hbm, w1_hbm, w3_hbm, w2_hbm, c_hbm, wm_hbm,
             fwd_hbm, inv_hbm, o_hbm,
             shk_ref, d_ref, c_ref, fwd_ref, inv_ref, sem_s,
             qb, kb, vb, sb, w1, w3, w2, wm, xs, zl, kf32, zb, yb, cpar, zero_s, par, x1b, h2b, ob, sem_in, sem_w, sem_o):
        def slab_copies(l):
            cs = pl.ds(l * 128, 128)
            return [
                pltpu.make_async_copy(ssm_hbm.bitcast(u32).at[pl.ds(l * 64, 64)], sb.at[l], sem_in.at[0, l]),
                pltpu.make_async_copy(k_hbm.bitcast(u32).at[:, cs], kb.at[l, pl.ds(8, S // 2)], sem_in.at[1, l]),
                pltpu.make_async_copy(v_hbm.bitcast(u32).at[:, cs], vb.at[l], sem_in.at[2, l]),
            ]
        def out_copy(s):
            r0 = pl.multiple_of(s * R, R) if not isinstance(s, int) else s * R
            return pltpu.make_async_copy(ob.at[pl.ds(r0, R)], o_hbm.at[pl.ds(r0, R)], sem_o.at[s])
        nt = F // TF
        cps = {}
        def weight_copy(name, src, dst):
            cps[name] = pltpu.make_async_copy(src, dst, sem_w.at[len(cps)])
        wm32, w132, w332, w232 = (a.bitcast(u32) for a in (wm_hbm, w1_hbm, w3_hbm, w2_hbm))
        def add(kind, t):
            if kind == 'wm': weight_copy((kind, t), wm32.at[:, pl.ds(t * D, D)], wm.at[:, pl.ds(t * D, D)])
            if kind == 'w1': weight_copy((kind, t), w132.at[:, pl.ds(t * TF, TF)], w1.at[:, pl.ds(t * TF, TF)])
            if kind == 'w3': weight_copy((kind, t), w332.at[:, pl.ds(t * TF, TF)], w3.at[:, pl.ds(t * TF, TF)])
            if kind == 'w2': weight_copy((kind, t), w232.at[pl.ds(t * TF // 2, TF // 2)], w2.at[pl.ds(t * TF // 2, TF // 2)])
            if kind == 'q':
                rows = pl.ds(t * R, R if t < 2 else S - 2 * R)
                weight_copy((kind, t), q_hbm.at[rows], qb.at[rows])
        for kind, t in [('wm', 1), ('wm', 2), ('wm', 0), ('wm', 4), ('wm', 3), ('q', 0),
                        ('w1', 0), ('w3', 0), ('w1', 1), ('w3', 1), ('q', 1), ('w2', 0), ('w1', 2), ('w3', 2),
                        ('wm', 5), ('w2', 1), ('w2', 2), ('q', 2)]:
            add(kind, t)
        def wait(*name):
            with sc_('wait_' + name[0] + str(name[1])):
                cps[name].wait()

        small = [pltpu.make_async_copy(a, b, sem_s.at[i]) for i, (a, b) in enumerate(
            [(shk_hbm, shk_ref), (d_hbm, d_ref), (c_hbm, c_ref), (fwd_hbm, fwd_ref), (inv_hbm, inv_ref)])]
        for cp in small[:4]: cp.start()
        for l in range(NL):
            for cp in slab_copies(l): cp.start()
            if l == 0: small[4].start()
        for cp in cps.values(): cp.start()

        def wload(w, r0, r1, c0, c1):
            return pltpu.bitcast(w[r0 // 2:r1 // 2, c0:c1], bf16)

        for cp in small[:3]: cp.wait()
        shk = shk_ref[...].astype(f32)
        dd = d_ref[...].astype(f32).reshape(1, D)
        for l in range(NL):
            kb[l, 0:8, :] = jnp.zeros((8, 128), u32)
            for j in range(4):
                cpar[l, j] = jnp.broadcast_to(shk[j:j + 1, l * 128:(l + 1) * 128], (8, 128))
            cpar[l, 4] = jnp.broadcast_to(dd[:, l * 128:(l + 1) * 128], (8, 128))

        zero_s[0] = 0
        H = C // 2
        z0 = pl.multiple_of(zero_s[0] * 1024, 1024)
        unpack = lambda w, i: pltpu.unpack_elementwise(w, index=i, packed_dtype=bf16, unpacked_dtype=f32)
        pack = lambda a, b: pltpu.bitcast(pltpu.pack_elementwise([a, b], packed_dtype=bf16), u32)
        fw = lambda i: pltpu.bitcast(fwd_ref[i * C:(i + 1) * C, :], bf16)
        iv = lambda i: pltpu.bitcast(inv_ref[i * H:(i + 1) * H, :], bf16)
        halves = lambda x: pltpu.bitcast(pack(x[:H], x[H:]), bf16)

        def dft_pieces(l, buf):
            bc = lambda j, rows: jnp.broadcast_to(cpar[l, j, 0:1, :], (rows, 128))

            def wait():
                with sc_('wait_slab'):
                    for cp in slab_copies(l): cp.wait()

            def xdft(j):
                def f():
                    kw = kb[l, j * C:j * C + C + 8, :]
                    ke, ko = unpack(kw, 0), unpack(kw, 1)
                    kf32[j][0] = ke
                    kf32[j][1] = ko
                    ke1, ko1, ko2 = kf32[j][0, 7:7 + C, :], kf32[j][1, 7:7 + C, :], kf32[j][1, 6:6 + C, :]
                    ke, ko = ke[8:], ko[8:]
                    w0, w1_, w2_, w3_ = (bc(t, C) for t in range(4))
                    se = w0 * ke + w1_ * ko1 + w2_ * ke1 + w3_ * ko2
                    so = w0 * ko + w1_ * ke + w2_ * ko1 + w3_ * ke1
                    vw = vb[l, j * C:(j + 1) * C, :]
                    pe = jnp.dot(fw(0), halves(se * unpack(vw, 0)), preferred_element_type=f32)
                    qo = jnp.dot(fw(1), halves(so * unpack(vw, 1)), preferred_element_type=f32)
                    a0 = addr(0, j, 0, 0)
                    xs[buf][a0:a0 + 2 * C, :] = pe + qo
                    xs[buf][a0 + 2 * C:a0 + 4 * C, :] = pe - qo
                return f

            def kdft(j):
                def f():
                    ta = sb[l, :, 2 * j * C:(2 * j + 1) * C]
                    tb = sb[l, :, (2 * j + 1) * C:(2 * j + 2) * C]
                    even = lax.broadcasted_iota(jnp.int32, ta.shape, 1) % 2 == 0
                    te = jnp.where(even, ta, pltpu.roll(tb, 1, 1))
                    to = jnp.where(even, pltpu.roll(ta, C - 1, 1), tb)
                    nt = (((1,), (1,)), ((), ()))
                    pe = lax.dot_general(fw(0), pltpu.bitcast(te, bf16), nt, preferred_element_type=f32)
                    qo = lax.dot_general(fw(1), pltpu.bitcast(to, bf16), nt, preferred_element_type=f32)
                    if j == 0:
                        is_re = lax.broadcasted_iota(jnp.int32, pe.shape, 0) % 16 < 8
                        pe = pe + jnp.where(is_re, bc(4, 2 * C), 0.0)
                    a0 = addr(1, j, 0, 0)
                    xs[buf][a0:a0 + 2 * C, :] = pe + qo
                    xs[buf][a0 + 2 * C:a0 + 4 * C, :] = pe - qo
                return f
            return [wait] + [f(j) for j in range(NBLK) for f in (xdft, kdft)]

        def mac_pieces(l, buf, split=False):
            def mac(p, t):
                def f():
                    res = []
                    for hf in range(2):
                        tt = hf * NT + t
                        acc = [None, None]
                        xc = {}
                        for m in range(2 * p + 2):
                            kk = [xs[buf][pl.ds(z0 + addr(1, m, tt, c), 8), :] for c in range(nc)]
                            for i in range(2):
                                j = 2 * p + i - m
                                if j < 0: continue
                                if j not in xc:
                                    xc[j] = [xs[buf][pl.ds(z0 + addr(0, j, tt, c), 8), :] for c in range(nc)]
                                xx = xc[j]
                                term = [kk[0] * xx[0] - kk[1] * xx[1], kk[0] * xx[1] + kk[1] * xx[0]]
                                acc[i] = term if acc[i] is None else [a + b for a, b in zip(acc[i], term)]
                        zrow = tt * 16
                        def ovl(z, zp):
                            return [z[0] - zp[1], z[1] + zp[0]] if t < NT // 2 else [z[0] + zp[1], z[1] - zp[0]]
                        w1_ = ovl(acc[1], acc[0])
                        w0_ = acc[0]
                        if p > 0:
                            w0_ = ovl(acc[0], [zl[p - 1][pl.ds(z0 + zrow + 8 * c, 8), :] for c in range(2)])
                        if p + 1 < NBLK // 2:
                            for c in range(2):
                                zl[p][zrow + 8 * c:zrow + 8 * c + 8, :] = acc[1][c]
                        res.append([w0_, w1_])
                    for i in range(2):
                        (ar, ai), (br, bi) = res[0][i], res[1][i]
                        zb[2 * p + i, 0, 8 * t:8 * t + 8, :] = pack(ar + br, ai + bi)
                        zb[2 * p + i, 1, 8 * t:8 * t + 8, :] = pack(ar - br, ai - bi)
                return f

            def idft(j):
                def f():
                    ye = jnp.dot(iv(0), pltpu.bitcast(zb[j, 0], bf16), preferred_element_type=f32)
                    yo = jnp.dot(iv(1), pltpu.bitcast(zb[j, 1], bf16), preferred_element_type=f32)
                    yb[l, j * C:(j + 1) * C, :] = pack(ye, yo)
                return f

            if split:
                return ([(4 * p + 3 + c0, mac(p, t)) for p in range(NBLK // 2) for t in range(NT)],
                        [idft(j) for j in range(NBLK)])
            P = []
            for p in range(NBLK // 2):
                for t in range(NT):
                    P.append((4 * p + 3 + c0, mac(p, t)))
                    if p > 0 and t in (NT // 4, 3 * NT // 4):
                        P.append((0, idft(2 * p - 2 + (t > NT // 2))))
            return P + [(0, idft(NBLK - 2)), (0, idft(NBLK - 1))]

        def conv_step(l, buf, with_next):
            mp = mac_pieces(l, buf)
            dp = dft_pieces(l + 1, 1 - buf) if with_next else []
            total, done, k = sum(w for w, _ in mp), 0, 0
            for w, f in mp:
                while k < len(dp) and k * total <= done * len(dp) / dspan:
                    dp[k](); k += 1
                f(); done += w
            for f in dp[k:]: f()

        with sc_('conv'):
            small[3].wait()
            for f in dft_pieces(0, 0): f()
            small[4].wait()
            def conv_body(i, carry):
                conv_step(2 * i, 0, True)
                conv_step(2 * i + 1, 1, True)
                return carry
            lax.fori_loop(0, NL // 2, conv_body, 0)

        cc = c_ref[...].astype(f32)
        sc = jnp.broadcast_to(cc * jax.nn.sigmoid(cc), (16, D)).astype(bf16)
        mod = lambda j: jnp.dot(sc, wload(wm, 0, D, j * D, (j + 1) * D), preferred_element_type=f32)[0:8]
        def finish_mod():
            ca, ga, sa, cb, sb_ = (mod(j) for j in (1, 2, 0, 4, 3))
            par[0] = ga * (1.0 + ca)
            par[1] = ga * sa
            par[2] = 1.0 + cb
            par[3] = sb_
        pb = lambda j, rows: jnp.broadcast_to(par[j, 0:1, :], (rows, D))

        def ln(x):
            mu = jnp.sum(x, axis=-1, keepdims=True) * (1.0 / D)
            xc = x - mu
            var = jnp.sum(xc * xc, axis=-1, keepdims=True) * (1.0 / D)
            return xc * lax.rsqrt(var + 1e-5)

        def pre_pieces(s):
            slot = s % 2 if isinstance(s, int) else lax.rem(s, 2)
            def piece(i):
                def f():
                    r = s * R + i * LR
                    if not isinstance(r, int): r = pl.multiple_of(r, LR)
                    x = qb[pl.ds(r, LR), :].astype(f32)
                    r2 = r // 2 if isinstance(r, int) else pl.multiple_of(s * (R // 2) + i * (LR // 2), LR // 2)
                    y = jnp.concatenate([pltpu.bitcast(yb[l, pl.ds(r2, LR // 2), :], bf16).astype(f32)
                                         for l in range(NL)], axis=1)
                    x1 = x + (ln(x) * pb(0, LR) + pb(1, LR)) * y
                    h2 = ln(x1) * pb(2, LR) + pb(3, LR)
                    x1b[slot, i * LR:(i + 1) * LR, :] = x1
                    h2b[slot, i * LR // 2:(i + 1) * LR // 2, :] = pltpu.bitcast(h2.astype(bf16), u32)
                return f
            return [piece(i) for i in range(R // LR)]

        def ffn_pieces(s, ups_first=False):
            slot = s % 2 if isinstance(s, int) else lax.rem(s, 2)
            r0 = s * R if isinstance(s, int) else pl.multiple_of(s * R, R)
            st = {}
            def gate(c):
                def f():
                    h = pltpu.bitcast(h2b[slot], bf16)
                    st['g', c] = jnp.dot(h, wload(w1, 0, D, c, c + PW), preferred_element_type=f32)
                return f
            def up(c):
                def f():
                    h = pltpu.bitcast(h2b[slot], bf16)
                    u = jnp.dot(h, wload(w3, 0, D, c, c + PW), preferred_element_type=f32)
                    hg = 0.5 * st['g', c]
                    st['a', c] = ((hg * jnp.tanh(hg) + hg) * u).astype(bf16)
                return f
            def down(t, c0_, c1_):
                def f():
                    a = jnp.concatenate([st['a', c] for c in range(t * TF, (t + 1) * TF, PW)], axis=1)
                    p = jnp.dot(a, wload(w2, t * TF, (t + 1) * TF, c0_, c1_), preferred_element_type=f32)
                    st['acc', c0_] = p if t == 0 else st['acc', c0_] + p
                return f
            cols = list(range(0, D, DW))
            ups = [[(PW * D, f(c)) for c in range(t * TF, (t + 1) * TF, PW) for f in (gate, up)] for t in range(nt)]
            downs = [[(TF * DW, down(t, c, c + DW)) for c in cols] for t in range(nt)]
            if ups_first:
                G = ups + downs
            else:
                G = [ups[0]]
                for t in range(nt):
                    if t + 1 < nt: G.append(ups[t + 1] if not mixud else _merge(ups[t + 1], downs[t]))
                    if not mixud or t + 1 == nt: G.append(downs[t])
            def fin():
                acc = jnp.concatenate([st['acc', c] for c in cols], axis=1)
                ob[pl.ds(r0, R), :] = (x1b[slot] + pb(4, R) * acc).astype(bf16)
                out_copy(s).start()
            return G, fin

        def run_mixed(main, side):
            tm, ts = sum(w for w, _ in main), sum(w for w, _ in side)
            dm = ds = k = 0
            for w, f in main:
                f(); dm += w
                while k < len(side) and (ds + 0.5 * side[k][0]) * tm <= dm * ts:
                    side[k][1](); ds += side[k][0]; k += 1
            for _, f in side[k:]: f()

        mp, inv_ = mac_pieces(NL - 1, 0, True)
        n0 = NT * m0
        for _, f in mp[:n0]: f()
        for j in range(5): wait('wm', j)
        wait('q', 0)
        finish_mod()
        for _, f in mp[n0:NT * m1]: f()
        inv_[0](); inv_[1]()
        run_mixed(mp[NT * max(m0, m1):], [(1, f) for f in pre_pieces(0)])
        for f in inv_[2:]: f()
        if do_ffn:
            def body(s, carry):
                G, fin = ffn_pieces(s)
                main = [p for g in G for p in g]
                n = int(len(main) * pspan)
                run_mixed(main[:n], [(1, f) for f in pre_pieces(s + 1)])
                run_mixed(main[n:], [])
                fin()
                return carry
            G, fin = ffn_pieces(0)
            pp = [(1, f) for f in pre_pieces(1)]
            for t in range(2): wait('w1', t); wait('w3', t)
            run_mixed(G[0] + G[1], [])
            wait('w2', 0); wait('w1', 2); wait('w3', 2); wait('q', 1)
            run_mixed(G[2] + G[3], pp[:len(pp) // 2])
            wait('w2', 1); wait('wm', 5)
            par[4] = mod(5)
            run_mixed(G[4], pp[len(pp) // 2:])
            wait('w2', 2)
            run_mixed(G[5], [])
            fin()
            wait('q', 2)
            with sc_('ffn_loop'):
                lax.fori_loop(1, NS - 1, body, 0, unroll=unroll)
            G, fin = ffn_pieces(NS - 1)
            run_mixed([p for g in G for p in g], [])
            fin()
            with sc_('wait_out'):
                for s in range(NS):
                    out_copy(s).wait()
        else:
            ob[0:R, :] = x1b[0].astype(bf16)
            w2_copy.wait(); q_copy.wait()
            out_copy(0).start(); out_copy(0).wait()

    def f(A_q, A_k, A_v, A_shift_k, A_ssm_k, A_ssm_D, B_x, B_w1, B_w3, B_w2, c, w_mod):
        hbm = pl.BlockSpec(memory_space=pl.ANY)
        vm = pl.BlockSpec(memory_space=pltpu.VMEM)
        out = pl.pallas_call(
            kern,
            in_specs=[hbm] * 13,
            out_specs=hbm,
            out_shape=jax.ShapeDtypeStruct((S, D), bf16),
            scratch_shapes=[
                pltpu.VMEM((4, D), bf16), pltpu.VMEM((D,), bf16), pltpu.VMEM((1, D), bf16),
                pltpu.VMEM(fwd_np.shape, u32), pltpu.VMEM(inv_np.shape, u32), pltpu.SemaphoreType.DMA((5,)),
                pltpu.VMEM((S, D), bf16), pltpu.VMEM((NL, S // 2 + 8, 128), u32), pltpu.VMEM((NL, S // 2, 128), u32),
                pltpu.VMEM((NL, 64, S), u32),
                pltpu.VMEM((D // 2, F), u32), pltpu.VMEM((D // 2, F), u32), pltpu.VMEM((F // 2, D), u32),
                pltpu.VMEM((D // 2, 6 * D), u32),
                [pltpu.VMEM((2 * KO + 512, 128), f32) for _ in range(2)],
                [pltpu.VMEM((4 * C, 128), f32) for _ in range(NBLK // 2 - 1)],
                [pltpu.VMEM((2, C + 8, 128), f32) for _ in range(NBLK)],
                pltpu.VMEM((NBLK, 2, C, 128), u32),
                pltpu.VMEM((NL, S // 2, 128), u32),
                pltpu.VMEM((NL, 5, 8, 128), f32), pltpu.SMEM((1,), jnp.int32), pltpu.VMEM((5, 8, D), f32),
                pltpu.VMEM((2, R, D), f32), pltpu.VMEM((2, R // 2, D), u32),
                pltpu.VMEM((S, D), bf16),
                pltpu.SemaphoreType.DMA((3, NL)), pltpu.SemaphoreType.DMA((9 + 3 * (F // TF),)), pltpu.SemaphoreType.DMA((NS,)),
            ],
            compiler_params=pltpu.CompilerParams(vmem_limit_bytes=100 * 2**20, flags=flags),
        )(A_q.reshape(S, D), A_k.reshape(S, D), A_v.reshape(S, D), A_shift_k.T, A_ssm_k, A_ssm_D,
          B_w1, B_w3, B_w2, c, w_mod, fwd_np, inv_np)
        return out.reshape(1, S, D)
    return f


@jax.jit
def pallas_adaLN_cond__ssm_conv_h3__glu_gated_swiglu__prompt_kernel(
    A_q: jax.Array,
    A_k: jax.Array,
    A_v: jax.Array,
    A_shift_k: jax.Array,
    A_ssm_k: jax.Array,
    A_ssm_D: jax.Array,
    B_x: jax.Array,
    B_w1: jax.Array,
    B_w3: jax.Array,
    B_w2: jax.Array,
    c: jax.Array,
    w_mod: jax.Array,
):
    return build()(A_q, A_k, A_v, A_shift_k, A_ssm_k, A_ssm_D, B_x, B_w1, B_w3, B_w2, c, w_mod)
```

```python
import contextlib
import functools
import numpy as np
import jax, jax.numpy as jnp
from jax import lax
from jax.experimental import pallas as pl
from jax.experimental.pallas import tpu as pltpu

S, D, F = 2048, 640, 1536
C = 128
NBLK = S // (2 * C)
NL = D // 128
f32, bf16, u32 = jnp.float32, jnp.bfloat16, jnp.uint32


def _dft_consts():
    f = np.concatenate([np.arange(0, C, 2), np.arange(1, C, 2)])
    zeta = 2 * np.pi * (f + 0.5) / (4 * C)

    def fwd(n):
        ang = zeta[:, None] * n[None, :]
        m = np.stack([np.cos(ang), -np.sin(ang)], 0)
        return m.reshape(2, C // 8, 8, C).transpose(1, 0, 2, 3).reshape(2 * C, C)

    def inv(n):
        ang = n[:, None] * zeta[None, :]
        return np.stack([np.cos(ang), -np.sin(ang)], -1).reshape(C, 2 * C) / (2 * C)

    j = np.arange(C)
    lane = (j // 2) * 2 + (j % 2) * C
    fw = np.concatenate([fwd(lane), fwd(lane + 1)], 0)
    iv = np.concatenate([inv(2 * j), inv(2 * j + 1)], 0)

    def words(m):
        b = np.asarray(m, np.float32).astype(jnp.bfloat16).view(np.uint16).astype(np.uint32)
        return b[0::2] | (b[1::2] << 16)
    return words(fw), words(iv)


def _merge(a, b):
    out, i, j = [], 0, 0
    while i < len(a) or j < len(b):
        if j >= len(b) or (i < len(a) and (i + 0.5) * len(b) <= (j + 0.5) * len(a)):
            out.append(a[i]); i += 1
        else:
            out.append(b[j]); j += 1
    return out


def build(R=256, TF=512, mul3=False, LR=32, do_conv=True, uload=True, skew=4, koff=2, early=True, do_ffn=True, scopes=False, unroll=1, NF=2, dstart=0.0, pfr=0.5, tailsplit=True, kfirst=False, sep=0, inv_late=True, zop=True, ipos=(4, 12), x_noinv=False, x_nox=False, x_nok=False, nochecks=False, m0=1, m1=2, nwait=3, wm5_early=True, flags=None, c0=2, PW=512, DW=(0, 256, 512, 640), mixud=False, pspan=0.9, dspan=0.9):
    sc_ = lambda n: jax.named_scope(n) if scopes else contextlib.nullcontext()
    NS = S // R
    fwd_np, inv_np = _dft_consts()
    nc = 2
    NT = C // 8
    BS = (2 * nc * NT + skew) * 8
    KO = (NBLK * BS + 511) // 512 * 512
    def addr(a, j, t, c):
        return a * KO + j * BS + (a * koff + t * nc + c) * 8

    def kern(q_hbm, k_hbm, v_hbm, shk_hbm, ssm_hbm, d_hbm, w1_hbm, w3_hbm, w2_hbm, c_hbm, wm_hbm,
             fwd_hbm, inv_hbm, o_hbm,
             shk_ref, d_ref, c_ref, fwd_ref, inv_ref, sem_s,
             qb, kb, vb, sb, w1, w3, w2, wm, xs, zl, kf32, zb, yb, cpar, zero_s, par, x1b, h2b, ob, sem_in, sem_f, sem_w, sem_o):
        def slab_copies(l):
            cs = pl.ds(l * 128, 128)
            return [
                pltpu.make_async_copy(ssm_hbm.bitcast(u32).at[pl.ds(l * 64, 64)], sb.at[l], sem_in.at[0, l]),
                pltpu.make_async_copy(k_hbm.bitcast(u32).at[:, cs], kb.at[l, pl.ds(8, S // 2)], sem_in.at[1, l]),
                pltpu.make_async_copy(v_hbm.bitcast(u32).at[:, cs], vb.at[l], sem_in.at[2, l]),
            ]
        def first_copies(h):
            cs, n = pl.ds(0, 128), S // NF
            return [
                pltpu.make_async_copy(ssm_hbm.bitcast(u32).at[pl.ds(0, 64), pl.ds(h * n, n)],
                                      sb.at[0, :, pl.ds(h * n, n)], sem_f.at[0, h]),
                pltpu.make_async_copy(k_hbm.bitcast(u32).at[pl.ds(h * n // 2, n // 2), cs],
                                      kb.at[0, pl.ds(8 + h * n // 2, n // 2)], sem_f.at[1, h]),
                pltpu.make_async_copy(v_hbm.bitcast(u32).at[pl.ds(h * n // 2, n // 2), cs],
                                      vb.at[0, pl.ds(h * n // 2, n // 2)], sem_f.at[2, h]),
            ]
        def last_copy(c0_, c1_):
            idx = (pl.ds(S - R, R), pl.ds(c0_, c1_ - c0_))
            return pltpu.make_async_copy(ob.at[idx], o_hbm.at[idx], sem_o.at[NS + DW.index(c0_)])
        def out_copy(s):
            r0 = pl.multiple_of(s * R, R) if not isinstance(s, int) else s * R
            return pltpu.make_async_copy(ob.at[pl.ds(r0, R)], o_hbm.at[pl.ds(r0, R)], sem_o.at[s])
        nt = F // TF
        cps = {}
        def weight_copy(name, src, dst):
            cps[name] = pltpu.make_async_copy(src, dst, sem_w.at[len(cps)])
        wm32, w132, w332, w232 = (a.bitcast(u32) for a in (wm_hbm, w1_hbm, w3_hbm, w2_hbm))
        def add(kind, t):
            if kind == 'wm': weight_copy((kind, t), wm32.at[:, pl.ds(t * D, D)], wm.at[:, pl.ds(t * D, D)])
            if kind == 'w1': weight_copy((kind, t), w132.at[:, pl.ds(t * TF, TF)], w1.at[:, pl.ds(t * TF, TF)])
            if kind == 'w3': weight_copy((kind, t), w332.at[:, pl.ds(t * TF, TF)], w3.at[:, pl.ds(t * TF, TF)])
            if kind == 'w2': weight_copy((kind, t), w232.at[pl.ds(t * TF // 2, TF // 2)], w2.at[pl.ds(t * TF // 2, TF // 2)])
            if kind == 'q':
                rows = pl.ds(t * R, R if t < 2 else S - 2 * R)
                weight_copy((kind, t), q_hbm.at[rows], qb.at[rows])
        for kind, t in [('wm', 1), ('wm', 2), ('wm', 0), ('wm', 4), ('wm', 3), ('q', 0),
                        ('w1', 0), ('w3', 0), ('w1', 1), ('w3', 1), ('q', 1), ('w2', 0), ('w1', 2), ('w3', 2),
                        ('wm', 5), ('w2', 1), ('w2', 2), ('q', 2)]:
            add(kind, t)
        def wait(*name):
            with sc_('wait_' + name[0] + str(name[1])):
                cps[name].wait()

        small = [pltpu.make_async_copy(a, b, sem_s.at[i]) for i, (a, b) in enumerate(
            [(shk_hbm, shk_ref), (d_hbm, d_ref), (c_hbm, c_ref), (fwd_hbm, fwd_ref), (inv_hbm, inv_ref)])]
        for cp in small[:4]: cp.start()
        for h in range(NF):
            for cp in first_copies(h): cp.start()
        if not inv_late: small[4].start()
        for l in range(1, NL):
            for cp in slab_copies(l): cp.start()
            if l == 1 and inv_late: small[4].start()
        for cp in cps.values(): cp.start()

        def wload(w, r0, r1, c0, c1):
            return pltpu.bitcast(w[r0 // 2:r1 // 2, c0:c1], bf16)

        for cp in small[:3]: cp.wait()
        shk = shk_ref[...].astype(f32)
        dd = d_ref[...].astype(f32).reshape(1, D)
        for l in range(NL):
            kb[l, 0:8, :] = jnp.zeros((8, 128), u32)
            for j in range(4):
                cpar[l, j] = jnp.broadcast_to(shk[j:j + 1, l * 128:(l + 1) * 128], (8, 128))
            cpar[l, 4] = jnp.broadcast_to(dd[:, l * 128:(l + 1) * 128], (8, 128))

        zero_s[0] = 0
        H = C // 2
        z0 = pl.multiple_of(zero_s[0] * 1024, 1024)
        unpack = lambda w, i: pltpu.unpack_elementwise(w, index=i, packed_dtype=bf16, unpacked_dtype=f32)
        pack = lambda a, b: pltpu.bitcast(pltpu.pack_elementwise([a, b], packed_dtype=bf16), u32)
        fw = lambda i: pltpu.bitcast(fwd_ref[i * C:(i + 1) * C, :], bf16)
        iv = lambda i: pltpu.bitcast(inv_ref[i * H:(i + 1) * H, :], bf16)
        halves = lambda x: pltpu.bitcast(pack(x[:H], x[H:]), bf16)

        def dft_pieces(l, buf):
            bc = lambda j, rows: jnp.broadcast_to(cpar[l, j, 0:1, :], (rows, 128))

            def wait():
                with sc_('wait_slab'):
                    for cp in slab_copies(l): cp.wait()

            kvs = {}
            def xprep(j):
                def f():
                    kw = kb[l, j * C:j * C + C + 8, :]
                    ke, ko = unpack(kw, 0), unpack(kw, 1)
                    kf32[j][0] = ke
                    kf32[j][1] = ko
                    ke1, ko1, ko2 = kf32[j][0, 7:7 + C, :], kf32[j][1, 7:7 + C, :], kf32[j][1, 6:6 + C, :]
                    ke, ko = ke[8:], ko[8:]
                    w0, w1_, w2_, w3_ = (bc(t, C) for t in range(4))
                    se = w0 * ke + w1_ * ko1 + w2_ * ke1 + w3_ * ko2
                    so = w0 * ko + w1_ * ke + w2_ * ko1 + w3_ * ke1
                    vw = vb[l, j * C:(j + 1) * C, :]
                    kvs[j] = halves(se * unpack(vw, 0)), halves(so * unpack(vw, 1))
                return f

            def xdft(j):
                def f():
                    if j not in kvs: xprep(j)()
                    pe = jnp.dot(fw(0), kvs[j][0], preferred_element_type=f32)
                    qo = jnp.dot(fw(1), kvs[j][1], preferred_element_type=f32)
                    a0 = addr(0, j, 0, 0)
                    xs[buf][a0:a0 + 2 * C, :] = pe + qo
                    xs[buf][a0 + 2 * C:a0 + 4 * C, :] = pe - qo
                    if sep and j + 1 < NBLK and not (isinstance(l, int) and l == 0): xprep(j + 1)()
                return f

            def kdft(j):
                def f():
                    ta = sb[l, :, 2 * j * C:(2 * j + 1) * C]
                    tb = sb[l, :, (2 * j + 1) * C:(2 * j + 2) * C]
                    even = lax.broadcasted_iota(jnp.int32, ta.shape, 1) % 2 == 0
                    te = jnp.where(even, ta, pltpu.roll(tb, 1, 1))
                    to = jnp.where(even, pltpu.roll(ta, C - 1, 1), tb)
                    nt = (((1,), (1,)), ((), ()))
                    pe = lax.dot_general(fw(0), pltpu.bitcast(te, bf16), nt, preferred_element_type=f32)
                    qo = lax.dot_general(fw(1), pltpu.bitcast(to, bf16), nt, preferred_element_type=f32)
                    if j == 0:
                        is_re = lax.broadcasted_iota(jnp.int32, pe.shape, 0) % 16 < 8
                        pe = pe + jnp.where(is_re, bc(4, 2 * C), 0.0)
                    a0 = addr(1, j, 0, 0)
                    xs[buf][a0:a0 + 2 * C, :] = pe + qo
                    xs[buf][a0 + 2 * C:a0 + 4 * C, :] = pe - qo
                return f
            if isinstance(l, int) and l == 0:
                def wait_first(h):
                    def f():
                        with sc_('wait_slab'):
                            for cp in first_copies(h): cp.wait()
                    return f
                n = NBLK // NF
                return [g for h in range(NF)
                        for g in [wait_first(h)] + [f(j) for j in range(h * n, (h + 1) * n) for f in (xdft, kdft)]]
            return [wait] + [f(j) for j in range(NBLK) for f in ((kdft, xdft) if kfirst else (xdft, kdft))]

        def mac_pieces(l, buf, split=False):
            def mac(p, t):
                def f():
                    res = []
                    for hf in range(2):
                        tt = hf * NT + t
                        acc = [None, None]
                        xc = {}
                        for m in range(2 * p + 2):
                            kk = [xs[buf][pl.ds(z0 + addr(1, m, tt, c), 8), :] for c in range(nc)]
                            for i in range(2):
                                j = 2 * p + i - m
                                if j < 0: continue
                                if j not in xc:
                                    xc[j] = [xs[buf][pl.ds(z0 + addr(0, j, tt, c), 8), :] for c in range(nc)]
                                xx = xc[j]
                                term = [kk[0] * xx[0] - kk[1] * xx[1], kk[0] * xx[1] + kk[1] * xx[0]]
                                acc[i] = term if acc[i] is None else [a + b for a, b in zip(acc[i], term)]
                        zrow = tt * 16
                        def ovl(z, zp):
                            return [z[0] - zp[1], z[1] + zp[0]] if t < NT // 2 else [z[0] + zp[1], z[1] - zp[0]]
                        w1_ = ovl(acc[1], acc[0])
                        w0_ = acc[0]
                        if p > 0:
                            w0_ = ovl(acc[0], [zl[p - 1][pl.ds(z0 + zrow + 8 * c, 8), :] for c in range(2)])
                        if p + 1 < NBLK // 2:
                            for c in range(2):
                                zl[p][zrow + 8 * c:zrow + 8 * c + 8, :] = acc[1][c]
                        res.append([w0_, w1_])
                    for i in range(2):
                        (ar, ai), (br, bi) = res[0][i], res[1][i]
                        zb[2 * p + i][0, 8 * t:8 * t + 8, :] = pack(ar + br, ai + bi)
                        zb[2 * p + i][1, 8 * t:8 * t + 8, :] = pack(ar - br, ai - bi)
                return f

            def idft(j):
                def f():
                    ye = jnp.dot(iv(0), pltpu.bitcast(zb[j][0, pl.ds(z0, C), :] if zop else zb[j][0], bf16), preferred_element_type=f32)
                    yo = jnp.dot(iv(1), pltpu.bitcast(zb[j][1, pl.ds(z0, C), :] if zop else zb[j][1], bf16), preferred_element_type=f32)
                    yb[l, j * C:(j + 1) * C, :] = pack(ye, yo)
                return f

            if split:
                return ([(4 * p + 3 + c0, mac(p, t)) for p in range(NBLK // 2) for t in range(NT)],
                        [idft(j) for j in range(NBLK)])
            P = []
            for p in range(NBLK // 2):
                for t in range(NT):
                    P.append((4 * p + 3 + c0, mac(p, t)))
                    if p > 0 and t in ipos and not x_noinv:
                        P.append((0, idft(2 * p - 2 + (t == ipos[1]))))
            return P + ([(0, idft(NBLK - 2)), (0, idft(NBLK - 1))] if not x_noinv else [])

        def conv_step(l, buf, with_next):
            mp = mac_pieces(l, buf)
            dp = dft_pieces(l + 1, 1 - buf) if with_next else []
            total, done, k = sum(w for w, _ in mp), 0, 0
            for w, f in mp:
                while k < len(dp) and k * total * (dspan - dstart) <= (done - dstart * total) * len(dp):
                    dp[k](); k += 1
                f(); done += w
            for f in dp[k:]: f()

        with sc_('conv'):
            small[3].wait()
            for f in dft_pieces(0, 0): f()
            if not inv_late: small[4].wait()
            if inv_late: small[4].wait()
            def conv_body(i, carry):
                conv_step(2 * i, 0, True)
                conv_step(2 * i + 1, 1, True)
                return carry
            lax.fori_loop(0, NL // 2, conv_body, 0)

        cc = c_ref[...].astype(f32)
        sc = jnp.broadcast_to(cc * jax.nn.sigmoid(cc), (16, D)).astype(bf16)
        mod = lambda j: jnp.dot(sc, wload(wm, 0, D, j * D, (j + 1) * D), preferred_element_type=f32)[0:8]
        def finish_mod():
            ca, ga, sa, cb, sb_ = (mod(j) for j in (1, 2, 0, 4, 3))
            par[0] = ga * (1.0 + ca)
            par[1] = ga * sa
            par[2] = 1.0 + cb
            par[3] = sb_
        pb = lambda j, rows: jnp.broadcast_to(par[j, 0:1, :], (rows, D))

        def ln(x):
            mu = jnp.sum(x, axis=-1, keepdims=True) * (1.0 / D)
            xc = x - mu
            var = jnp.sum(xc * xc, axis=-1, keepdims=True) * (1.0 / D)
            return xc * lax.rsqrt(var + 1e-5)

        def pre_pieces(s):
            slot = s % 2 if isinstance(s, int) else lax.rem(s, 2)
            def piece(i):
                def f():
                    r = s * R + i * LR
                    if not isinstance(r, int): r = pl.multiple_of(r, LR)
                    x = qb[pl.ds(r, LR), :].astype(f32)
                    r2 = r // 2 if isinstance(r, int) else pl.multiple_of(s * (R // 2) + i * (LR // 2), LR // 2)
                    y = jnp.concatenate([pltpu.bitcast(yb[l, pl.ds(r2, LR // 2), :], bf16).astype(f32)
                                         for l in range(NL)], axis=1)
                    x1 = x + (ln(x) * pb(0, LR) + pb(1, LR)) * y
                    h2 = ln(x1) * pb(2, LR) + pb(3, LR)
                    x1b[slot, i * LR:(i + 1) * LR, :] = x1
                    h2b[slot, i * LR // 2:(i + 1) * LR // 2, :] = pltpu.bitcast(h2.astype(bf16), u32)
                return f
            return [piece(i) for i in range(R // LR)]

        def ffn_pieces(s, ups_first=False):
            slot = s % 2 if isinstance(s, int) else lax.rem(s, 2)
            r0 = s * R if isinstance(s, int) else pl.multiple_of(s * R, R)
            st = {}
            def gate(c):
                def f():
                    h = pltpu.bitcast(h2b[slot], bf16)
                    st['g', c] = jnp.dot(h, wload(w1, 0, D, c, c + PW), preferred_element_type=f32)
                return f
            def up(c):
                def f():
                    h = pltpu.bitcast(h2b[slot], bf16)
                    u = jnp.dot(h, wload(w3, 0, D, c, c + PW), preferred_element_type=f32)
                    hg = 0.5 * st['g', c]
                    st['a', c] = ((hg * jnp.tanh(hg) + hg) * u).astype(bf16)
                return f
            def down(t, c0_, c1_):
                def f():
                    a = jnp.concatenate([st['a', c] for c in range(t * TF, (t + 1) * TF, PW)], axis=1)
                    p = jnp.dot(a, wload(w2, t * TF, (t + 1) * TF, c0_, c1_), preferred_element_type=f32)
                    if t == 0:
                        st['acc'] = p
                    elif t + 1 < nt:
                        st['acc'] = st['acc'] + p
                    else:
                        gb = jnp.broadcast_to(par[4, 0:1, c0_:c1_], (R, c1_ - c0_))
                        y = st['acc'][:, c0_:c1_] + p
                        ob[pl.ds(r0, R), c0_:c1_] = (x1b[slot, :, c0_:c1_] + gb * y).astype(bf16)
                        if tailsplit and isinstance(s, int) and s == NS - 1:
                            last_copy(c0_, c1_).start()
                return f
            ups = [[(PW * D, f(c)) for c in range(t * TF, (t + 1) * TF, PW) for f in (gate, up)] for t in range(nt)]
            downs = [[(TF * D, down(t, 0, D))] for t in range(nt - 1)]
            downs.append([(TF * (c1 - c), down(nt - 1, c, c1)) for c, c1 in zip(DW[:-1], DW[1:])])
            if ups_first:
                G = ups + downs
            else:
                G = [ups[0]]
                for t in range(nt):
                    if t + 1 < nt: G.append(ups[t + 1] if not mixud else _merge(ups[t + 1], downs[t]))
                    if not mixud or t + 1 == nt: G.append(downs[t])
            def fin():
                out_copy(s).start()
            return G, fin

        def run_mixed(main, side):
            tm, ts = sum(w for w, _ in main), sum(w for w, _ in side)
            dm = ds = k = 0
            for w, f in main:
                f(); dm += w
                while k < len(side) and (ds + 0.5 * side[k][0]) * tm <= dm * ts:
                    side[k][1](); ds += side[k][0]; k += 1
            for _, f in side[k:]: f()

        mp, inv_ = mac_pieces(NL - 1, 0, True)
        n0 = NT * m0
        for _, f in mp[:n0]: f()
        for j in range(5): wait('wm', j)
        wait('q', 0)
        finish_mod()
        for _, f in mp[n0:NT * m1]: f()
        inv_[0](); inv_[1]()
        run_mixed(mp[NT * max(m0, m1):], [(1, f) for f in pre_pieces(0)])
        for f in inv_[2:]: f()
        if do_ffn:
            def body(s, carry):
                G, fin = ffn_pieces(s)
                main = [p for g in G for p in g]
                n = int(len(main) * pspan)
                run_mixed(main[:n], [(1, f) for f in pre_pieces(s + 1)])
                run_mixed(main[n:], [])
                fin()
                return carry
            G, fin = ffn_pieces(0)
            pp = [(1, f) for f in pre_pieces(1)]
            for t in range(2): wait('w1', t); wait('w3', t)
            run_mixed(G[0] + G[1], [])
            wait('w2', 0); wait('w1', 2); wait('w3', 2); wait('q', 1)
            run_mixed(G[2] + G[3], pp[:int(len(pp) * pfr)])
            wait('w2', 1); wait('wm', 5)
            par[4] = mod(5)
            run_mixed(G[4], pp[int(len(pp) * pfr):])
            wait('w2', 2)
            run_mixed(G[5], [])
            fin()
            wait('q', 2)
            with sc_('ffn_loop'):
                lax.fori_loop(1, NS - 1, body, 0, unroll=unroll)
            G, fin = ffn_pieces(NS - 1)
            run_mixed([p for g in G for p in g], [])
            if not tailsplit: fin()
            with sc_('wait_out'):
                for s in range(NS - 1 if tailsplit else NS):
                    out_copy(s).wait()
                if tailsplit:
                    for c, c1 in zip(DW[:-1], DW[1:]): last_copy(c, c1).wait()
        else:
            ob[0:R, :] = x1b[0].astype(bf16)
            w2_copy.wait(); q_copy.wait()
            out_copy(0).start(); out_copy(0).wait()

    def f(A_q, A_k, A_v, A_shift_k, A_ssm_k, A_ssm_D, B_x, B_w1, B_w3, B_w2, c, w_mod):
        hbm = pl.BlockSpec(memory_space=pl.ANY)
        vm = pl.BlockSpec(memory_space=pltpu.VMEM)
        out = pl.pallas_call(
            kern,
            in_specs=[hbm] * 13,
            out_specs=hbm,
            out_shape=jax.ShapeDtypeStruct((S, D), bf16),
            scratch_shapes=[
                pltpu.VMEM((4, D), bf16), pltpu.VMEM((D,), bf16), pltpu.VMEM((1, D), bf16),
                pltpu.VMEM(fwd_np.shape, u32), pltpu.VMEM(inv_np.shape, u32), pltpu.SemaphoreType.DMA((5,)),
                pltpu.VMEM((S, D), bf16), pltpu.VMEM((NL, S // 2 + 8, 128), u32), pltpu.VMEM((NL, S // 2, 128), u32),
                pltpu.VMEM((NL, 64, S), u32),
                pltpu.VMEM((D // 2, F), u32), pltpu.VMEM((D // 2, F), u32), pltpu.VMEM((F // 2, D), u32),
                pltpu.VMEM((D // 2, 6 * D), u32),
                [pltpu.VMEM((2 * KO + 512, 128), f32) for _ in range(2)],
                [pltpu.VMEM((4 * C, 128), f32) for _ in range(NBLK // 2 - 1)],
                [pltpu.VMEM((2, C + 8, 128), f32) for _ in range(NBLK)],
                [pltpu.VMEM((2, C, 128), u32) for _ in range(NBLK)],
                pltpu.VMEM((NL, S // 2, 128), u32),
                pltpu.VMEM((NL, 5, 8, 128), f32), pltpu.SMEM((1,), jnp.int32), pltpu.VMEM((5, 8, D), f32),
                pltpu.VMEM((2, R, D), f32), pltpu.VMEM((2, R // 2, D), u32),
                pltpu.VMEM((S, D), bf16),
                pltpu.SemaphoreType.DMA((3, NL)), pltpu.SemaphoreType.DMA((3, NF)), pltpu.SemaphoreType.DMA((9 + 3 * (F // TF),)), pltpu.SemaphoreType.DMA((NS + len(DW),)),
            ],
            compiler_params=pltpu.CompilerParams(vmem_limit_bytes=100 * 2**20, flags=flags, disable_bounds_checks=nochecks),
        )(A_q.reshape(S, D), A_k.reshape(S, D), A_v.reshape(S, D), A_shift_k.T, A_ssm_k, A_ssm_D,
          B_w1, B_w3, B_w2, c, w_mod, fwd_np, inv_np)
        return out.reshape(1, S, D)
    return f


@jax.jit
def pallas_adaLN_cond__ssm_conv_h3__glu_gated_swiglu__prompt_kernel(
    A_q: jax.Array,
    A_k: jax.Array,
    A_v: jax.Array,
    A_shift_k: jax.Array,
    A_ssm_k: jax.Array,
    A_ssm_D: jax.Array,
    B_x: jax.Array,
    B_w1: jax.Array,
    B_w3: jax.Array,
    B_w2: jax.Array,
    c: jax.Array,
    w_mod: jax.Array,
):
    return build()(A_q, A_k, A_v, A_shift_k, A_ssm_k, A_ssm_D, B_x, B_w1, B_w3, B_w2, c, w_mod)
```

```python
import contextlib

import jax
import jax.numpy as jnp
import numpy as np
from jax import lax
from jax.experimental import pallas as pl
from jax.experimental.pallas import tpu as pltpu

S, D, F = 2048, 640, 1536
KS = 4
EPS = 1e-5
C = 128
H = C // 2
NBLK = S // (2 * C)
NL = D // 128
NT = C // 8
R = 256
LR = 32
TF = 512
OUT_COLS = (0, 256, 512, D)
NS = S // R
NG = F // TF
BS = (4 * NT + 4) * 8
KO = (NBLK * BS + 511) // 512 * 512 + 16
DFT_SPAN = 0.9
PRE_SPAN = 0.9

f32, bf16, u32 = jnp.float32, jnp.bfloat16, jnp.uint32


def _scope(name):
    del name
    return contextlib.nullcontext()


def _dft_matrices():
    f = np.concatenate([np.arange(0, C, 2), np.arange(1, C, 2)])
    zeta = 2 * np.pi * (f + 0.5) / (4 * C)

    def fwd(n):
        ang = zeta[:, None] * n[None, :]
        m = np.stack([np.cos(ang), -np.sin(ang)], 0)
        return m.reshape(2, NT, 8, C).transpose(1, 0, 2, 3).reshape(2 * C, C)

    def inv(n):
        ang = n[:, None] * zeta[None, :]
        return np.stack([np.cos(ang), -np.sin(ang)], -1).reshape(C, 2 * C) / (2 * C)

    def words(m):
        b = m.astype(np.float32).astype(bf16).view(np.uint16).astype(np.uint32)
        return b[0::2] | (b[1::2] << 16)

    j = np.arange(C)
    even = (j // 2) * 2 + (j % 2) * C
    return (words(np.concatenate([fwd(even), fwd(even + 1)], 0)),
            words(np.concatenate([inv(2 * j), inv(2 * j + 1)], 0)))


def _spec_row(filt, block, tile=0, part=0):
    return filt * KO + block * BS + (2 * tile + part) * 8


def _unpack(w, i):
    return pltpu.unpack_elementwise(w, index=i, packed_dtype=bf16, unpacked_dtype=f32)


def _pack(a, b):
    return pltpu.bitcast(pltpu.pack_elementwise([a, b], packed_dtype=bf16), u32)


def _as_bf16(w):
    return pltpu.bitcast(w, bf16)


def _dot(a, b):
    return jnp.dot(a, b, preferred_element_type=f32)


def _layernorm(x):
    xc = x - jnp.sum(x, axis=-1, keepdims=True) * (1.0 / D)
    var = jnp.sum(xc * xc, axis=-1, keepdims=True) * (1.0 / D)
    return xc * lax.rsqrt(var + EPS)


def _run_mixed(main, side):
    total, done, k = sum(w for w, _ in main), 0, 0
    for w, f in main:
        f()
        done += w
        while k < len(side) and (k + 0.5) * total <= done * len(side):
            side[k]()
            k += 1
    for f in side[k:]:
        f()


def _kernel(q_hbm, k_hbm, v_hbm, shk_hbm, ssm_hbm, d_hbm, w1_hbm, w3_hbm, w2_hbm, c_hbm, wm_hbm,
            fwd_hbm, inv_hbm, o_hbm,
            shk, dvec, cvec, fwd, inv, qb, kb, vb, sb, w1, w3, w2, wm,
            spec, zlast, kf, zb, yb, cpar, zero, par, x1b, h2b, ob, sems):
    k32, v32, s32, wm32, w132, w332, w232 = (
        a.bitcast(u32) for a in (k_hbm, v_hbm, ssm_hbm, wm_hbm, w1_hbm, w3_hbm, w2_hbm))

    def conv_inputs(l, t0, n):
        cols = pl.ds(l * 128, 128)
        return [(s32.at[pl.ds(l * H, H), pl.ds(t0, n)], sb.at[l, :, pl.ds(t0, n)]),
                (k32.at[pl.ds(t0 // 2, n // 2), cols], kb.at[l, pl.ds(8 + t0 // 2, n // 2)]),
                (v32.at[pl.ds(t0 // 2, n // 2), cols], vb.at[l, pl.ds(t0 // 2, n // 2)])]

    def same(src, dst, *idx):
        return src.at[idx], dst.at[idx]

    mod_cols = lambda j: same(wm32, wm, slice(None), pl.ds(j * D, D))
    up_cols = lambda g: [same(w132, w1, slice(None), pl.ds(g * TF, TF)),
                         same(w332, w3, slice(None), pl.ds(g * TF, TF))]
    down_rows = lambda g: same(w232, w2, pl.ds(g * TF // 2, TF // 2))
    q_rows = lambda r0, n: same(q_hbm, qb, pl.ds(r0, n))
    groups = {
        'params': [(shk_hbm, shk), (d_hbm, dvec), (c_hbm, cvec)],
        'first': [(fwd_hbm, fwd)] + conv_inputs(0, 0, S // 2),
        0: conv_inputs(0, S // 2, S // 2),
        1: conv_inputs(1, 0, S),
        'inv': [(inv_hbm, inv)],
        **{l: conv_inputs(l, 0, S) for l in range(2, NL)},
        'mod': [mod_cols(j) for j in range(5)] + [q_rows(0, R)],
        'up01': up_cols(0) + up_cols(1),
        'up2': [q_rows(R, R), down_rows(0)] + up_cols(2),
        'down1': [mod_cols(5), down_rows(1)],
        'down2': [down_rows(2)],
        'q': [q_rows(2 * R, S - 2 * R)],
    }
    named = [g for g in groups if isinstance(g, str)]
    sem_of = lambda g: sems.at[NL + named.index(g) if isinstance(g, str) else g]
    out_sem = sems.at[NL + len(named)]

    def wait(g, pairs=None):
        with _scope('wait_' + (g if isinstance(g, str) else 'slab')):
            for src, dst in (groups[g] if pairs is None else pairs):
                pltpu.make_async_copy(src, dst, sem_of(g)).wait()

    def out_copy(r0, cols=slice(None)):
        return pltpu.make_async_copy(*same(ob, o_hbm, pl.ds(r0, R), cols), out_sem)

    for g, pairs in groups.items():
        for src, dst in pairs:
            pltpu.make_async_copy(src, dst, sem_of(g)).start()

    wait('params')
    taps = shk[...].astype(f32)
    skip = dvec[...].astype(f32).reshape(1, D)
    for l in range(NL):
        kb[l, 0:8, :] = jnp.zeros((8, 128), u32)
        for j in range(KS):
            cpar[l, j] = jnp.broadcast_to(taps[j:j + 1, l * 128:(l + 1) * 128], (8, 128))
        cpar[l, KS] = jnp.broadcast_to(skip[:, l * 128:(l + 1) * 128], (8, 128))
    zero[0] = 0
    z0 = pl.multiple_of(zero[0] * 1024, 1024)

    def forward_pieces(l, buf):
        param = lambda j, rows: jnp.broadcast_to(cpar[l, j, 0:1, :], (rows, 128))
        mat = lambda i: _as_bf16(fwd[i * C:(i + 1) * C, :])

        def butterfly(filt, j, even, odd):
            r = _spec_row(filt, j)
            spec[buf][r:r + 2 * C, :] = even + odd
            spec[buf][r + 2 * C:r + 4 * C, :] = even - odd

        def signal(j):
            def f():
                kw = kb[l, j * C:j * C + C + 8, :]
                ke, ko = _unpack(kw, 0), _unpack(kw, 1)
                kf[j][0] = ke
                kf[j][1] = ko
                ke1, ko1, ko2 = kf[j][0, 7:7 + C, :], kf[j][1, 7:7 + C, :], kf[j][1, 6:6 + C, :]
                ke, ko = ke[8:], ko[8:]
                t0, t1, t2, t3 = (param(t, C) for t in range(KS))
                vw = vb[l, j * C:(j + 1) * C, :]
                xe = (t0 * ke + t1 * ko1 + t2 * ke1 + t3 * ko2) * _unpack(vw, 0)
                xo = (t0 * ko + t1 * ke + t2 * ko1 + t3 * ke1) * _unpack(vw, 1)
                butterfly(0, j, _dot(mat(0), _as_bf16(_pack(xe[:H], xe[H:]))),
                          _dot(mat(1), _as_bf16(_pack(xo[:H], xo[H:]))))
            return f

        def long_filter(j):
            def f():
                lo = sb[l, :, 2 * j * C:(2 * j + 1) * C]
                hi = sb[l, :, (2 * j + 1) * C:(2 * j + 2) * C]
                even_lane = lax.broadcasted_iota(jnp.int32, lo.shape, 1) % 2 == 0
                te = jnp.where(even_lane, lo, pltpu.roll(hi, 1, 1))
                to = jnp.where(even_lane, pltpu.roll(lo, C - 1, 1), hi)
                dims = (((1,), (1,)), ((), ()))
                pe = lax.dot_general(mat(0), _as_bf16(te), dims, preferred_element_type=f32)
                po = lax.dot_general(mat(1), _as_bf16(to), dims, preferred_element_type=f32)
                if j == 0:
                    real = lax.broadcasted_iota(jnp.int32, pe.shape, 0) % 16 < 8
                    pe = pe + jnp.where(real, param(KS, 2 * C), 0.0)
                butterfly(1, j, pe, po)
            return f
        return [piece(j) for j in range(NBLK) for piece in (signal, long_filter)]

    def product_pieces(buf):
        load = lambda filt, j, tile: [
            spec[buf][pl.ds(z0 + _spec_row(filt, j, tile, c), 8), :] for c in range(2)]

        def piece(p, t):
            def plus_tail(z, prev):
                if t < NT // 2:
                    return [z[0] - prev[1], z[1] + prev[0]]
                return [z[0] + prev[1], z[1] - prev[0]]

            def f():
                res = []
                for tile in (t, NT + t):
                    acc, xs = [None, None], {}
                    for m in range(2 * p + 2):
                        kr, ki = load(1, m, tile)
                        for i in range(2):
                            j = 2 * p + i - m
                            if j < 0:
                                continue
                            if j not in xs:
                                xs[j] = load(0, j, tile)
                            xr, xi = xs[j]
                            term = [kr * xr - ki * xi, kr * xi + ki * xr]
                            acc[i] = term if acc[i] is None else [a + b for a, b in zip(acc[i], term)]
                    row = tile * 16
                    first = acc[0]
                    if p > 0:
                        first = plus_tail(first, [zlast[p - 1][pl.ds(z0 + row + 8 * c, 8), :] for c in range(2)])
                    if 2 * p + 2 < NBLK:
                        for c in range(2):
                            zlast[p][row + 8 * c:row + 8 * c + 8, :] = acc[1][c]
                    res.append([first, plus_tail(acc[1], acc[0])])
                for i in range(2):
                    (ar, ai), (br, bi) = res[0][i], res[1][i]
                    zb[2 * p + i][0, 8 * t:8 * t + 8, :] = _pack(ar + br, ai + bi)
                    zb[2 * p + i][1, 8 * t:8 * t + 8, :] = _pack(ar - br, ai - bi)
            return f
        return [(4 * p + 5, piece(p, t)) for p in range(NBLK // 2) for t in range(NT)]

    def inverse(l, j):
        ye, yo = (_dot(_as_bf16(inv[i * H:(i + 1) * H, :]), _as_bf16(zb[j][i, pl.ds(z0, C), :]))
                  for i in range(2))
        yb[l, j * C:(j + 1) * C, :] = _pack(ye, yo)

    def conv_step(l, buf):
        wait(l + 1, conv_inputs(l + 1, 0, S))
        ahead = forward_pieces(l + 1, 1 - buf)
        products = product_pieces(buf)
        total, done, k = sum(w for w, _ in products), 0, 0
        for i, (w, f) in enumerate(products):
            while k < len(ahead) and (k + 1) * total * DFT_SPAN <= done * (len(ahead) + 1):
                ahead[k]()
                k += 1
            f()
            done += w
            p, t = divmod(i, NT)
            if p > 0 and t in (NT // 4, 3 * NT // 4):
                inverse(l, 2 * p - 2 + (t > NT // 2))
        for f in ahead[k:]:
            f()
        inverse(l, NBLK - 2)
        inverse(l, NBLK - 1)

    ahead = forward_pieces(0, 0)
    wait('first')
    for f in ahead[:NBLK]:
        f()
    wait(0)
    for f in ahead[NBLK:]:
        f()
    wait('inv')

    def conv_body(i, carry):
        conv_step(2 * i, 0)
        conv_step(2 * i + 1, 1)
        return carry
    lax.fori_loop(0, NL // 2, conv_body, 0)

    cond = cvec[...].astype(f32)
    cond = jnp.broadcast_to(cond * jax.nn.sigmoid(cond), (16, D)).astype(bf16)
    mod = lambda j: _dot(cond, _as_bf16(wm[:, j * D:(j + 1) * D]))[0:8]
    row = lambda j, rows, cols=slice(None): par[j, 0:1, cols]

    def norm_pieces(s):
        static = isinstance(s, int)
        slot = s % 2 if static else lax.rem(s, 2)

        def piece(i):
            def f():
                r, r2 = s * R + i * LR, s * (R // 2) + i * (LR // 2)
                if not static:
                    r, r2 = pl.multiple_of(r, LR), pl.multiple_of(r2, LR // 2)
                x = qb[pl.ds(r, LR), :].astype(f32)
                y = jnp.concatenate(
                    [_as_bf16(yb[l, pl.ds(r2, LR // 2), :]).astype(f32) for l in range(NL)], axis=1)
                x = x + (_layernorm(x) * row(0, LR) + row(1, LR)) * y
                h = _layernorm(x) * row(2, LR) + row(3, LR)
                x1b[slot, i * LR:(i + 1) * LR, :] = x
                h2b[slot, i * LR // 2:(i + 1) * LR // 2, :] = pltpu.bitcast(h.astype(bf16), u32)
            return f
        return [piece(i) for i in range(R // LR)]

    def ffn_groups(s):
        static = isinstance(s, int)
        slot = s % 2 if static else lax.rem(s, 2)
        r0 = s * R if static else pl.multiple_of(s * R, R)
        st = {}

        def gate(g):
            def f():
                st['gate'] = _dot(_as_bf16(h2b[slot]), _as_bf16(w1[:, g * TF:(g + 1) * TF]))
            return f

        def up(g):
            def f():
                u = _dot(_as_bf16(h2b[slot]), _as_bf16(w3[:, g * TF:(g + 1) * TF]))
                half = 0.5 * st['gate']
                st[g] = ((half * jnp.tanh(half) + half) * u).astype(bf16)
            return f

        def down(g, c0, c1):
            def f():
                p = _dot(st[g], _as_bf16(w2[g * TF // 2:(g + 1) * TF // 2, c0:c1]))
                if g + 1 < NG:
                    st['acc'] = p if g == 0 else st['acc'] + p
                    return
                y = st['acc'][:, c0:c1] + p
                ob[pl.ds(r0, R), c0:c1] = (x1b[slot, :, c0:c1] + row(4, R, slice(c0, c1)) * y).astype(bf16)
                if static and s == NS - 1:
                    out_copy(r0, pl.ds(c0, c1 - c0)).start()
            return f
        ups = [[(D, gate(g)), (D, up(g))] for g in range(NG)]
        downs = [[(D, down(g, 0, D))] for g in range(NG - 1)]
        downs.append([(c1 - c0, down(NG - 1, c0, c1)) for c0, c1 in zip(OUT_COLS[:-1], OUT_COLS[1:])])
        return [ups[0], ups[1], downs[0], ups[2], downs[1], downs[2]]

    products = product_pieces(0)
    for _, f in products[:NT]:
        f()
    wait('mod')
    scale_a, gate_a, shift_a, scale_b, shift_b = (mod(j) for j in (1, 2, 0, 4, 3))
    par[0] = gate_a * (1.0 + scale_a)
    par[1] = gate_a * shift_a
    par[2] = 1.0 + scale_b
    par[3] = shift_b
    for _, f in products[NT:2 * NT]:
        f()
    inverse(NL - 1, 0)
    inverse(NL - 1, 1)
    _run_mixed(products[2 * NT:], norm_pieces(0))
    for j in range(2, NBLK):
        inverse(NL - 1, j)

    ffn, norms = ffn_groups(0), norm_pieces(1)
    wait('up01')
    _run_mixed(ffn[0] + ffn[1], [])
    wait('up2')
    _run_mixed(ffn[2] + ffn[3], norms[:len(norms) // 2])
    wait('down1')
    par[4] = mod(5)
    _run_mixed(ffn[4], norms[len(norms) // 2:])
    wait('down2')
    _run_mixed(ffn[5], [])
    out_copy(0).start()
    wait('q')

    def ffn_body(s, carry):
        pieces = [p for g in ffn_groups(s) for p in g]
        n = int(len(pieces) * PRE_SPAN)
        _run_mixed(pieces[:n], norm_pieces(s + 1))
        _run_mixed(pieces[n:], [])
        out_copy(pl.multiple_of(s * R, R)).start()
        return carry
    with _scope('ffn_loop'):
        lax.fori_loop(1, NS - 1, ffn_body, 0)
    _run_mixed([p for g in ffn_groups(NS - 1) for p in g], [])

    with _scope('wait_out'):
        for s in range(NS - 1):
            out_copy(s * R).wait()
        for c0, c1 in zip(OUT_COLS[:-1], OUT_COLS[1:]):
            out_copy(S - R, pl.ds(c0, c1 - c0)).wait()


@jax.jit
def pallas_adaLN_cond__ssm_conv_h3__glu_gated_swiglu__prompt_kernel(
    A_q: jax.Array,
    A_k: jax.Array,
    A_v: jax.Array,
    A_shift_k: jax.Array,
    A_ssm_k: jax.Array,
    A_ssm_D: jax.Array,
    B_x: jax.Array,
    B_w1: jax.Array,
    B_w3: jax.Array,
    B_w2: jax.Array,
    c: jax.Array,
    w_mod: jax.Array,
):
    del B_x
    fwd, inv = _dft_matrices()
    hbm = pl.BlockSpec(memory_space=pl.ANY)
    vmem = pltpu.VMEM
    out = pl.pallas_call(
        _kernel,
        in_specs=[hbm] * 13,
        out_specs=hbm,
        out_shape=jax.ShapeDtypeStruct((S, D), bf16),
        scratch_shapes=[
            vmem((KS, D), bf16), vmem((D,), bf16), vmem((1, D), bf16),
            vmem(fwd.shape, u32), vmem(inv.shape, u32),
            vmem((S, D), bf16),
            vmem((NL, S // 2 + 8, 128), u32), vmem((NL, S // 2, 128), u32),
            vmem((NL, H, S), u32),
            vmem((D // 2, F), u32), vmem((D // 2, F), u32), vmem((F // 2, D), u32),
            vmem((D // 2, 6 * D), u32),
            [vmem((2 * KO + 512, 128), f32) for _ in range(2)],
            [vmem((4 * C, 128), f32) for _ in range(NBLK // 2 - 1)],
            [vmem((2, C + 8, 128), f32) for _ in range(NBLK)],
            [vmem((2, C, 128), u32) for _ in range(NBLK)],
            vmem((NL, S // 2, 128), u32),
            vmem((NL, KS + 1, 8, 128), f32), pltpu.SMEM((1,), jnp.int32), vmem((5, 8, D), f32),
            vmem((2, R, D), f32), vmem((2, R // 2, D), u32),
            vmem((S, D), bf16),
            pltpu.SemaphoreType.DMA((NL + 10,)),
        ],
        compiler_params=pltpu.CompilerParams(vmem_limit_bytes=100 * 2**20),
    )(A_q.reshape(S, D), A_k.reshape(S, D), A_v.reshape(S, D), A_shift_k.T, A_ssm_k, A_ssm_D,
      B_w1, B_w3, B_w2, c, w_mod, fwd, inv)
    return out.reshape(1, S, D)
```

```python
import contextlib
import functools

import jax
import jax.numpy as jnp
import numpy as np
from jax import lax
from jax.experimental import pallas as pl
from jax.experimental.pallas import tpu as pltpu

S, D, F = 2048, 640, 1536
KS = 4
EPS = 1e-5
C = 128
H = C // 2
NBLK = S // (2 * C)
NL = D // 128
NT = C // 8
R = 256
LR = 32
TF = 512
OUT_COLS = (0, 256, 512, D)
NS = S // R
NG = F // TF
BS = (4 * NT + 4) * 8
KO = (NBLK * BS + 511) // 512 * 512 + 16
DFT_SPAN = 0.9
PFR = 0.75
PEEL = 3
M0 = 5
EARLY_INV = False
PRE_SPAN = 0.9

f32, bf16, u32 = jnp.float32, jnp.bfloat16, jnp.uint32


def _scope(name):
    del name
    return contextlib.nullcontext()


def _dft_matrices():
    f = np.concatenate([np.arange(0, C, 2), np.arange(1, C, 2)])
    zeta = 2 * np.pi * (f + 0.5) / (4 * C)

    def fwd(n):
        ang = zeta[:, None] * n[None, :]
        m = np.stack([np.cos(ang), -np.sin(ang)], 0)
        return m.reshape(2, NT, 8, C).transpose(1, 0, 2, 3).reshape(2 * C, C)

    def inv(n):
        ang = n[:, None] * zeta[None, :]
        return np.stack([np.cos(ang), -np.sin(ang)], -1).reshape(C, 2 * C) / (2 * C)

    def words(m):
        b = m.astype(np.float32).astype(bf16).view(np.uint16).astype(np.uint32)
        return b[0::2] | (b[1::2] << 16)

    j = np.arange(C)
    even = (j // 2) * 2 + (j % 2) * C
    return (words(np.concatenate([fwd(even), fwd(even + 1)], 0)),
            words(np.concatenate([inv(2 * j), inv(2 * j + 1)], 0)))


def _spec_row(filt, block, tile=0, part=0):
    return filt * KO + block * BS + (2 * tile + part) * 8


def _unpack(w, i):
    return pltpu.unpack_elementwise(w, index=i, packed_dtype=bf16, unpacked_dtype=f32)


def _pack(a, b):
    return pltpu.bitcast(pltpu.pack_elementwise([a, b], packed_dtype=bf16), u32)


def _as_bf16(w):
    return pltpu.bitcast(w, bf16)


def _dot(a, b):
    return jnp.dot(a, b, preferred_element_type=f32)


def _layernorm(x):
    xc = x - jnp.sum(x, axis=-1, keepdims=True) * (1.0 / D)
    var = jnp.sum(xc * xc, axis=-1, keepdims=True) * (1.0 / D)
    return xc * lax.rsqrt(var + EPS)


def _run_mixed(main, side):
    total, done, k = sum(w for w, _ in main), 0, 0
    for w, f in main:
        f()
        done += w
        while k < len(side) and (k + 0.5) * total <= done * len(side):
            side[k]()
            k += 1
    for f in side[k:]:
        f()


def _kernel(q_hbm, k_hbm, v_hbm, shk_hbm, ssm_hbm, d_hbm, w1_hbm, w3_hbm, w2_hbm, c_hbm, wm_hbm,
            fwd_hbm, inv_hbm, o_hbm,
            shk, dvec, cvec, fwd, inv, qb, kb, vb, sb, w1, w3, w2, wm,
            spec, zlast, kf, zb, yb, cpar, zero, par, x1b, h2b, ob, sems):
    k32, v32, s32, wm32, w132, w332, w232 = (
        a.bitcast(u32) for a in (k_hbm, v_hbm, ssm_hbm, wm_hbm, w1_hbm, w3_hbm, w2_hbm))

    def conv_inputs(l, t0, n):
        cols = pl.ds(l * 128, 128)
        return [(s32.at[pl.ds(l * H, H), pl.ds(t0, n)], sb.at[l, :, pl.ds(t0, n)]),
                (k32.at[pl.ds(t0 // 2, n // 2), cols], kb.at[l, pl.ds(8 + t0 // 2, n // 2)]),
                (v32.at[pl.ds(t0 // 2, n // 2), cols], vb.at[l, pl.ds(t0 // 2, n // 2)])]

    def same(src, dst, *idx):
        return src.at[idx], dst.at[idx]

    mod_cols = lambda j: same(wm32, wm, slice(None), pl.ds(j * D, D))
    up_cols = lambda g: [same(w132, w1, slice(None), pl.ds(g * TF, TF)),
                         same(w332, w3, slice(None), pl.ds(g * TF, TF))]
    down_rows = lambda g: same(w232, w2, pl.ds(g * TF // 2, TF // 2))
    q_rows = lambda r0, n: same(q_hbm, qb, pl.ds(r0, n))
    groups = {
        'params': [(shk_hbm, shk), (d_hbm, dvec), (c_hbm, cvec)],
        'first': [(fwd_hbm, fwd)] + conv_inputs(0, 0, S // 2),
        0: conv_inputs(0, S // 2, S // 2),
        1: conv_inputs(1, 0, S),
        'inv': [(inv_hbm, inv)],
        **{l: conv_inputs(l, 0, S) for l in range(2, NL)},
        'mod': [mod_cols(j) for j in range(5)] + [q_rows(0, R)],
        'ffn0': up_cols(0) + up_cols(1)[:1],
        'ffn1': up_cols(1)[1:] + [down_rows(0)] + up_cols(2)[:1],
        'ffn2': [q_rows(R, R)] + up_cols(2)[1:] + [down_rows(1)],
        'ffn3': [mod_cols(5), down_rows(2)],
        'q': [q_rows(2 * R, 2 * R)],
        'q_late': [q_rows(4 * R, S - 4 * R)],
    }
    named = [g for g in groups if isinstance(g, str)]
    sem_of = lambda g: sems.at[NL + named.index(g) if isinstance(g, str) else g]
    out_sem = sems.at[NL + len(named)]

    def wait(g, pairs=None):
        with _scope('wait_' + (g if isinstance(g, str) else 'slab')):
            for src, dst in (groups[g] if pairs is None else pairs):
                pltpu.make_async_copy(src, dst, sem_of(g)).wait()

    def out_copy(r0, cols=slice(None)):
        return pltpu.make_async_copy(*same(ob, o_hbm, pl.ds(r0, R), cols), out_sem)

    for g, pairs in groups.items():
        for src, dst in pairs:
            pltpu.make_async_copy(src, dst, sem_of(g)).start()

    wait('params')
    taps = shk[...].astype(f32)
    skip = dvec[...].astype(f32).reshape(1, D)
    for l in range(NL):
        kb[l, 0:8, :] = jnp.zeros((8, 128), u32)
        for j in range(KS):
            cpar[l, j] = jnp.broadcast_to(taps[j:j + 1, l * 128:(l + 1) * 128], (8, 128))
        cpar[l, KS] = jnp.broadcast_to(skip[:, l * 128:(l + 1) * 128], (8, 128))
    zero[0] = 0
    z0 = pl.multiple_of(zero[0] * 1024, 1024)

    def forward_pieces(l, buf):
        param = lambda j, rows: jnp.broadcast_to(cpar[l, j, 0:1, :], (rows, 128))
        mat = lambda i: _as_bf16(fwd[i * C:(i + 1) * C, :])

        def butterfly(filt, j, even, odd):
            r = _spec_row(filt, j)
            spec[buf][r:r + 2 * C, :] = even + odd
            spec[buf][r + 2 * C:r + 4 * C, :] = even - odd

        def signal(j):
            def f():
                kw = kb[l, j * C:j * C + C + 8, :]
                ke, ko = _unpack(kw, 0), _unpack(kw, 1)
                kf[j][0] = ke
                kf[j][1] = ko
                ke1, ko1, ko2 = kf[j][0, 7:7 + C, :], kf[j][1, 7:7 + C, :], kf[j][1, 6:6 + C, :]
                ke, ko = ke[8:], ko[8:]
                t0, t1, t2, t3 = (param(t, C) for t in range(KS))
                vw = vb[l, j * C:(j + 1) * C, :]
                xe = (t0 * ke + t1 * ko1 + t2 * ke1 + t3 * ko2) * _unpack(vw, 0)
                xo = (t0 * ko + t1 * ke + t2 * ko1 + t3 * ke1) * _unpack(vw, 1)
                butterfly(0, j, _dot(mat(0), _as_bf16(_pack(xe[:H], xe[H:]))),
                          _dot(mat(1), _as_bf16(_pack(xo[:H], xo[H:]))))
            return f

        def long_filter(j):
            def f():
                lo = sb[l, :, 2 * j * C:(2 * j + 1) * C]
                hi = sb[l, :, (2 * j + 1) * C:(2 * j + 2) * C]
                even_lane = lax.broadcasted_iota(jnp.int32, lo.shape, 1) % 2 == 0
                te = jnp.where(even_lane, lo, pltpu.roll(hi, 1, 1))
                to = jnp.where(even_lane, pltpu.roll(lo, C - 1, 1), hi)
                dims = (((1,), (1,)), ((), ()))
                pe = lax.dot_general(mat(0), _as_bf16(te), dims, preferred_element_type=f32)
                po = lax.dot_general(mat(1), _as_bf16(to), dims, preferred_element_type=f32)
                if j == 0:
                    real = lax.broadcasted_iota(jnp.int32, pe.shape, 0) % 16 < 8
                    pe = pe + jnp.where(real, param(KS, 2 * C), 0.0)
                butterfly(1, j, pe, po)
            return f
        return [piece(j) for j in range(NBLK) for piece in (signal, long_filter)]

    def product_pieces(buf):
        load = lambda filt, j, tile: [
            spec[buf][pl.ds(z0 + _spec_row(filt, j, tile, c), 8), :] for c in range(2)]

        def piece(p, t):
            def plus_tail(z, prev):
                if t < NT // 2:
                    return [z[0] - prev[1], z[1] + prev[0]]
                return [z[0] + prev[1], z[1] - prev[0]]

            def f():
                res = []
                for tile in (t, NT + t):
                    acc, xs = [None, None], {}
                    for m in range(2 * p + 2):
                        kr, ki = load(1, m, tile)
                        for i in range(2):
                            j = 2 * p + i - m
                            if j < 0:
                                continue
                            if j not in xs:
                                xs[j] = load(0, j, tile)
                            xr, xi = xs[j]
                            term = [kr * xr - ki * xi, kr * xi + ki * xr]
                            acc[i] = term if acc[i] is None else [a + b for a, b in zip(acc[i], term)]
                    row = tile * 16
                    first = acc[0]
                    if p > 0:
                        first = plus_tail(first, [zlast[p - 1][pl.ds(z0 + row + 8 * c, 8), :] for c in range(2)])
                    if 2 * p + 2 < NBLK:
                        for c in range(2):
                            zlast[p][row + 8 * c:row + 8 * c + 8, :] = acc[1][c]
                    res.append([first, plus_tail(acc[1], acc[0])])
                for i in range(2):
                    (ar, ai), (br, bi) = res[0][i], res[1][i]
                    zb[2 * p + i][0, 8 * t:8 * t + 8, :] = _pack(ar + br, ai + bi)
                    zb[2 * p + i][1, 8 * t:8 * t + 8, :] = _pack(ar - br, ai - bi)
            return f
        return [(4 * p + 5, piece(p, t)) for p in range(NBLK // 2) for t in range(NT)]

    def inverse(l, j):
        ye, yo = (_dot(_as_bf16(inv[i * H:(i + 1) * H, :]), _as_bf16(zb[j][i, pl.ds(z0, C), :]))
                  for i in range(2))
        yb[l, j * C:(j + 1) * C, :] = _pack(ye, yo)

    def conv_step(l, buf, early=0):
        products = product_pieces(buf)
        for _, f in products[:early]:
            f()
        if early:
            wait('inv')
        wait(l + 1, conv_inputs(l + 1, 0, S))
        for j in range(2 * (early // NT) - 2):
            inverse(l, j)
        ahead = forward_pieces(l + 1, 1 - buf)
        total, done, k = sum(w for w, _ in products[early:]), 0, 0
        for i, (w, f) in list(enumerate(products))[early:]:
            while k < len(ahead) and (k + 1) * total * DFT_SPAN <= done * (len(ahead) + 1):
                ahead[k]()
                k += 1
            f()
            done += w
            p, t = divmod(i, NT)
            if p > 0 and t in (NT // 4, 3 * NT // 4):
                inverse(l, 2 * p - 2 + (t > NT // 2))
        for f in ahead[k:]:
            f()
        inverse(l, NBLK - 2)
        inverse(l, NBLK - 1)

    ahead = forward_pieces(0, 0)
    wait('first')
    for f in ahead[:NBLK]:
        f()
    wait(0)
    for f in ahead[NBLK:]:
        f()
    if PEEL:
        conv_step(0, 0, PEEL * NT)
        for l in range(1, NL - 1):
            conv_step(l, l % 2)
    else:
        wait('inv')

        def conv_body(i, carry):
            conv_step(2 * i, 0)
            conv_step(2 * i + 1, 1)
            return carry
        lax.fori_loop(0, NL // 2, conv_body, 0)

    cond = cvec[...].astype(f32)
    cond = jnp.broadcast_to(cond * jax.nn.sigmoid(cond), (16, D)).astype(bf16)
    mod = lambda j: _dot(cond, _as_bf16(wm[:, j * D:(j + 1) * D]))[0:8]
    row = lambda j, rows, cols=slice(None): par[j, 0:1, cols]

    def norm_pieces(s):
        static = isinstance(s, int)
        slot = s % 2 if static else lax.rem(s, 2)

        def piece(i):
            def f():
                r, r2 = s * R + i * LR, s * (R // 2) + i * (LR // 2)
                if not static:
                    r, r2 = pl.multiple_of(r, LR), pl.multiple_of(r2, LR // 2)
                x = qb[pl.ds(r, LR), :].astype(f32)
                y = jnp.concatenate(
                    [_as_bf16(yb[l, pl.ds(r2, LR // 2), :]).astype(f32) for l in range(NL)], axis=1)
                x = x + (_layernorm(x) * row(0, LR) + row(1, LR)) * y
                h = _layernorm(x) * row(2, LR) + row(3, LR)
                x1b[slot, i * LR:(i + 1) * LR, :] = x
                h2b[slot, i * LR // 2:(i + 1) * LR // 2, :] = pltpu.bitcast(h.astype(bf16), u32)
            return f
        return [piece(i) for i in range(R // LR)]

    def ffn_groups(s):
        static = isinstance(s, int)
        slot = s % 2 if static else lax.rem(s, 2)
        r0 = s * R if static else pl.multiple_of(s * R, R)
        st = {}

        def gate(g):
            def f():
                st['gate'] = _dot(_as_bf16(h2b[slot]), _as_bf16(w1[:, g * TF:(g + 1) * TF]))
            return f

        def up(g):
            def f():
                u = _dot(_as_bf16(h2b[slot]), _as_bf16(w3[:, g * TF:(g + 1) * TF]))
                half = 0.5 * st['gate']
                st[g] = ((half * jnp.tanh(half) + half) * u).astype(bf16)
            return f

        def down(g, c0, c1):
            def f():
                p = _dot(st[g], _as_bf16(w2[g * TF // 2:(g + 1) * TF // 2, c0:c1]))
                if g + 1 < NG:
                    st['acc'] = p if g == 0 else st['acc'] + p
                    return
                y = st['acc'][:, c0:c1] + p
                ob[pl.ds(r0, R), c0:c1] = (x1b[slot, :, c0:c1] + row(4, R, slice(c0, c1)) * y).astype(bf16)
                if static and s == NS - 1:
                    out_copy(r0, pl.ds(c0, c1 - c0)).start()
            return f
        ups = [[(D, gate(g)), (D, up(g))] for g in range(NG)]
        downs = [[(D, down(g, 0, D))] for g in range(NG - 1)]
        downs.append([(c1 - c0, down(NG - 1, c0, c1)) for c0, c1 in zip(OUT_COLS[:-1], OUT_COLS[1:])])
        return [ups[0], ups[1], downs[0], ups[2], downs[1], downs[2]]

    products = product_pieces(0)
    for _, f in products[:M0 * NT // 2]:
        f()
    wait('mod')
    scale_a, gate_a, shift_a, scale_b, shift_b = (mod(j) for j in (1, 2, 0, 4, 3))
    par[0] = gate_a * (1.0 + scale_a)
    par[1] = gate_a * shift_a
    par[2] = 1.0 + scale_b
    par[3] = shift_b
    if EARLY_INV:
        inverse(NL - 1, 0)
        inverse(NL - 1, 1)
    for _, f in products[M0 * NT // 2:]:
        f()
    if not EARLY_INV:
        inverse(NL - 1, 0)
        inverse(NL - 1, 1)
    _run_mixed([(1, f) for f in norm_pieces(0)],
               [functools.partial(inverse, NL - 1, j) for j in range(2, NBLK)])

    ffn, norms = [p for g in ffn_groups(0) for p in g], norm_pieces(1)
    n = int(len(norms) * PFR)
    wait('ffn0')
    _run_mixed(ffn[:3], [])
    wait('ffn1')
    _run_mixed(ffn[3:6], [])
    wait('ffn2')
    _run_mixed(ffn[6:8], norms[:n])
    wait('ffn3')
    par[4] = mod(5)
    _run_mixed(ffn[8:], norms[n:])
    out_copy(0).start()
    wait('q')

    def ffn_body(s, carry):
        pl.when(s == 3)(lambda: wait('q_late'))
        pieces = [p for g in ffn_groups(s) for p in g]
        n = int(len(pieces) * PRE_SPAN)
        _run_mixed(pieces[:n], norm_pieces(s + 1))
        _run_mixed(pieces[n:], [])
        out_copy(pl.multiple_of(s * R, R)).start()
        return carry
    with _scope('ffn_loop'):
        lax.fori_loop(1, NS - 1, ffn_body, 0)
    _run_mixed([p for g in ffn_groups(NS - 1) for p in g], [])

    with _scope('wait_out'):
        for s in range(NS - 1):
            out_copy(s * R).wait()
        for c0, c1 in zip(OUT_COLS[:-1], OUT_COLS[1:]):
            out_copy(S - R, pl.ds(c0, c1 - c0)).wait()


@jax.jit
def pallas_adaLN_cond__ssm_conv_h3__glu_gated_swiglu__prompt_kernel(
    A_q: jax.Array,
    A_k: jax.Array,
    A_v: jax.Array,
    A_shift_k: jax.Array,
    A_ssm_k: jax.Array,
    A_ssm_D: jax.Array,
    B_x: jax.Array,
    B_w1: jax.Array,
    B_w3: jax.Array,
    B_w2: jax.Array,
    c: jax.Array,
    w_mod: jax.Array,
):
    del B_x
    fwd, inv = _dft_matrices()
    hbm = pl.BlockSpec(memory_space=pl.ANY)
    vmem = pltpu.VMEM
    out = pl.pallas_call(
        _kernel,
        in_specs=[hbm] * 13,
        out_specs=hbm,
        out_shape=jax.ShapeDtypeStruct((S, D), bf16),
        scratch_shapes=[
            vmem((KS, D), bf16), vmem((D,), bf16), vmem((1, D), bf16),
            vmem(fwd.shape, u32), vmem(inv.shape, u32),
            vmem((S, D), bf16),
            vmem((NL, S // 2 + 8, 128), u32), vmem((NL, S // 2, 128), u32),
            vmem((NL, H, S), u32),
            vmem((D // 2, F), u32), vmem((D // 2, F), u32), vmem((F // 2, D), u32),
            vmem((D // 2, 6 * D), u32),
            [vmem((2 * KO + 512, 128), f32) for _ in range(2)],
            [vmem((4 * C, 128), f32) for _ in range(NBLK // 2 - 1)],
            [vmem((2, C + 8, 128), f32) for _ in range(NBLK)],
            [vmem((2, C, 128), u32) for _ in range(NBLK)],
            vmem((NL, S // 2, 128), u32),
            vmem((NL, KS + 1, 8, 128), f32), pltpu.SMEM((1,), jnp.int32), vmem((5, 8, D), f32),
            vmem((2, R, D), f32), vmem((2, R // 2, D), u32),
            vmem((S, D), bf16),
            pltpu.SemaphoreType.DMA((NL + 11,)),
        ],
        compiler_params=pltpu.CompilerParams(vmem_limit_bytes=100 * 2**20),
    )(A_q.reshape(S, D), A_k.reshape(S, D), A_v.reshape(S, D), A_shift_k.T, A_ssm_k, A_ssm_D,
      B_w1, B_w3, B_w2, c, w_mod, fwd, inv)
    return out.reshape(1, S, D)
```

```python
import contextlib
import functools

import jax
import jax.numpy as jnp
import numpy as np
from jax import lax
from jax.experimental import pallas as pl
from jax.experimental.pallas import tpu as pltpu

S, D, F = 2048, 640, 1536
KS = 4
EPS = 1e-5
C = 128
H = C // 2
NBLK = S // (2 * C)
NL = D // 128
NT = C // 8
R = 256
LR = 32
TF = 512
OUT_COLS = (0, 256, 512, D)
NS = S // R
NG = F // TF
BS = (4 * NT + 4) * 8
KO = (NBLK * BS + 511) // 512 * 512 + 16
DFT_SPAN = 0.9
PFR = 0.75
PEEL = 3
M0 = 5
EARLY_INV = False
PRE_SPAN = 0.9

f32, bf16, u32 = jnp.float32, jnp.bfloat16, jnp.uint32


def _scope(name):
    del name
    return contextlib.nullcontext()


def _dft_matrices():
    f = np.concatenate([np.arange(0, C, 2), np.arange(1, C, 2)])
    zeta = 2 * np.pi * (f + 0.5) / (4 * C)

    def fwd(n):
        ang = zeta[:, None] * n[None, :]
        m = np.stack([np.cos(ang), -np.sin(ang)], 0)
        return m.reshape(2, NT, 8, C).transpose(1, 0, 2, 3).reshape(2 * C, C)

    def inv(n):
        ang = n[:, None] * zeta[None, :]
        return np.stack([np.cos(ang), -np.sin(ang)], -1).reshape(C, 2 * C) / (2 * C)

    def words(m):
        b = m.astype(np.float32).astype(bf16).view(np.uint16).astype(np.uint32)
        return b[0::2] | (b[1::2] << 16)

    j = np.arange(C)
    even = (j // 2) * 2 + (j % 2) * C
    return (words(np.concatenate([fwd(even), fwd(even + 1)], 0)),
            words(np.concatenate([inv(2 * j), inv(2 * j + 1)], 0)))


def _spec_row(filt, block, tile=0, part=0):
    return filt * KO + block * BS + (2 * tile + part) * 8


def _unpack(w, i):
    return pltpu.unpack_elementwise(w, index=i, packed_dtype=bf16, unpacked_dtype=f32)


def _pack(a, b):
    return pltpu.bitcast(pltpu.pack_elementwise([a, b], packed_dtype=bf16), u32)


def _as_bf16(w):
    return pltpu.bitcast(w, bf16)


def _dot(a, b):
    return jnp.dot(a, b, preferred_element_type=f32)


def _layernorm(x):
    xc = x - jnp.sum(x, axis=-1, keepdims=True) * (1.0 / D)
    var = jnp.sum(xc * xc, axis=-1, keepdims=True) * (1.0 / D)
    return xc * lax.rsqrt(var + EPS)


def _run_mixed(main, side):
    total, done, k = sum(w for w, _ in main), 0, 0
    for w, f in main:
        f()
        done += w
        while k < len(side) and (k + 0.5) * total <= done * len(side):
            side[k]()
            k += 1
    for f in side[k:]:
        f()


def _kernel(q_hbm, k_hbm, v_hbm, shk_hbm, ssm_hbm, d_hbm, w1_hbm, w3_hbm, w2_hbm, c_hbm, wm_hbm,
            fwd_hbm, inv_hbm, o_hbm,
            shk, dvec, cvec, fwd, inv, qb, kb, vb, sb, w1, w3, w2, wm,
            spec, zlast, kf, zb, yb, cpar, zero, par, x1b, h2b, ob, sems):
    k32, v32, s32, wm32, w132, w332, w232 = (
        a.bitcast(u32) for a in (k_hbm, v_hbm, ssm_hbm, wm_hbm, w1_hbm, w3_hbm, w2_hbm))

    def conv_inputs(l, t0, n):
        cols = pl.ds(l * 128, 128)
        return [(s32.at[pl.ds(l * H, H), pl.ds(t0, n)], sb.at[l, :, pl.ds(t0, n)]),
                (k32.at[pl.ds(t0 // 2, n // 2), cols], kb.at[l, pl.ds(8 + t0 // 2, n // 2)]),
                (v32.at[pl.ds(t0 // 2, n // 2), cols], vb.at[l, pl.ds(t0 // 2, n // 2)])]

    def same(src, dst, *idx):
        return src.at[idx], dst.at[idx]

    mod_cols = lambda c0, n: same(wm32, wm, slice(None), pl.ds(c0, n))
    up_cols = lambda g: [same(w132, w1, slice(None), pl.ds(g * TF, TF)),
                         same(w332, w3, slice(None), pl.ds(g * TF, TF))]
    down_rows = lambda g: same(w232, w2, pl.ds(g * TF // 2, TF // 2))
    q_rows = lambda r0, n: same(q_hbm, qb, pl.ds(r0, n))
    groups = {
        'params': [(shk_hbm, shk), (d_hbm, dvec), (c_hbm, cvec)],
        'first': [(fwd_hbm, fwd)] + conv_inputs(0, 0, S // 2),
        0: conv_inputs(0, S // 2, S // 2),
        1: conv_inputs(1, 0, S),
        'inv': [(inv_hbm, inv)],
        **{l: conv_inputs(l, 0, S) for l in range(2, NL)},
        'mod': [mod_cols(0, 5 * D), q_rows(0, R)],
        'ffn0': [same(w132, w1, slice(None), pl.ds(0, 2 * TF)), up_cols(0)[1]],
        'ffn1': up_cols(1)[1:] + [down_rows(0)] + up_cols(2)[:1],
        'ffn2': [q_rows(R, R)] + up_cols(2)[1:] + [down_rows(1)],
        'ffn3': [mod_cols(5 * D, D), down_rows(2)],
        'q': [q_rows(2 * R, 2 * R)],
        'q_late': [q_rows(4 * R, S - 4 * R)],
    }
    named = [g for g in groups if isinstance(g, str)]
    sem_of = lambda g: sems.at[NL + named.index(g) if isinstance(g, str) else g]
    out_sem = sems.at[NL + len(named)]

    def wait(g, pairs=None):
        with _scope('wait_' + (g if isinstance(g, str) else 'slab')):
            for src, dst in (groups[g] if pairs is None else pairs):
                pltpu.make_async_copy(src, dst, sem_of(g)).wait()

    def out_copy(r0, cols=slice(None)):
        return pltpu.make_async_copy(*same(ob, o_hbm, pl.ds(r0, R), cols), out_sem)

    for g, pairs in groups.items():
        for src, dst in pairs:
            pltpu.make_async_copy(src, dst, sem_of(g)).start()

    wait('params')
    taps = shk[...].astype(f32)
    skip = dvec[...].astype(f32).reshape(1, D)
    for l in range(NL):
        kb[l, 0:8, :] = jnp.zeros((8, 128), u32)
        for j in range(KS):
            cpar[l, j] = jnp.broadcast_to(taps[j:j + 1, l * 128:(l + 1) * 128], (8, 128))
        cpar[l, KS] = jnp.broadcast_to(skip[:, l * 128:(l + 1) * 128], (8, 128))
    zero[0] = 0
    z0 = pl.multiple_of(zero[0] * 1024, 1024)

    def forward_pieces(l, buf):
        param = lambda j, rows: jnp.broadcast_to(cpar[l, j, 0:1, :], (rows, 128))
        mat = lambda i: _as_bf16(fwd[i * C:(i + 1) * C, :])

        def butterfly(filt, j, even, odd):
            r = _spec_row(filt, j)
            spec[buf][r:r + 2 * C, :] = even + odd
            spec[buf][r + 2 * C:r + 4 * C, :] = even - odd

        def signal(j):
            def f():
                kw = kb[l, j * C:j * C + C + 8, :]
                ke, ko = _unpack(kw, 0), _unpack(kw, 1)
                kf[j][0] = ke
                kf[j][1] = ko
                ke1, ko1, ko2 = kf[j][0, 7:7 + C, :], kf[j][1, 7:7 + C, :], kf[j][1, 6:6 + C, :]
                ke, ko = ke[8:], ko[8:]
                t0, t1, t2, t3 = (param(t, C) for t in range(KS))
                vw = vb[l, j * C:(j + 1) * C, :]
                xe = (t0 * ke + t1 * ko1 + t2 * ke1 + t3 * ko2) * _unpack(vw, 0)
                xo = (t0 * ko + t1 * ke + t2 * ko1 + t3 * ke1) * _unpack(vw, 1)
                butterfly(0, j, _dot(mat(0), _as_bf16(_pack(xe[:H], xe[H:]))),
                          _dot(mat(1), _as_bf16(_pack(xo[:H], xo[H:]))))
            return f

        def long_filter(j):
            def f():
                lo = sb[l, :, 2 * j * C:(2 * j + 1) * C]
                hi = sb[l, :, (2 * j + 1) * C:(2 * j + 2) * C]
                even_lane = lax.broadcasted_iota(jnp.int32, lo.shape, 1) % 2 == 0
                te = jnp.where(even_lane, lo, pltpu.roll(hi, 1, 1))
                to = jnp.where(even_lane, pltpu.roll(lo, C - 1, 1), hi)
                dims = (((1,), (1,)), ((), ()))
                pe = lax.dot_general(mat(0), _as_bf16(te), dims, preferred_element_type=f32)
                po = lax.dot_general(mat(1), _as_bf16(to), dims, preferred_element_type=f32)
                if j == 0:
                    real = lax.broadcasted_iota(jnp.int32, pe.shape, 0) % 16 < 8
                    pe = pe + jnp.where(real, param(KS, 2 * C), 0.0)
                butterfly(1, j, pe, po)
            return f
        return [piece(j) for j in range(NBLK) for piece in (signal, long_filter)]

    def product_pieces(buf):
        load = lambda filt, j, tile: [
            spec[buf][pl.ds(z0 + _spec_row(filt, j, tile, c), 8), :] for c in range(2)]

        def piece(p, t):
            def plus_tail(z, prev):
                if t < NT // 2:
                    return [z[0] - prev[1], z[1] + prev[0]]
                return [z[0] + prev[1], z[1] - prev[0]]

            def f():
                res = []
                for tile in (t, NT + t):
                    acc, xs = [None, None], {}
                    for m in range(2 * p + 2):
                        kr, ki = load(1, m, tile)
                        for i in range(2):
                            j = 2 * p + i - m
                            if j < 0:
                                continue
                            if j not in xs:
                                xs[j] = load(0, j, tile)
                            xr, xi = xs[j]
                            term = [kr * xr - ki * xi, kr * xi + ki * xr]
                            acc[i] = term if acc[i] is None else [a + b for a, b in zip(acc[i], term)]
                    row = tile * 16
                    first = acc[0]
                    if p > 0:
                        first = plus_tail(first, [zlast[p - 1][pl.ds(z0 + row + 8 * c, 8), :] for c in range(2)])
                    if 2 * p + 2 < NBLK:
                        for c in range(2):
                            zlast[p][row + 8 * c:row + 8 * c + 8, :] = acc[1][c]
                    res.append([first, plus_tail(acc[1], acc[0])])
                for i in range(2):
                    (ar, ai), (br, bi) = res[0][i], res[1][i]
                    zb[2 * p + i][0, 8 * t:8 * t + 8, :] = _pack(ar + br, ai + bi)
                    zb[2 * p + i][1, 8 * t:8 * t + 8, :] = _pack(ar - br, ai - bi)
            return f
        return [(4 * p + 5, piece(p, t)) for p in range(NBLK // 2) for t in range(NT)]

    def inverse(l, j):
        ye, yo = (_dot(_as_bf16(inv[i * H:(i + 1) * H, :]), _as_bf16(zb[j][i, pl.ds(z0, C), :]))
                  for i in range(2))
        yb[l, j * C:(j + 1) * C, :] = _pack(ye, yo)

    def conv_step(l, buf, early=0):
        products = product_pieces(buf)
        for _, f in products[:early]:
            f()
        if early:
            wait('inv')
        wait(l + 1, conv_inputs(l + 1, 0, S))
        for j in range(2 * (early // NT) - 2):
            inverse(l, j)
        ahead = forward_pieces(l + 1, 1 - buf)
        total, done, k = sum(w for w, _ in products[early:]), 0, 0
        for i, (w, f) in list(enumerate(products))[early:]:
            while k < len(ahead) and (k + 1) * total * DFT_SPAN <= done * (len(ahead) + 1):
                ahead[k]()
                k += 1
            f()
            done += w
            p, t = divmod(i, NT)
            if p > 0 and t in (NT // 4, 3 * NT // 4):
                inverse(l, 2 * p - 2 + (t > NT // 2))
        for f in ahead[k:]:
            f()
        inverse(l, NBLK - 2)
        inverse(l, NBLK - 1)

    ahead = forward_pieces(0, 0)
    wait('first')
    for f in ahead[:NBLK]:
        f()
    wait(0)
    for f in ahead[NBLK:]:
        f()
    if PEEL:
        conv_step(0, 0, PEEL * NT)
        for l in range(1, NL - 1):
            conv_step(l, l % 2)
    else:
        wait('inv')

        def conv_body(i, carry):
            conv_step(2 * i, 0)
            conv_step(2 * i + 1, 1)
            return carry
        lax.fori_loop(0, NL // 2, conv_body, 0)

    cond = cvec[...].astype(f32)
    cond = jnp.broadcast_to(cond * jax.nn.sigmoid(cond), (16, D)).astype(bf16)
    mod = lambda j: _dot(cond, _as_bf16(wm[:, j * D:(j + 1) * D]))[0:8]
    row = lambda j, rows, cols=slice(None): par[j, 0:1, cols]

    def norm_pieces(s):
        static = isinstance(s, int)
        slot = s % 2 if static else lax.rem(s, 2)

        def piece(i):
            def f():
                r, r2 = s * R + i * LR, s * (R // 2) + i * (LR // 2)
                if not static:
                    r, r2 = pl.multiple_of(r, LR), pl.multiple_of(r2, LR // 2)
                x = qb[pl.ds(r, LR), :].astype(f32)
                y = jnp.concatenate(
                    [_as_bf16(yb[l, pl.ds(r2, LR // 2), :]).astype(f32) for l in range(NL)], axis=1)
                x = x + (_layernorm(x) * row(0, LR) + row(1, LR)) * y
                h = _layernorm(x) * row(2, LR) + row(3, LR)
                x1b[slot, i * LR:(i + 1) * LR, :] = x
                h2b[slot, i * LR // 2:(i + 1) * LR // 2, :] = pltpu.bitcast(h.astype(bf16), u32)
            return f
        return [piece(i) for i in range(R // LR)]

    def ffn_groups(s):
        static = isinstance(s, int)
        slot = s % 2 if static else lax.rem(s, 2)
        r0 = s * R if static else pl.multiple_of(s * R, R)
        st = {}

        def gate(g):
            def f():
                st['gate'] = _dot(_as_bf16(h2b[slot]), _as_bf16(w1[:, g * TF:(g + 1) * TF]))
            return f

        def up(g):
            def f():
                u = _dot(_as_bf16(h2b[slot]), _as_bf16(w3[:, g * TF:(g + 1) * TF]))
                half = 0.5 * st['gate']
                st[g] = ((half * jnp.tanh(half) + half) * u).astype(bf16)
            return f

        def down(g, c0, c1):
            def f():
                p = _dot(st[g], _as_bf16(w2[g * TF // 2:(g + 1) * TF // 2, c0:c1]))
                if g + 1 < NG:
                    st['acc'] = p if g == 0 else st['acc'] + p
                    return
                y = st['acc'][:, c0:c1] + p
                ob[pl.ds(r0, R), c0:c1] = (x1b[slot, :, c0:c1] + row(4, R, slice(c0, c1)) * y).astype(bf16)
                if static and s == NS - 1:
                    out_copy(r0, pl.ds(c0, c1 - c0)).start()
            return f
        ups = [[(D, gate(g)), (D, up(g))] for g in range(NG)]
        downs = [[(D, down(g, 0, D))] for g in range(NG - 1)]
        downs.append([(c1 - c0, down(NG - 1, c0, c1)) for c0, c1 in zip(OUT_COLS[:-1], OUT_COLS[1:])])
        return [ups[0], ups[1], downs[0], ups[2], downs[1], downs[2]]

    products = product_pieces(0)
    for _, f in products[:M0 * NT // 2]:
        f()
    wait('mod')
    scale_a, gate_a, shift_a, scale_b, shift_b = (mod(j) for j in (1, 2, 0, 4, 3))
    par[0] = gate_a * (1.0 + scale_a)
    par[1] = gate_a * shift_a
    par[2] = 1.0 + scale_b
    par[3] = shift_b
    if EARLY_INV:
        inverse(NL - 1, 0)
        inverse(NL - 1, 1)
    for _, f in products[M0 * NT // 2:]:
        f()
    if not EARLY_INV:
        inverse(NL - 1, 0)
        inverse(NL - 1, 1)
    _run_mixed([(1, f) for f in norm_pieces(0)],
               [functools.partial(inverse, NL - 1, j) for j in range(2, NBLK)])

    ffn, norms = [p for g in ffn_groups(0) for p in g], norm_pieces(1)
    n = int(len(norms) * PFR)
    wait('ffn0')
    _run_mixed(ffn[:3], [])
    wait('ffn1')
    _run_mixed(ffn[3:6], [])
    wait('ffn2')
    _run_mixed(ffn[6:8], norms[:n])
    wait('ffn3')
    par[4] = mod(5)
    _run_mixed(ffn[8:], norms[n:])
    out_copy(0).start()
    wait('q')

    def ffn_body(s, carry):
        pl.when(s == 3)(lambda: wait('q_late'))
        pieces = [p for g in ffn_groups(s) for p in g]
        n = int(len(pieces) * PRE_SPAN)
        _run_mixed(pieces[:n], norm_pieces(s + 1))
        _run_mixed(pieces[n:], [])
        out_copy(pl.multiple_of(s * R, R)).start()
        return carry
    with _scope('ffn_loop'):
        lax.fori_loop(1, NS - 1, ffn_body, 0)
    _run_mixed([p for g in ffn_groups(NS - 1) for p in g], [])

    with _scope('wait_out'):
        for s in range(NS - 1):
            out_copy(s * R).wait()
        for c0, c1 in zip(OUT_COLS[:-1], OUT_COLS[1:]):
            out_copy(S - R, pl.ds(c0, c1 - c0)).wait()


@jax.jit
def pallas_adaLN_cond__ssm_conv_h3__glu_gated_swiglu__prompt_kernel(
    A_q: jax.Array,
    A_k: jax.Array,
    A_v: jax.Array,
    A_shift_k: jax.Array,
    A_ssm_k: jax.Array,
    A_ssm_D: jax.Array,
    B_x: jax.Array,
    B_w1: jax.Array,
    B_w3: jax.Array,
    B_w2: jax.Array,
    c: jax.Array,
    w_mod: jax.Array,
):
    del B_x
    fwd, inv = _dft_matrices()
    hbm = pl.BlockSpec(memory_space=pl.ANY)
    vmem = pltpu.VMEM
    out = pl.pallas_call(
        _kernel,
        in_specs=[hbm] * 13,
        out_specs=hbm,
        out_shape=jax.ShapeDtypeStruct((S, D), bf16),
        scratch_shapes=[
            vmem((KS, D), bf16), vmem((D,), bf16), vmem((1, D), bf16),
            vmem(fwd.shape, u32), vmem(inv.shape, u32),
            vmem((S, D), bf16),
            vmem((NL, S // 2 + 8, 128), u32), vmem((NL, S // 2, 128), u32),
            vmem((NL, H, S), u32),
            vmem((D // 2, F), u32), vmem((D // 2, F), u32), vmem((F // 2, D), u32),
            vmem((D // 2, 6 * D), u32),
            [vmem((2 * KO + 512, 128), f32) for _ in range(2)],
            [vmem((4 * C, 128), f32) for _ in range(NBLK // 2 - 1)],
            [vmem((2, C + 8, 128), f32) for _ in range(NBLK)],
            [vmem((2, C, 128), u32) for _ in range(NBLK)],
            vmem((NL, S // 2, 128), u32),
            vmem((NL, KS + 1, 8, 128), f32), pltpu.SMEM((1,), jnp.int32), vmem((5, 8, D), f32),
            vmem((2, R, D), f32), vmem((2, R // 2, D), u32),
            vmem((S, D), bf16),
            pltpu.SemaphoreType.DMA((NL + 11,)),
        ],
        compiler_params=pltpu.CompilerParams(vmem_limit_bytes=100 * 2**20),
    )(A_q.reshape(S, D), A_k.reshape(S, D), A_v.reshape(S, D), A_shift_k.T, A_ssm_k, A_ssm_D,
      B_w1, B_w3, B_w2, c, w_mod, fwd, inv)
    return out.reshape(1, S, D)
```

```python
import contextlib
import functools

import jax
import jax.numpy as jnp
import numpy as np
from jax import lax
from jax.experimental import pallas as pl
from jax.experimental.pallas import tpu as pltpu

S, D, F = 2048, 640, 1536
KS = 4
EPS = 1e-5
C = 128
H = C // 2
NBLK = S // (2 * C)
NL = D // 128
NT = C // 8
R = 256
LR = 32
TF = 512
OUT_COLS = (0, 256, 512, D)
NS = S // R
NG = F // TF
BS = (4 * NT + 4) * 8
KO = (NBLK * BS + 511) // 512 * 512 + 16
DFT_SPAN = 0.9
PRE_SPAN = 0.9

f32, bf16, u32 = jnp.float32, jnp.bfloat16, jnp.uint32


def _scope(name):
    del name
    return contextlib.nullcontext()


def _dft_matrices():
    f = np.concatenate([np.arange(0, C, 2), np.arange(1, C, 2)])
    zeta = 2 * np.pi * (f + 0.5) / (4 * C)

    def fwd(n):
        ang = zeta[:, None] * n[None, :]
        m = np.stack([np.cos(ang), -np.sin(ang)], 0)
        return m.reshape(2, NT, 8, C).transpose(1, 0, 2, 3).reshape(2 * C, C)

    def inv(n):
        ang = n[:, None] * zeta[None, :]
        return np.stack([np.cos(ang), -np.sin(ang)], -1).reshape(C, 2 * C) / (2 * C)

    def words(m):
        b = m.astype(np.float32).astype(bf16).view(np.uint16).astype(np.uint32)
        return b[0::2] | (b[1::2] << 16)

    j = np.arange(C)
    even = (j // 2) * 2 + (j % 2) * C
    return (words(np.concatenate([fwd(even), fwd(even + 1)], 0)),
            words(np.concatenate([inv(2 * j), inv(2 * j + 1)], 0)))


def _spec_row(filt, block, tile=0, part=0):
    return filt * KO + block * BS + (2 * tile + part) * 8


def _unpack(w, i):
    return pltpu.unpack_elementwise(w, index=i, packed_dtype=bf16, unpacked_dtype=f32)


def _pack(a, b):
    return pltpu.bitcast(pltpu.pack_elementwise([a, b], packed_dtype=bf16), u32)


def _as_bf16(w):
    return pltpu.bitcast(w, bf16)


def _dot(a, b):
    return jnp.dot(a, b, preferred_element_type=f32)


def _layernorm(x):
    xc = x - jnp.sum(x, axis=-1, keepdims=True) * (1.0 / D)
    var = jnp.sum(xc * xc, axis=-1, keepdims=True) * (1.0 / D)
    return xc * lax.rsqrt(var + EPS)


def _run_mixed(main, side):
    total, done, k = sum(w for w, _ in main), 0, 0
    for w, f in main:
        f()
        done += w
        while k < len(side) and (k + 0.5) * total <= done * len(side):
            side[k]()
            k += 1
    for f in side[k:]:
        f()


def _kernel(q_hbm, k_hbm, v_hbm, shk_hbm, ssm_hbm, d_hbm, w1_hbm, w3_hbm, w2_hbm, c_hbm, wm_hbm,
            fwd_hbm, inv_hbm, o_hbm,
            shk, dvec, cvec, fwd, inv, qb, kb, vb, sb, w1, w3, w2, wm,
            spec, zlast, kf, zb, yb, cpar, zero, par, x1b, h2b, ob, sems):
    k32, v32, s32, wm32, w132, w332, w232 = (
        a.bitcast(u32) for a in (k_hbm, v_hbm, ssm_hbm, wm_hbm, w1_hbm, w3_hbm, w2_hbm))

    def conv_inputs(l, t0, n):
        cols = pl.ds(l * 128, 128)
        return [(s32.at[pl.ds(l * H, H), pl.ds(t0, n)], sb.at[l, :, pl.ds(t0, n)]),
                (k32.at[pl.ds(t0 // 2, n // 2), cols], kb.at[l, pl.ds(8 + t0 // 2, n // 2)]),
                (v32.at[pl.ds(t0 // 2, n // 2), cols], vb.at[l, pl.ds(t0 // 2, n // 2)])]

    def same(src, dst, *idx):
        return src.at[idx], dst.at[idx]

    mod_cols = lambda c0, n: same(wm32, wm, slice(None), pl.ds(c0, n))
    up_cols = lambda g: [same(w132, w1, slice(None), pl.ds(g * TF, TF)),
                         same(w332, w3, slice(None), pl.ds(g * TF, TF))]
    down_rows = lambda g: same(w232, w2, pl.ds(g * TF // 2, TF // 2))
    q_rows = lambda r0, n: same(q_hbm, qb, pl.ds(r0, n))
    groups = {
        'params': [(shk_hbm, shk), (d_hbm, dvec), (c_hbm, cvec)],
        'first': [(fwd_hbm, fwd)] + conv_inputs(0, 0, S // 2),
        0: conv_inputs(0, S // 2, S // 2),
        1: conv_inputs(1, 0, S),
        'inv': [(inv_hbm, inv)],
        **{l: conv_inputs(l, 0, S) for l in range(2, NL)},
        'mod': [mod_cols(0, 5 * D), q_rows(0, R)],
        'ffn0': [same(w132, w1, slice(None), pl.ds(0, 2 * TF)), up_cols(0)[1]],
        'ffn1': up_cols(1)[1:] + [down_rows(0)] + up_cols(2)[:1],
        'ffn2': [q_rows(R, R)] + up_cols(2)[1:] + [down_rows(1)],
        'ffn3': [mod_cols(5 * D, D), down_rows(2)],
        'q': [q_rows(2 * R, 2 * R)],
        'q_late': [q_rows(4 * R, S - 4 * R)],
    }
    named = [g for g in groups if isinstance(g, str)]
    sem_of = lambda g: sems.at[NL + named.index(g) if isinstance(g, str) else g]
    out_sem = sems.at[NL + len(named)]

    def wait(g, pairs=None):
        with _scope('wait_' + (g if isinstance(g, str) else 'slab')):
            for src, dst in (groups[g] if pairs is None else pairs):
                pltpu.make_async_copy(src, dst, sem_of(g)).wait()

    def out_copy(r0, cols=slice(None)):
        return pltpu.make_async_copy(*same(ob, o_hbm, pl.ds(r0, R), cols), out_sem)

    for g, pairs in groups.items():
        for src, dst in pairs:
            pltpu.make_async_copy(src, dst, sem_of(g)).start()

    wait('params')
    taps = shk[...].astype(f32)
    skip = dvec[...].astype(f32).reshape(1, D)
    for l in range(NL):
        kb[l, 0:8, :] = jnp.zeros((8, 128), u32)
        for j in range(KS):
            cpar[l, j] = jnp.broadcast_to(taps[j:j + 1, l * 128:(l + 1) * 128], (8, 128))
        cpar[l, KS] = jnp.broadcast_to(skip[:, l * 128:(l + 1) * 128], (8, 128))
    zero[0] = 0
    z0 = pl.multiple_of(zero[0] * 1024, 1024)

    def forward_pieces(l, buf):
        param = lambda j, rows: jnp.broadcast_to(cpar[l, j, 0:1, :], (rows, 128))
        mat = lambda i: _as_bf16(fwd[i * C:(i + 1) * C, :])

        def butterfly(filt, j, even, odd):
            r = _spec_row(filt, j)
            spec[buf][r:r + 2 * C, :] = even + odd
            spec[buf][r + 2 * C:r + 4 * C, :] = even - odd

        def signal(j):
            def f():
                kw = kb[l, j * C:j * C + C + 8, :]
                ke, ko = _unpack(kw, 0), _unpack(kw, 1)
                kf[j][0] = ke
                kf[j][1] = ko
                ke1, ko1, ko2 = kf[j][0, 7:7 + C, :], kf[j][1, 7:7 + C, :], kf[j][1, 6:6 + C, :]
                ke, ko = ke[8:], ko[8:]
                t0, t1, t2, t3 = (param(t, C) for t in range(KS))
                vw = vb[l, j * C:(j + 1) * C, :]
                xe = (t0 * ke + t1 * ko1 + t2 * ke1 + t3 * ko2) * _unpack(vw, 0)
                xo = (t0 * ko + t1 * ke + t2 * ko1 + t3 * ke1) * _unpack(vw, 1)
                butterfly(0, j, _dot(mat(0), _as_bf16(_pack(xe[:H], xe[H:]))),
                          _dot(mat(1), _as_bf16(_pack(xo[:H], xo[H:]))))
            return f

        def long_filter(j):
            def f():
                lo = sb[l, :, 2 * j * C:(2 * j + 1) * C]
                hi = sb[l, :, (2 * j + 1) * C:(2 * j + 2) * C]
                even_lane = lax.broadcasted_iota(jnp.int32, lo.shape, 1) % 2 == 0
                te = jnp.where(even_lane, lo, pltpu.roll(hi, 1, 1))
                to = jnp.where(even_lane, pltpu.roll(lo, C - 1, 1), hi)
                dims = (((1,), (1,)), ((), ()))
                pe = lax.dot_general(mat(0), _as_bf16(te), dims, preferred_element_type=f32)
                po = lax.dot_general(mat(1), _as_bf16(to), dims, preferred_element_type=f32)
                if j == 0:
                    real = lax.broadcasted_iota(jnp.int32, pe.shape, 0) % 16 < 8
                    pe = pe + jnp.where(real, param(KS, 2 * C), 0.0)
                butterfly(1, j, pe, po)
            return f
        return [piece(j) for j in range(NBLK) for piece in (signal, long_filter)]

    def product_pieces(buf):
        load = lambda filt, j, tile: [
            spec[buf][pl.ds(z0 + _spec_row(filt, j, tile, c), 8), :] for c in range(2)]

        def piece(p, t):
            def plus_tail(z, prev):
                if t < NT // 2:
                    return [z[0] - prev[1], z[1] + prev[0]]
                return [z[0] + prev[1], z[1] - prev[0]]

            def f():
                res = []
                for tile in (t, NT + t):
                    acc, xs = [None, None], {}
                    for m in range(2 * p + 2):
                        kr, ki = load(1, m, tile)
                        for i in range(2):
                            j = 2 * p + i - m
                            if j < 0:
                                continue
                            if j not in xs:
                                xs[j] = load(0, j, tile)
                            xr, xi = xs[j]
                            term = [kr * xr - ki * xi, kr * xi + ki * xr]
                            acc[i] = term if acc[i] is None else [a + b for a, b in zip(acc[i], term)]
                    row = tile * 16
                    first = acc[0]
                    if p > 0:
                        first = plus_tail(first, [zlast[p - 1][pl.ds(z0 + row + 8 * c, 8), :] for c in range(2)])
                    if 2 * p + 2 < NBLK:
                        for c in range(2):
                            zlast[p][row + 8 * c:row + 8 * c + 8, :] = acc[1][c]
                    res.append([first, plus_tail(acc[1], acc[0])])
                for i in range(2):
                    (ar, ai), (br, bi) = res[0][i], res[1][i]
                    zb[2 * p + i][0, 8 * t:8 * t + 8, :] = _pack(ar + br, ai + bi)
                    zb[2 * p + i][1, 8 * t:8 * t + 8, :] = _pack(ar - br, ai - bi)
            return f
        return [(4 * p + 5, piece(p, t)) for p in range(NBLK // 2) for t in range(NT)]

    def inverse(l, j):
        ye, yo = (_dot(_as_bf16(inv[i * H:(i + 1) * H, :]), _as_bf16(zb[j][i, pl.ds(z0, C), :]))
                  for i in range(2))
        yb[l, j * C:(j + 1) * C, :] = _pack(ye, yo)

    def conv_step(l, buf, early=0):
        products = product_pieces(buf)
        for _, f in products[:early]:
            f()
        if early:
            wait('inv')
        wait(l + 1, conv_inputs(l + 1, 0, S))
        for j in range(2 * (early // NT) - 2):
            inverse(l, j)
        ahead = forward_pieces(l + 1, 1 - buf)
        total, done, k = sum(w for w, _ in products[early:]), 0, 0
        for i, (w, f) in list(enumerate(products))[early:]:
            while k < len(ahead) and (k + 1) * total * DFT_SPAN <= done * (len(ahead) + 1):
                ahead[k]()
                k += 1
            f()
            done += w
            p, t = divmod(i, NT)
            if p > 0 and t in (NT // 4, 3 * NT // 4):
                inverse(l, 2 * p - 2 + (t > NT // 2))
        for f in ahead[k:]:
            f()
        inverse(l, NBLK - 2)
        inverse(l, NBLK - 1)

    ahead = forward_pieces(0, 0)
    wait('first')
    for f in ahead[:NBLK]:
        f()
    wait(0)
    for f in ahead[NBLK:]:
        f()
    conv_step(0, 0, early=3 * NT)
    for l in range(1, NL - 1):
        conv_step(l, l % 2)

    cond = cvec[...].astype(f32)
    cond = jnp.broadcast_to(cond * jax.nn.sigmoid(cond), (16, D)).astype(bf16)
    mod = lambda j: _dot(cond, _as_bf16(wm[:, j * D:(j + 1) * D]))[0:8]
    row = lambda j, rows, cols=slice(None): par[j, 0:1, cols]

    def norm_pieces(s):
        static = isinstance(s, int)
        slot = s % 2 if static else lax.rem(s, 2)

        def piece(i):
            def f():
                r, r2 = s * R + i * LR, s * (R // 2) + i * (LR // 2)
                if not static:
                    r, r2 = pl.multiple_of(r, LR), pl.multiple_of(r2, LR // 2)
                x = qb[pl.ds(r, LR), :].astype(f32)
                y = jnp.concatenate(
                    [_as_bf16(yb[l, pl.ds(r2, LR // 2), :]).astype(f32) for l in range(NL)], axis=1)
                x = x + (_layernorm(x) * row(0, LR) + row(1, LR)) * y
                h = _layernorm(x) * row(2, LR) + row(3, LR)
                x1b[slot, i * LR:(i + 1) * LR, :] = x
                h2b[slot, i * LR // 2:(i + 1) * LR // 2, :] = pltpu.bitcast(h.astype(bf16), u32)
            return f
        return [piece(i) for i in range(R // LR)]

    def ffn_pieces(s):
        static = isinstance(s, int)
        slot = s % 2 if static else lax.rem(s, 2)
        r0 = s * R if static else pl.multiple_of(s * R, R)
        st = {}

        def gate(g):
            def f():
                st['gate'] = _dot(_as_bf16(h2b[slot]), _as_bf16(w1[:, g * TF:(g + 1) * TF]))
            return f

        def up(g):
            def f():
                u = _dot(_as_bf16(h2b[slot]), _as_bf16(w3[:, g * TF:(g + 1) * TF]))
                half = 0.5 * st['gate']
                st[g] = ((half * jnp.tanh(half) + half) * u).astype(bf16)
            return f

        def down(g, c0, c1):
            def f():
                p = _dot(st[g], _as_bf16(w2[g * TF // 2:(g + 1) * TF // 2, c0:c1]))
                if g + 1 < NG:
                    st['acc'] = p if g == 0 else st['acc'] + p
                    return
                y = st['acc'][:, c0:c1] + p
                ob[pl.ds(r0, R), c0:c1] = (x1b[slot, :, c0:c1] + row(4, R, slice(c0, c1)) * y).astype(bf16)
                if static and s == NS - 1:
                    out_copy(r0, pl.ds(c0, c1 - c0)).start()
            return f
        ups = [[(D, gate(g)), (D, up(g))] for g in range(NG)]
        downs = [[(D, down(g, 0, D))] for g in range(NG - 1)]
        downs.append([(c1 - c0, down(NG - 1, c0, c1)) for c0, c1 in zip(OUT_COLS[:-1], OUT_COLS[1:])])
        return ups[0] + ups[1] + downs[0] + ups[2] + downs[1] + downs[2]

    products = product_pieces(0)
    for _, f in products[:5 * NT // 2]:
        f()
    wait('mod')
    scale_a, gate_a, shift_a, scale_b, shift_b = (mod(j) for j in (1, 2, 0, 4, 3))
    par[0] = gate_a * (1.0 + scale_a)
    par[1] = gate_a * shift_a
    par[2] = 1.0 + scale_b
    par[3] = shift_b
    for _, f in products[5 * NT // 2:]:
        f()
    inverse(NL - 1, 0)
    inverse(NL - 1, 1)
    _run_mixed([(1, f) for f in norm_pieces(0)],
               [functools.partial(inverse, NL - 1, j) for j in range(2, NBLK)])

    ffn, norms = ffn_pieces(0), norm_pieces(1)
    n = 3 * len(norms) // 4
    wait('ffn0')
    _run_mixed(ffn[:3], [])
    wait('ffn1')
    _run_mixed(ffn[3:6], [])
    wait('ffn2')
    _run_mixed(ffn[6:8], norms[:n])
    wait('ffn3')
    par[4] = mod(5)
    _run_mixed(ffn[8:], norms[n:])
    out_copy(0).start()
    wait('q')

    def ffn_body(s, carry):
        pl.when(s == 3)(lambda: wait('q_late'))
        pieces = ffn_pieces(s)
        n = int(len(pieces) * PRE_SPAN)
        _run_mixed(pieces[:n], norm_pieces(s + 1))
        _run_mixed(pieces[n:], [])
        out_copy(pl.multiple_of(s * R, R)).start()
        return carry
    with _scope('ffn_loop'):
        lax.fori_loop(1, NS - 1, ffn_body, 0)
    _run_mixed(ffn_pieces(NS - 1), [])

    with _scope('wait_out'):
        for s in range(NS - 1):
            out_copy(s * R).wait()
        for c0, c1 in zip(OUT_COLS[:-1], OUT_COLS[1:]):
            out_copy(S - R, pl.ds(c0, c1 - c0)).wait()


@jax.jit
def pallas_adaLN_cond__ssm_conv_h3__glu_gated_swiglu__prompt_kernel(
    A_q: jax.Array,
    A_k: jax.Array,
    A_v: jax.Array,
    A_shift_k: jax.Array,
    A_ssm_k: jax.Array,
    A_ssm_D: jax.Array,
    B_x: jax.Array,
    B_w1: jax.Array,
    B_w3: jax.Array,
    B_w2: jax.Array,
    c: jax.Array,
    w_mod: jax.Array,
):
    del B_x
    fwd, inv = _dft_matrices()
    hbm = pl.BlockSpec(memory_space=pl.ANY)
    vmem = pltpu.VMEM
    out = pl.pallas_call(
        _kernel,
        in_specs=[hbm] * 13,
        out_specs=hbm,
        out_shape=jax.ShapeDtypeStruct((S, D), bf16),
        scratch_shapes=[
            vmem((KS, D), bf16), vmem((D,), bf16), vmem((1, D), bf16),
            vmem(fwd.shape, u32), vmem(inv.shape, u32),
            vmem((S, D), bf16),
            vmem((NL, S // 2 + 8, 128), u32), vmem((NL, S // 2, 128), u32),
            vmem((NL, H, S), u32),
            vmem((D // 2, F), u32), vmem((D // 2, F), u32), vmem((F // 2, D), u32),
            vmem((D // 2, 6 * D), u32),
            [vmem((2 * KO + 512, 128), f32) for _ in range(2)],
            [vmem((4 * C, 128), f32) for _ in range(NBLK // 2 - 1)],
            [vmem((2, C + 8, 128), f32) for _ in range(NBLK)],
            [vmem((2, C, 128), u32) for _ in range(NBLK)],
            vmem((NL, S // 2, 128), u32),
            vmem((NL, KS + 1, 8, 128), f32), pltpu.SMEM((1,), jnp.int32), vmem((5, 8, D), f32),
            vmem((2, R, D), f32), vmem((2, R // 2, D), u32),
            vmem((S, D), bf16),
            pltpu.SemaphoreType.DMA((NL + 11,)),
        ],
        compiler_params=pltpu.CompilerParams(vmem_limit_bytes=100 * 2**20),
    )(A_q.reshape(S, D), A_k.reshape(S, D), A_v.reshape(S, D), A_shift_k.T, A_ssm_k, A_ssm_D,
      B_w1, B_w3, B_w2, c, w_mod, fwd, inv)
    return out.reshape(1, S, D)
```

```python
import contextlib
import functools

import jax
import jax.numpy as jnp
import numpy as np
from jax import lax
from jax.experimental import pallas as pl
from jax.experimental.pallas import tpu as pltpu

S, D, F = 2048, 640, 1536
KS = 4
EPS = 1e-5
C = 128
H = C // 2
NBLK = S // (2 * C)
NL = D // 128
NT = C // 8
R = 256
LR = 32
TF = 512
OUT_COLS = (0, 256, 512, D)
NS = S // R
NG = F // TF
RH, DH, FH = R // 2, 256, F // 2
BS = (4 * NT + 4) * 8
KO = (NBLK * BS + 511) // 512 * 512 + 16
DFT_SPAN = 0.9
PRE_SPAN = 0.9

f32, bf16, u32 = jnp.float32, jnp.bfloat16, jnp.uint32


def _scope(name):
    del name
    return contextlib.nullcontext()


def _dft_matrices():
    f = np.concatenate([np.arange(0, C, 2), np.arange(1, C, 2)])
    zeta = 2 * np.pi * (f + 0.5) / (4 * C)

    def fwd(n):
        ang = zeta[:, None] * n[None, :]
        m = np.stack([np.cos(ang), -np.sin(ang)], 0)
        return m.reshape(2, NT, 8, C).transpose(1, 0, 2, 3).reshape(2 * C, C)

    def inv(n):
        ang = n[:, None] * zeta[None, :]
        return np.stack([np.cos(ang), -np.sin(ang)], -1).reshape(C, 2 * C) / (2 * C)

    def words(m):
        b = m.astype(np.float32).astype(bf16).view(np.uint16).astype(np.uint32)
        return b[0::2] | (b[1::2] << 16)

    j = np.arange(C)
    even = (j // 2) * 2 + (j % 2) * C
    return (words(np.concatenate([fwd(even), fwd(even + 1)], 0)),
            words(np.concatenate([inv(2 * j), inv(2 * j + 1)], 0)))


def _spec_row(filt, block, tile=0, part=0):
    return filt * KO + block * BS + (2 * tile + part) * 8


def _unpack(w, i):
    return pltpu.unpack_elementwise(w, index=i, packed_dtype=bf16, unpacked_dtype=f32)


def _pack(a, b):
    return pltpu.bitcast(pltpu.pack_elementwise([a, b], packed_dtype=bf16), u32)


def _as_bf16(w):
    return pltpu.bitcast(w, bf16)


def _dot(a, b):
    return jnp.dot(a, b, preferred_element_type=f32)


def _layernorm(x):
    xc = x - jnp.sum(x, axis=-1, keepdims=True) * (1.0 / D)
    var = jnp.sum(xc * xc, axis=-1, keepdims=True) * (1.0 / D)
    return xc * lax.rsqrt(var + EPS)


def _strassen_lhs(a11, a12, a21, a22):
    return [a11 + a22, a21 + a22, a11, a22, a11 + a12, a21 - a11, a12 - a22]


def _strassen_rhs(b11, b12, b21, b22):
    return [b11 + b22, b12 - b22, b21 - b11, b11 + b12, b21 + b22]


def _strassen(lhs, sums, b11, b22):
    rhs = [sums(0), b11, sums(1), sums(2), b22, sums(3), sums(4)]
    m = [_dot(a, _as_bf16(b)) for a, b in zip(lhs, rhs)]
    return (jnp.concatenate([m[0] + m[3] - m[4] + m[6], m[1] + m[3]], axis=0),
            jnp.concatenate([m[2] + m[4], m[0] - m[1] + m[2] + m[5]], axis=0))


def _swiglu(gate, up):
    half = 0.5 * gate
    return (half * jnp.tanh(half) + half) * up


def _run_mixed(main, side):
    total, done, k = sum(w for w, _ in main), 0, 0
    for w, f in main:
        f()
        done += w
        while k < len(side) and (k + 0.5) * total <= done * len(side):
            side[k]()
            k += 1
    for f in side[k:]:
        f()


def _kernel(q_hbm, k_hbm, v_hbm, shk_hbm, ssm_hbm, d_hbm, w1_hbm, w3_hbm, w2_hbm, c_hbm, wm_hbm,
            fwd_hbm, inv_hbm, o_hbm,
            shk, dvec, cvec, fwd, inv, qb, kb, vb, sb, w1, w3, w2, wm,
            spec, zlast, kf, zb, yb, cpar, zero, par, x1b, h2b, hs, he, up_sums, down_sums, ob, sems):
    k32, v32, s32, wm32, w132, w332, w232 = (
        a.bitcast(u32) for a in (k_hbm, v_hbm, ssm_hbm, wm_hbm, w1_hbm, w3_hbm, w2_hbm))

    def conv_inputs(l, t0, n):
        cols = pl.ds(l * 128, 128)
        return [(s32.at[pl.ds(l * H, H), pl.ds(t0, n)], sb.at[l, :, pl.ds(t0, n)]),
                (k32.at[pl.ds(t0 // 2, n // 2), cols], kb.at[l, pl.ds(8 + t0 // 2, n // 2)]),
                (v32.at[pl.ds(t0 // 2, n // 2), cols], vb.at[l, pl.ds(t0 // 2, n // 2)])]

    def same(src, dst, *idx):
        return src.at[idx], dst.at[idx]

    mod_cols = lambda c0, n: same(wm32, wm, slice(None), pl.ds(c0, n))
    up_cols = lambda g: [same(w132, w1, slice(None), pl.ds(g * TF, TF)),
                         same(w332, w3, slice(None), pl.ds(g * TF, TF))]
    down_rows = lambda g: same(w232, w2, pl.ds(g * TF // 2, TF // 2))
    q_rows = lambda r0, n: same(q_hbm, qb, pl.ds(r0, n))
    groups = {
        'params': [(shk_hbm, shk), (d_hbm, dvec), (c_hbm, cvec)],
        'first': [(fwd_hbm, fwd)] + conv_inputs(0, 0, S // 2),
        0: conv_inputs(0, S // 2, S // 2),
        1: conv_inputs(1, 0, S),
        'inv': [(inv_hbm, inv)],
        **{l: conv_inputs(l, 0, S) for l in range(2, NL)},
        'mod': [mod_cols(0, 5 * D), q_rows(0, R)],
        'ffn0': [same(w132, w1, slice(None), pl.ds(0, 2 * TF)), up_cols(0)[1]],
        'ffn1': up_cols(1)[1:] + [down_rows(0)] + up_cols(2)[:1],
        'ffn2': [q_rows(R, R)] + up_cols(2)[1:] + [down_rows(1)],
        'ffn3': [mod_cols(5 * D, D), down_rows(2)],
        'q': [q_rows(2 * R, 2 * R)],
        'q_late': [q_rows(4 * R, S - 4 * R)],
    }
    named = [g for g in groups if isinstance(g, str)]
    sem_of = lambda g: sems.at[NL + named.index(g) if isinstance(g, str) else g]
    out_sem = sems.at[NL + len(named)]

    def wait(g, pairs=None):
        with _scope('wait_' + (g if isinstance(g, str) else 'slab')):
            for src, dst in (groups[g] if pairs is None else pairs):
                pltpu.make_async_copy(src, dst, sem_of(g)).wait()

    def out_copy(r0, cols=slice(None)):
        return pltpu.make_async_copy(*same(ob, o_hbm, pl.ds(r0, R), cols), out_sem)

    for g, pairs in groups.items():
        for src, dst in pairs:
            pltpu.make_async_copy(src, dst, sem_of(g)).start()

    wait('params')
    taps = shk[...].astype(f32)
    skip = dvec[...].astype(f32).reshape(1, D)
    for l in range(NL):
        kb[l, 0:8, :] = jnp.zeros((8, 128), u32)
        for j in range(KS):
            cpar[l, j] = jnp.broadcast_to(taps[j:j + 1, l * 128:(l + 1) * 128], (8, 128))
        cpar[l, KS] = jnp.broadcast_to(skip[:, l * 128:(l + 1) * 128], (8, 128))
    zero[0] = 0
    z0 = pl.multiple_of(zero[0] * 1024, 1024)

    def forward_pieces(l, buf):
        param = lambda j, rows: jnp.broadcast_to(cpar[l, j, 0:1, :], (rows, 128))
        mat = lambda i: _as_bf16(fwd[i * C:(i + 1) * C, :])

        def butterfly(filt, j, even, odd):
            r = _spec_row(filt, j)
            spec[buf][r:r + 2 * C, :] = even + odd
            spec[buf][r + 2 * C:r + 4 * C, :] = even - odd

        def signal(j):
            def f():
                kw = kb[l, j * C:j * C + C + 8, :]
                ke, ko = _unpack(kw, 0), _unpack(kw, 1)
                kf[j][0] = ke
                kf[j][1] = ko
                ke1, ko1, ko2 = kf[j][0, 7:7 + C, :], kf[j][1, 7:7 + C, :], kf[j][1, 6:6 + C, :]
                ke, ko = ke[8:], ko[8:]
                t0, t1, t2, t3 = (param(t, C) for t in range(KS))
                vw = vb[l, j * C:(j + 1) * C, :]
                xe = (t0 * ke + t1 * ko1 + t2 * ke1 + t3 * ko2) * _unpack(vw, 0)
                xo = (t0 * ko + t1 * ke + t2 * ko1 + t3 * ke1) * _unpack(vw, 1)
                butterfly(0, j, _dot(mat(0), _as_bf16(_pack(xe[:H], xe[H:]))),
                          _dot(mat(1), _as_bf16(_pack(xo[:H], xo[H:]))))
            return f

        def long_filter(j):
            def f():
                lo = sb[l, :, 2 * j * C:(2 * j + 1) * C]
                hi = sb[l, :, (2 * j + 1) * C:(2 * j + 2) * C]
                even_lane = lax.broadcasted_iota(jnp.int32, lo.shape, 1) % 2 == 0
                te = jnp.where(even_lane, lo, pltpu.roll(hi, 1, 1))
                to = jnp.where(even_lane, pltpu.roll(lo, C - 1, 1), hi)
                dims = (((1,), (1,)), ((), ()))
                pe = lax.dot_general(mat(0), _as_bf16(te), dims, preferred_element_type=f32)
                po = lax.dot_general(mat(1), _as_bf16(to), dims, preferred_element_type=f32)
                if j == 0:
                    real = lax.broadcasted_iota(jnp.int32, pe.shape, 0) % 16 < 8
                    pe = pe + jnp.where(real, param(KS, 2 * C), 0.0)
                butterfly(1, j, pe, po)
            return f
        return [piece(j) for j in range(NBLK) for piece in (signal, long_filter)]

    def product_pieces(buf):
        load = lambda filt, j, tile: [
            spec[buf][pl.ds(z0 + _spec_row(filt, j, tile, c), 8), :] for c in range(2)]

        def piece(p, t):
            def plus_tail(z, prev):
                if t < NT // 2:
                    return [z[0] - prev[1], z[1] + prev[0]]
                return [z[0] + prev[1], z[1] - prev[0]]

            def f():
                res = []
                for tile in (t, NT + t):
                    acc, xs = [None, None], {}
                    for m in range(2 * p + 2):
                        kr, ki = load(1, m, tile)
                        for i in range(2):
                            j = 2 * p + i - m
                            if j < 0:
                                continue
                            if j not in xs:
                                xs[j] = load(0, j, tile)
                            xr, xi = xs[j]
                            term = [kr * xr - ki * xi, kr * xi + ki * xr]
                            acc[i] = term if acc[i] is None else [a + b for a, b in zip(acc[i], term)]
                    row = tile * 16
                    first = acc[0]
                    if p > 0:
                        first = plus_tail(first, [zlast[p - 1][pl.ds(z0 + row + 8 * c, 8), :] for c in range(2)])
                    if 2 * p + 2 < NBLK:
                        for c in range(2):
                            zlast[p][row + 8 * c:row + 8 * c + 8, :] = acc[1][c]
                    res.append([first, plus_tail(acc[1], acc[0])])
                for i in range(2):
                    (ar, ai), (br, bi) = res[0][i], res[1][i]
                    zb[2 * p + i][0, 8 * t:8 * t + 8, :] = _pack(ar + br, ai + bi)
                    zb[2 * p + i][1, 8 * t:8 * t + 8, :] = _pack(ar - br, ai - bi)
            return f
        return [(4 * p + 5, piece(p, t)) for p in range(NBLK // 2) for t in range(NT)]

    def inverse(l, j):
        ye, yo = (_dot(_as_bf16(inv[i * H:(i + 1) * H, :]), _as_bf16(zb[j][i, pl.ds(z0, C), :]))
                  for i in range(2))
        yb[l, j * C:(j + 1) * C, :] = _pack(ye, yo)

    def conv_step(l, buf, early=0):
        products = product_pieces(buf)
        for _, f in products[:early]:
            f()
        if early:
            wait('inv')
        wait(l + 1, conv_inputs(l + 1, 0, S))
        for j in range(2 * (early // NT) - 2):
            inverse(l, j)
        ahead = forward_pieces(l + 1, 1 - buf)
        total, done, k = sum(w for w, _ in products[early:]), 0, 0
        for i, (w, f) in list(enumerate(products))[early:]:
            while k < len(ahead) and (k + 1) * total * DFT_SPAN <= done * (len(ahead) + 1):
                ahead[k]()
                k += 1
            f()
            done += w
            p, t = divmod(i, NT)
            if p > 0 and t in (NT // 4, 3 * NT // 4):
                inverse(l, 2 * p - 2 + (t > NT // 2))
        for f in ahead[k:]:
            f()
        inverse(l, NBLK - 2)
        inverse(l, NBLK - 1)

    ahead = forward_pieces(0, 0)
    wait('first')
    for f in ahead[:NBLK]:
        f()
    wait(0)
    for f in ahead[NBLK:]:
        f()
    conv_step(0, 0, early=3 * NT)
    for l in range(1, NL - 1):
        conv_step(l, l % 2)

    cond = cvec[...].astype(f32)
    cond = jnp.broadcast_to(cond * jax.nn.sigmoid(cond), (16, D)).astype(bf16)
    mod = lambda j: _dot(cond, _as_bf16(wm[:, j * D:(j + 1) * D]))[0:8]
    row = lambda j, rows, cols=slice(None): par[j, 0:1, cols]

    words = lambda x: pltpu.bitcast(x.astype(bf16), u32)

    def chunk(s):
        if isinstance(s, int):
            return s % 2, s * R
        return lax.rem(s, 2), pl.multiple_of(s * R, R)

    def norm_pieces(s):
        slot, _ = chunk(s)
        n = LR // 2

        def rows(ref_at, scale, i):
            starts = [s * (R // scale) + (half * RH + i * n) // scale for half in range(2)]
            if not isinstance(s, int):
                starts = [pl.multiple_of(r, n // scale) for r in starts]
            return jnp.concatenate([ref_at(pl.ds(r, n // scale)) for r in starts], axis=0)

        def piece(i):
            def f():
                x = rows(lambda r: qb[r, :], 1, i).astype(f32)
                y = jnp.concatenate(
                    [_as_bf16(rows(lambda r: yb[l, r, :], 2, i)).astype(f32) for l in range(NL)], axis=1)
                x = x + (_layernorm(x) * row(0, LR) + row(1, LR)) * y
                h = _layernorm(x) * row(2, LR) + row(3, LR)
                at = [slice((half * RH + i * n) // 2, (half * RH + (i + 1) * n) // 2) for half in range(2)]
                for half in range(2):
                    r = half * RH + i * n
                    x1b[slot, r:r + n, :] = x[half * n:(half + 1) * n]
                top, bottom = h[:n], h[n:]
                if isinstance(s, int) and s == 0:
                    h2b[at[0], :], h2b[at[1], :] = words(top), words(bottom)
                    return
                he[slot, at[0], :], he[slot, at[1], :] = words(top[:, 2 * DH:]), words(bottom[:, 2 * DH:])
                sums = _strassen_lhs(top[:, :DH], top[:, DH:2 * DH], bottom[:, :DH], bottom[:, DH:2 * DH])
                for k, v in enumerate(sums):
                    hs[slot, k, at[0], :] = words(v)
            return f
        return [piece(i) for i in range(R // LR)]

    def weight_sum_pieces(w, nk, nn, out):
        def piece(r):
            def f():
                quads = [w[k0 + r:k0 + r + 8, n0:n0 + nn] for k0 in (0, nk // 2) for n0 in (0, nn)]
                even, odd = (_strassen_rhs(*[_unpack(q, i) for q in quads]) for i in range(2))
                for k in range(5):
                    out[k, r:r + 8, :] = _pack(even[k], odd[k])
            return f
        return [piece(r) for r in range(0, nk // 2, 8)]

    def residual(s, y, c0):
        slot, r0 = chunk(s)
        cols = slice(c0, c0 + y.shape[1])
        ob[pl.ds(r0, R), cols] = (x1b[slot, :, cols] + row(4, R, cols) * y).astype(bf16)

    def first_ffn_pieces():
        st = {}

        def gate(g):
            def f():
                st['gate'] = _dot(_as_bf16(h2b[...]), _as_bf16(w1[:, g * TF:(g + 1) * TF]))
            return f

        def up(g):
            def f():
                u = _dot(_as_bf16(h2b[...]), _as_bf16(w3[:, g * TF:(g + 1) * TF]))
                st[g] = _swiglu(st['gate'], u).astype(bf16)
            return f

        def down(g, c0, c1):
            def f():
                p = _dot(st[g], _as_bf16(w2[g * TF // 2:(g + 1) * TF // 2, c0:c1]))
                if g + 1 < NG:
                    st['acc'] = p if g == 0 else st['acc'] + p
                else:
                    residual(0, st['acc'][:, c0:c1] + p, c0)
            return f
        ups = [[(D, gate(g)), (D, up(g))] for g in range(NG)]
        downs = [[(D, down(g, 0, D))] for g in range(NG - 1)]
        downs.append([(c1 - c0, down(NG - 1, c0, c1)) for c0, c1 in zip(OUT_COLS[:-1], OUT_COLS[1:])])
        return ups[0] + ups[1] + downs[0] + ups[2] + downs[1] + downs[2]

    def ffn_pieces(s):
        slot, r0 = chunk(s)
        last = isinstance(s, int) and s == NS - 1
        lhs, hidden = [], [[], []]

        def up(n):
            left, right = slice(n, n + 128), slice(FH + n, FH + n + 128)

            def project(i, w):
                a = [_as_bf16(hs[slot, k]) for k in range(7)]
                both = _strassen(a, lambda k: up_sums[i, k, :, left],
                                 w[0:DH // 2, left], w[DH // 2:DH, right])
                rest = _as_bf16(he[slot])
                return [p + _dot(rest, _as_bf16(w[DH:, cols])) for p, cols in zip(both, (left, right))]

            def f():
                a1, a2 = (_swiglu(g, u) for g, u in zip(project(0, w1), project(1, w3)))
                lhs.append([v.astype(bf16) for v in _strassen_lhs(a1[:RH], a2[:RH], a1[RH:], a2[RH:])])
                hidden[0].append(a1.astype(bf16))
                hidden[1].append(a2.astype(bf16))
            return f

        def down(n):
            def f():
                a = [jnp.concatenate([t[k] for t in lhs], axis=1) for k in range(7)]
                y1, y2 = _strassen(a, lambda k: down_sums[k, :, n:n + 128],
                                   w2[0:FH // 2, n:n + 128], w2[FH // 2:, DH + n:DH + n + 128])
                residual(s, y1, n)
                residual(s, y2, DH + n)
                if last and n + 128 == DH:
                    out_copy(r0, pl.ds(0, 2 * DH)).start()
            return f

        def down_rest():
            a = jnp.concatenate(hidden[0] + hidden[1], axis=1)
            residual(s, _dot(a, _as_bf16(w2[:, 2 * DH:])), 2 * DH)
            if last:
                out_copy(r0, pl.ds(2 * DH, D - 2 * DH)).start()
        return ([(18, up(n)) for n in range(0, FH, 128)] + [(21, down(n)) for n in range(0, DH, 128)]
                + [(12, down_rest)])

    products = product_pieces(0)
    for _, f in products[:5 * NT // 2]:
        f()
    wait('mod')
    scale_a, gate_a, shift_a, scale_b, shift_b = (mod(j) for j in (1, 2, 0, 4, 3))
    par[0] = gate_a * (1.0 + scale_a)
    par[1] = gate_a * shift_a
    par[2] = 1.0 + scale_b
    par[3] = shift_b
    for _, f in products[5 * NT // 2:]:
        f()
    inverse(NL - 1, 0)
    inverse(NL - 1, 1)
    _run_mixed([(1, f) for f in norm_pieces(0)],
               [functools.partial(inverse, NL - 1, j) for j in range(2, NBLK)])

    ffn, norms = first_ffn_pieces(), norm_pieces(1)
    sums = weight_sum_pieces(w1, DH, FH, up_sums.at[0]) + weight_sum_pieces(w3, DH, FH, up_sums.at[1])
    n = 3 * len(norms) // 4
    wait('ffn0')
    _run_mixed(ffn[:3], [])
    wait('ffn1')
    _run_mixed(ffn[3:6], sums[:len(sums) // 2])
    wait('ffn2')
    _run_mixed(ffn[6:8], norms[:n] + sums[len(sums) // 2:])
    wait('ffn3')
    par[4] = mod(5)
    _run_mixed(ffn[8:], norms[n:] + weight_sum_pieces(w2, FH, DH, down_sums))
    out_copy(0).start()
    wait('q')

    def ffn_body(s, carry):
        pl.when(s == 3)(lambda: wait('q_late'))
        pieces = ffn_pieces(s)
        n = int(len(pieces) * PRE_SPAN)
        _run_mixed(pieces[:n], norm_pieces(s + 1))
        _run_mixed(pieces[n:], [])
        out_copy(pl.multiple_of(s * R, R)).start()
        return carry
    with _scope('ffn_loop'):
        lax.fori_loop(1, NS - 1, ffn_body, 0)
    _run_mixed(ffn_pieces(NS - 1), [])

    with _scope('wait_out'):
        for s in range(NS - 1):
            out_copy(s * R).wait()
        out_copy(S - R, pl.ds(0, 2 * DH)).wait()
        out_copy(S - R, pl.ds(2 * DH, D - 2 * DH)).wait()


@jax.jit
def pallas_adaLN_cond__ssm_conv_h3__glu_gated_swiglu__prompt_kernel(
    A_q: jax.Array,
    A_k: jax.Array,
    A_v: jax.Array,
    A_shift_k: jax.Array,
    A_ssm_k: jax.Array,
    A_ssm_D: jax.Array,
    B_x: jax.Array,
    B_w1: jax.Array,
    B_w3: jax.Array,
    B_w2: jax.Array,
    c: jax.Array,
    w_mod: jax.Array,
):
    del B_x
    fwd, inv = _dft_matrices()
    hbm = pl.BlockSpec(memory_space=pl.ANY)
    vmem = pltpu.VMEM
    out = pl.pallas_call(
        _kernel,
        in_specs=[hbm] * 13,
        out_specs=hbm,
        out_shape=jax.ShapeDtypeStruct((S, D), bf16),
        scratch_shapes=[
            vmem((KS, D), bf16), vmem((D,), bf16), vmem((1, D), bf16),
            vmem(fwd.shape, u32), vmem(inv.shape, u32),
            vmem((S, D), bf16),
            vmem((NL, S // 2 + 8, 128), u32), vmem((NL, S // 2, 128), u32),
            vmem((NL, H, S), u32),
            vmem((D // 2, F), u32), vmem((D // 2, F), u32), vmem((F // 2, D), u32),
            vmem((D // 2, 6 * D), u32),
            [vmem((2 * KO + 512, 128), f32) for _ in range(2)],
            [vmem((4 * C, 128), f32) for _ in range(NBLK // 2 - 1)],
            [vmem((2, C + 8, 128), f32) for _ in range(NBLK)],
            [vmem((2, C, 128), u32) for _ in range(NBLK)],
            vmem((NL, S // 2, 128), u32),
            vmem((NL, KS + 1, 8, 128), f32), pltpu.SMEM((1,), jnp.int32), vmem((5, 8, D), f32),
            vmem((2, R, D), f32), vmem((R // 2, D), u32),
            vmem((2, 7, RH // 2, DH), u32), vmem((2, R // 2, D - 2 * DH), u32),
            vmem((2, 5, DH // 2, FH), u32), vmem((5, FH // 2, DH), u32),
            vmem((S, D), bf16),
            pltpu.SemaphoreType.DMA((NL + 11,)),
        ],
        compiler_params=pltpu.CompilerParams(vmem_limit_bytes=100 * 2**20),
    )(A_q.reshape(S, D), A_k.reshape(S, D), A_v.reshape(S, D), A_shift_k.T, A_ssm_k, A_ssm_D,
      B_w1, B_w3, B_w2, c, w_mod, fwd, inv)
    return out.reshape(1, S, D)
```

```python
import contextlib
import functools

import jax
import jax.numpy as jnp
import numpy as np
from jax import lax
from jax.experimental import pallas as pl
from jax.experimental.pallas import tpu as pltpu

S, D, F = 2048, 640, 1536
KS = 4
EPS = 1e-5
C = 128
H = C // 2
NBLK = S // (2 * C)
NL = D // 128
NT = C // 8
R = 256
LR = 32
TF = 512
PW = 256
OUT_COLS = (0, 256, 512, D)
NS = S // R
NG = F // TF
RH, DH, FH = R // 2, 256, F // 2
BS = (4 * NT + 4) * 8
KO = (NBLK * BS + 511) // 512 * 512 + 16
DFT_SPAN = 0.9
PRE_SPAN = 0.9

f32, bf16, u32 = jnp.float32, jnp.bfloat16, jnp.uint32


def _scope(name):
    del name
    return contextlib.nullcontext()


def _dft_matrices():
    f = np.concatenate([np.arange(0, C, 2), np.arange(1, C, 2)])
    zeta = 2 * np.pi * (f + 0.5) / (4 * C)

    def fwd(n):
        ang = zeta[:, None] * n[None, :]
        m = np.stack([np.cos(ang), -np.sin(ang)], 0)
        return m.reshape(2, NT, 8, C).transpose(1, 0, 2, 3).reshape(2 * C, C)

    def inv(n):
        ang = n[:, None] * zeta[None, :]
        return np.stack([np.cos(ang), -np.sin(ang)], -1).reshape(C, 2 * C) / (2 * C)

    def words(m):
        b = m.astype(np.float32).astype(bf16).view(np.uint16).astype(np.uint32)
        return b[0::2] | (b[1::2] << 16)

    j = np.arange(C)
    even = (j // 2) * 2 + (j % 2) * C
    return (words(np.concatenate([fwd(even), fwd(even + 1)], 0)),
            words(np.concatenate([inv(2 * j), inv(2 * j + 1)], 0)))


def _spec_row(filt, block, tile=0, part=0):
    return filt * KO + block * BS + (2 * tile + part) * 8


def _unpack(w, i):
    return pltpu.unpack_elementwise(w, index=i, packed_dtype=bf16, unpacked_dtype=f32)


def _pack(a, b):
    return pltpu.bitcast(pltpu.pack_elementwise([a, b], packed_dtype=bf16), u32)


def _as_bf16(w):
    return pltpu.bitcast(w, bf16)


def _dot(a, b):
    return jnp.dot(a, b, preferred_element_type=f32)


def _layernorm(x):
    xc = x - jnp.sum(x, axis=-1, keepdims=True) * (1.0 / D)
    var = jnp.sum(xc * xc, axis=-1, keepdims=True) * (1.0 / D)
    return xc * lax.rsqrt(var + EPS)


def _strassen_lhs(a11, a12, a21, a22):
    return [a11 + a22, a21 + a22, a11, a22, a11 + a12, a21 - a11, a12 - a22]


def _strassen_rhs(b11, b12, b21, b22):
    return [b11 + b22, b12 - b22, b21 - b11, b11 + b12, b21 + b22]


def _strassen(lhs, sums, b11, b22):
    rhs = [sums(0), b11, sums(1), sums(2), b22, sums(3), sums(4)]
    m = [_dot(a, _as_bf16(b)) for a, b in zip(lhs, rhs)]
    return (jnp.concatenate([m[0] + m[3] - m[4] + m[6], m[1] + m[3]], axis=0),
            jnp.concatenate([m[2] + m[4], m[0] - m[1] + m[2] + m[5]], axis=0))


def _swiglu(gate, up):
    half = 0.5 * gate
    return (half * jnp.tanh(half) + half) * up


def _run_mixed(main, side):
    total, done, k = sum(w for w, _ in main), 0, 0
    for w, f in main:
        f()
        done += w
        while k < len(side) and (k + 0.5) * total <= done * len(side):
            side[k]()
            k += 1
    for f in side[k:]:
        f()


def _kernel(q_hbm, k_hbm, v_hbm, shk_hbm, ssm_hbm, d_hbm, w1_hbm, w3_hbm, w2_hbm, c_hbm, wm_hbm,
            fwd_hbm, inv_hbm, o_hbm,
            shk, dvec, cvec, fwd, inv, qb, kb, vb, sb, w1, w3, w2, wm,
            spec, zlast, kf, zb, yb, cpar, zero, par, x1b, h2b, hs, he, up_sums, down_sums, ob, sems):
    k32, v32, s32, wm32, w132, w332, w232 = (
        a.bitcast(u32) for a in (k_hbm, v_hbm, ssm_hbm, wm_hbm, w1_hbm, w3_hbm, w2_hbm))

    def conv_inputs(l, t0, n):
        cols = pl.ds(l * 128, 128)
        return [(s32.at[pl.ds(l * H, H), pl.ds(t0, n)], sb.at[l, :, pl.ds(t0, n)]),
                (k32.at[pl.ds(t0 // 2, n // 2), cols], kb.at[l, pl.ds(8 + t0 // 2, n // 2)]),
                (v32.at[pl.ds(t0 // 2, n // 2), cols], vb.at[l, pl.ds(t0 // 2, n // 2)])]

    def same(src, dst, *idx):
        return src.at[idx], dst.at[idx]

    mod_cols = lambda c0, n: same(wm32, wm, slice(None), pl.ds(c0, n))
    up_cols = lambda g: [same(w132, w1, slice(None), pl.ds(g * TF, TF)),
                         same(w332, w3, slice(None), pl.ds(g * TF, TF))]
    down_rows = lambda g: same(w232, w2, pl.ds(g * TF // 2, TF // 2))
    q_rows = lambda r0, n: same(q_hbm, qb, pl.ds(r0, n))
    groups = {
        'params': [(shk_hbm, shk), (d_hbm, dvec), (c_hbm, cvec)],
        'first': [(fwd_hbm, fwd)] + conv_inputs(0, 0, S // 2),
        0: conv_inputs(0, S // 2, S // 2),
        1: conv_inputs(1, 0, S),
        'inv': [(inv_hbm, inv)],
        **{l: conv_inputs(l, 0, S) for l in range(2, NL)},
        'mod': [mod_cols(0, 5 * D), q_rows(0, R)],
        'ffn0': [same(w132, w1, slice(None), pl.ds(0, 2 * TF)), up_cols(0)[1]],
        'ffn1': up_cols(1)[1:] + [down_rows(0)] + up_cols(2)[:1],
        'ffn2': [q_rows(R, R)] + up_cols(2)[1:] + [down_rows(1)],
        'ffn3': [mod_cols(5 * D, D), down_rows(2)],
        'q': [q_rows(2 * R, 2 * R)],
        'q_late': [q_rows(4 * R, S - 4 * R)],
    }
    named = [g for g in groups if isinstance(g, str)]
    sem_of = lambda g: sems.at[NL + named.index(g) if isinstance(g, str) else g]
    out_sem = sems.at[NL + len(named)]

    def wait(g, pairs=None):
        with _scope('wait_' + (g if isinstance(g, str) else 'slab')):
            for src, dst in (groups[g] if pairs is None else pairs):
                pltpu.make_async_copy(src, dst, sem_of(g)).wait()

    def out_copy(r0, cols=slice(None)):
        return pltpu.make_async_copy(*same(ob, o_hbm, pl.ds(r0, R), cols), out_sem)

    for g, pairs in groups.items():
        for src, dst in pairs:
            pltpu.make_async_copy(src, dst, sem_of(g)).start()

    wait('params')
    taps = shk[...].astype(f32)
    skip = dvec[...].astype(f32).reshape(1, D)
    for l in range(NL):
        kb[l, 0:8, :] = jnp.zeros((8, 128), u32)
        for j in range(KS):
            cpar[l, j] = jnp.broadcast_to(taps[j:j + 1, l * 128:(l + 1) * 128], (8, 128))
        cpar[l, KS] = jnp.broadcast_to(skip[:, l * 128:(l + 1) * 128], (8, 128))
    zero[0] = 0
    z0 = pl.multiple_of(zero[0] * 1024, 1024)

    def forward_pieces(l, buf):
        param = lambda j, rows: jnp.broadcast_to(cpar[l, j, 0:1, :], (rows, 128))
        mat = lambda i: _as_bf16(fwd[i * C:(i + 1) * C, :])

        def butterfly(filt, j, even, odd):
            r = _spec_row(filt, j)
            spec[buf][r:r + 2 * C, :] = even + odd
            spec[buf][r + 2 * C:r + 4 * C, :] = even - odd

        def signal(j):
            def f():
                kw = kb[l, j * C:j * C + C + 8, :]
                ke, ko = _unpack(kw, 0), _unpack(kw, 1)
                kf[j][0] = ke
                kf[j][1] = ko
                ke1, ko1, ko2 = kf[j][0, 7:7 + C, :], kf[j][1, 7:7 + C, :], kf[j][1, 6:6 + C, :]
                ke, ko = ke[8:], ko[8:]
                t0, t1, t2, t3 = (param(t, C) for t in range(KS))
                vw = vb[l, j * C:(j + 1) * C, :]
                xe = (t0 * ke + t1 * ko1 + t2 * ke1 + t3 * ko2) * _unpack(vw, 0)
                xo = (t0 * ko + t1 * ke + t2 * ko1 + t3 * ke1) * _unpack(vw, 1)
                butterfly(0, j, _dot(mat(0), _as_bf16(_pack(xe[:H], xe[H:]))),
                          _dot(mat(1), _as_bf16(_pack(xo[:H], xo[H:]))))
            return f

        def long_filter(j):
            def f():
                lo = sb[l, :, 2 * j * C:(2 * j + 1) * C]
                hi = sb[l, :, (2 * j + 1) * C:(2 * j + 2) * C]
                even_lane = lax.broadcasted_iota(jnp.int32, lo.shape, 1) % 2 == 0
                te = jnp.where(even_lane, lo, pltpu.roll(hi, 1, 1))
                to = jnp.where(even_lane, pltpu.roll(lo, C - 1, 1), hi)
                dims = (((1,), (1,)), ((), ()))
                pe = lax.dot_general(mat(0), _as_bf16(te), dims, preferred_element_type=f32)
                po = lax.dot_general(mat(1), _as_bf16(to), dims, preferred_element_type=f32)
                if j == 0:
                    real = lax.broadcasted_iota(jnp.int32, pe.shape, 0) % 16 < 8
                    pe = pe + jnp.where(real, param(KS, 2 * C), 0.0)
                butterfly(1, j, pe, po)
            return f
        return [piece(j) for j in range(NBLK) for piece in (signal, long_filter)]

    def product_pieces(buf):
        load = lambda filt, j, tile: [
            spec[buf][pl.ds(z0 + _spec_row(filt, j, tile, c), 8), :] for c in range(2)]

        def piece(p, t):
            def plus_tail(z, prev):
                if t < NT // 2:
                    return [z[0] - prev[1], z[1] + prev[0]]
                return [z[0] + prev[1], z[1] - prev[0]]

            def f():
                res = []
                for tile in (t, NT + t):
                    acc, xs = [None, None], {}
                    for m in range(2 * p + 2):
                        kr, ki = load(1, m, tile)
                        for i in range(2):
                            j = 2 * p + i - m
                            if j < 0:
                                continue
                            if j not in xs:
                                xs[j] = load(0, j, tile)
                            xr, xi = xs[j]
                            term = [kr * xr - ki * xi, kr * xi + ki * xr]
                            acc[i] = term if acc[i] is None else [a + b for a, b in zip(acc[i], term)]
                    row = tile * 16
                    first = acc[0]
                    if p > 0:
                        first = plus_tail(first, [zlast[p - 1][pl.ds(z0 + row + 8 * c, 8), :] for c in range(2)])
                    if 2 * p + 2 < NBLK:
                        for c in range(2):
                            zlast[p][row + 8 * c:row + 8 * c + 8, :] = acc[1][c]
                    res.append([first, plus_tail(acc[1], acc[0])])
                for i in range(2):
                    (ar, ai), (br, bi) = res[0][i], res[1][i]
                    zb[2 * p + i][0, 8 * t:8 * t + 8, :] = _pack(ar + br, ai + bi)
                    zb[2 * p + i][1, 8 * t:8 * t + 8, :] = _pack(ar - br, ai - bi)
            return f
        return [(4 * p + 5, piece(p, t)) for p in range(NBLK // 2) for t in range(NT)]

    def inverse(l, j):
        ye, yo = (_dot(_as_bf16(inv[i * H:(i + 1) * H, :]), _as_bf16(zb[j][i, pl.ds(z0, C), :]))
                  for i in range(2))
        yb[l, j * C:(j + 1) * C, :] = _pack(ye, yo)

    def conv_step(l, buf, early=0):
        products = product_pieces(buf)
        for _, f in products[:early]:
            f()
        if early:
            wait('inv')
        wait(l + 1, conv_inputs(l + 1, 0, S))
        for j in range(2 * (early // NT) - 2):
            inverse(l, j)
        ahead = forward_pieces(l + 1, 1 - buf)
        total, done, k = sum(w for w, _ in products[early:]), 0, 0
        for i, (w, f) in list(enumerate(products))[early:]:
            while k < len(ahead) and (k + 1) * total * DFT_SPAN <= done * (len(ahead) + 1):
                ahead[k]()
                k += 1
            f()
            done += w
            p, t = divmod(i, NT)
            if p > 0 and t in (NT // 4, 3 * NT // 4):
                inverse(l, 2 * p - 2 + (t > NT // 2))
        for f in ahead[k:]:
            f()
        inverse(l, NBLK - 2)
        inverse(l, NBLK - 1)

    ahead = forward_pieces(0, 0)
    wait('first')
    for f in ahead[:NBLK]:
        f()
    wait(0)
    for f in ahead[NBLK:]:
        f()
    conv_step(0, 0, early=3 * NT)
    for l in range(1, NL - 1):
        conv_step(l, l % 2)

    cond = cvec[...].astype(f32)
    cond = jnp.broadcast_to(cond * jax.nn.sigmoid(cond), (16, D)).astype(bf16)
    mod = lambda j: _dot(cond, _as_bf16(wm[:, j * D:(j + 1) * D]))[0:8]
    row = lambda j, rows, cols=slice(None): par[j, 0:1, cols]

    words = lambda x: pltpu.bitcast(x.astype(bf16), u32)

    def chunk(s):
        if isinstance(s, int):
            return s % 2, s * R
        return lax.rem(s, 2), pl.multiple_of(s * R, R)

    def norm_pieces(s):
        slot, _ = chunk(s)
        n = LR // 2

        def rows(ref_at, scale, i):
            starts = [s * (R // scale) + (half * RH + i * n) // scale for half in range(2)]
            if not isinstance(s, int):
                starts = [pl.multiple_of(r, n // scale) for r in starts]
            return jnp.concatenate([ref_at(pl.ds(r, n // scale)) for r in starts], axis=0)

        def piece(i):
            def f():
                x = rows(lambda r: qb[r, :], 1, i).astype(f32)
                y = jnp.concatenate(
                    [_as_bf16(rows(lambda r: yb[l, r, :], 2, i)).astype(f32) for l in range(NL)], axis=1)
                x = x + (_layernorm(x) * row(0, LR) + row(1, LR)) * y
                h = _layernorm(x) * row(2, LR) + row(3, LR)
                at = [slice((half * RH + i * n) // 2, (half * RH + (i + 1) * n) // 2) for half in range(2)]
                for half in range(2):
                    r = half * RH + i * n
                    x1b[slot, r:r + n, :] = x[half * n:(half + 1) * n]
                top, bottom = h[:n], h[n:]
                if isinstance(s, int) and s == 0:
                    h2b[at[0], :], h2b[at[1], :] = words(top), words(bottom)
                    return
                he[slot, at[0], :], he[slot, at[1], :] = words(top[:, 2 * DH:]), words(bottom[:, 2 * DH:])
                sums = _strassen_lhs(top[:, :DH], top[:, DH:2 * DH], bottom[:, :DH], bottom[:, DH:2 * DH])
                for k, v in enumerate(sums):
                    hs[slot, k, at[0], :] = words(v)
            return f
        return [piece(i) for i in range(R // LR)]

    def weight_sum_pieces(w, nk, nn, out):
        def piece(r, c):
            def f():
                quads = [w[k0 + r:k0 + r + 8, n0 + c:n0 + c + 128] for k0 in (0, nk // 2) for n0 in (0, nn)]
                even, odd = (_strassen_rhs(*[_unpack(q, i) for q in quads]) for i in range(2))
                for k in range(5):
                    out[k, r:r + 8, c:c + 128] = _pack(even[k], odd[k])
            return f
        return [piece(r, c) for r in range(0, nk // 2, 8) for c in range(0, nn, 128)]

    def residual(s, y, c0):
        slot, r0 = chunk(s)
        cols = slice(c0, c0 + y.shape[1])
        ob[pl.ds(r0, R), cols] = (x1b[slot, :, cols] + row(4, R, cols) * y).astype(bf16)

    def first_ffn_pieces():
        st = {}

        def gate(c):
            def f():
                st['gate', c] = _dot(_as_bf16(h2b[...]), _as_bf16(w1[:, c:c + PW]))
            return f

        def up(c):
            def f():
                u = _dot(_as_bf16(h2b[...]), _as_bf16(w3[:, c:c + PW]))
                st[c] = _swiglu(st['gate', c], u).astype(bf16)
            return f

        def down(g, c0, c1):
            def f():
                a = jnp.concatenate([st[c] for c in range(g * TF, (g + 1) * TF, PW)], axis=1)
                p = _dot(a, _as_bf16(w2[g * TF // 2:(g + 1) * TF // 2, c0:c1]))
                st['acc', c0] = p if g == 0 else st['acc', c0] + p
                if g + 1 == NG:
                    residual(0, st['acc', c0], c0)
            return f
        cols = lambda g: range(g * TF, (g + 1) * TF, PW)
        return ([[(PW, gate(c)) for c in cols(g)] for g in range(NG)],
                [[(PW, up(c)) for c in cols(g)] for g in range(NG)],
                [[(c1 - c0, down(g, c0, c1)) for c0, c1 in zip(OUT_COLS[:-1], OUT_COLS[1:])] for g in range(NG)])

    def ffn_pieces(s):
        slot, r0 = chunk(s)
        last = isinstance(s, int) and s == NS - 1
        lhs, hidden = [], [[], []]

        def up(n):
            left, right = slice(n, n + 128), slice(FH + n, FH + n + 128)

            def project(i, w):
                a = [_as_bf16(hs[slot, k]) for k in range(7)]
                both = _strassen(a, lambda k: up_sums[i, k, :, left],
                                 w[0:DH // 2, left], w[DH // 2:DH, right])
                rest = _as_bf16(he[slot])
                return [p + _dot(rest, _as_bf16(w[DH:, cols])) for p, cols in zip(both, (left, right))]

            def f():
                a1, a2 = (_swiglu(g, u) for g, u in zip(project(0, w1), project(1, w3)))
                lhs.append([v.astype(bf16) for v in _strassen_lhs(a1[:RH], a2[:RH], a1[RH:], a2[RH:])])
                hidden[0].append(a1.astype(bf16))
                hidden[1].append(a2.astype(bf16))
            return f

        def down(n):
            def f():
                a = [jnp.concatenate([t[k] for t in lhs], axis=1) for k in range(7)]
                y1, y2 = _strassen(a, lambda k: down_sums[k, :, n:n + 128],
                                   w2[0:FH // 2, n:n + 128], w2[FH // 2:, DH + n:DH + n + 128])
                residual(s, y1, n)
                residual(s, y2, DH + n)
                if last and n + 128 == DH:
                    out_copy(r0, pl.ds(0, 2 * DH)).start()
            return f

        def down_rest():
            a = jnp.concatenate(hidden[0] + hidden[1], axis=1)
            residual(s, _dot(a, _as_bf16(w2[:, 2 * DH:])), 2 * DH)
            if last:
                out_copy(r0, pl.ds(2 * DH, D - 2 * DH)).start()
        ups, downs = [(18, up(n)) for n in range(0, FH, 128)], [(21, down(n)) for n in range(0, DH, 128)]
        if last:
            return ups + downs + [(12, down_rest)]
        return ups + [(12, down_rest)] + downs

    products = product_pieces(0)
    for _, f in products[:5 * NT // 2]:
        f()
    wait('mod')
    scale_a, gate_a, shift_a, scale_b, shift_b = (mod(j) for j in (1, 2, 0, 4, 3))
    par[0] = gate_a * (1.0 + scale_a)
    par[1] = gate_a * shift_a
    par[2] = 1.0 + scale_b
    par[3] = shift_b
    for _, f in products[5 * NT // 2:]:
        f()
    inverse(NL - 1, 0)
    inverse(NL - 1, 1)
    _run_mixed([(1, f) for f in norm_pieces(0)],
               [functools.partial(inverse, NL - 1, j) for j in range(2, NBLK)])

    gates, ups, downs = first_ffn_pieces()
    norms = norm_pieces(1)
    n = len(norms) // 2
    wait('ffn0')
    _run_mixed(gates[0] + ups[0] + gates[1], [])
    wait('ffn1')
    _run_mixed(ups[1] + downs[0] + gates[2], weight_sum_pieces(w1, DH, FH, up_sums.at[0]))
    wait('ffn2')
    _run_mixed(ups[2] + downs[1], weight_sum_pieces(w3, DH, FH, up_sums.at[1]) + norms[:n])
    wait('ffn3')
    par[4] = mod(5)
    _run_mixed(downs[2], weight_sum_pieces(w2, FH, DH, down_sums) + norms[n:])
    out_copy(0).start()
    wait('q')

    def ffn_body(s, carry):
        pl.when(s == 3)(lambda: wait('q_late'))
        pieces = ffn_pieces(s)
        n = int(len(pieces) * PRE_SPAN)
        _run_mixed(pieces[:n], norm_pieces(s + 1))
        _run_mixed(pieces[n:], [])
        out_copy(pl.multiple_of(s * R, R)).start()
        return carry
    with _scope('ffn_loop'):
        lax.fori_loop(1, NS - 1, ffn_body, 0)
    _run_mixed(ffn_pieces(NS - 1), [])

    with _scope('wait_out'):
        for s in range(NS - 1):
            out_copy(s * R).wait()
        out_copy(S - R, pl.ds(0, 2 * DH)).wait()
        out_copy(S - R, pl.ds(2 * DH, D - 2 * DH)).wait()


@jax.jit
def pallas_adaLN_cond__ssm_conv_h3__glu_gated_swiglu__prompt_kernel(
    A_q: jax.Array,
    A_k: jax.Array,
    A_v: jax.Array,
    A_shift_k: jax.Array,
    A_ssm_k: jax.Array,
    A_ssm_D: jax.Array,
    B_x: jax.Array,
    B_w1: jax.Array,
    B_w3: jax.Array,
    B_w2: jax.Array,
    c: jax.Array,
    w_mod: jax.Array,
):
    del B_x
    fwd, inv = _dft_matrices()
    hbm = pl.BlockSpec(memory_space=pl.ANY)
    vmem = pltpu.VMEM
    out = pl.pallas_call(
        _kernel,
        in_specs=[hbm] * 13,
        out_specs=hbm,
        out_shape=jax.ShapeDtypeStruct((S, D), bf16),
        scratch_shapes=[
            vmem((KS, D), bf16), vmem((D,), bf16), vmem((1, D), bf16),
            vmem(fwd.shape, u32), vmem(inv.shape, u32),
            vmem((S, D), bf16),
            vmem((NL, S // 2 + 8, 128), u32), vmem((NL, S // 2, 128), u32),
            vmem((NL, H, S), u32),
            vmem((D // 2, F), u32), vmem((D // 2, F), u32), vmem((F // 2, D), u32),
            vmem((D // 2, 6 * D), u32),
            [vmem((2 * KO + 512, 128), f32) for _ in range(2)],
            [vmem((4 * C, 128), f32) for _ in range(NBLK // 2 - 1)],
            [vmem((2, C + 8, 128), f32) for _ in range(NBLK)],
            [vmem((2, C, 128), u32) for _ in range(NBLK)],
            vmem((NL, S // 2, 128), u32),
            vmem((NL, KS + 1, 8, 128), f32), pltpu.SMEM((1,), jnp.int32), vmem((5, 8, D), f32),
            vmem((2, R, D), f32), vmem((R // 2, D), u32),
            vmem((2, 7, RH // 2, DH), u32), vmem((2, R // 2, D - 2 * DH), u32),
            vmem((2, 5, DH // 2, FH), u32), vmem((5, FH // 2, DH), u32),
            vmem((S, D), bf16),
            pltpu.SemaphoreType.DMA((NL + 11,)),
        ],
        compiler_params=pltpu.CompilerParams(vmem_limit_bytes=100 * 2**20),
    )(A_q.reshape(S, D), A_k.reshape(S, D), A_v.reshape(S, D), A_shift_k.T, A_ssm_k, A_ssm_D,
      B_w1, B_w3, B_w2, c, w_mod, fwd, inv)
    return out.reshape(1, S, D)
```

```python
import contextlib
import functools

import jax
import jax.numpy as jnp
import numpy as np
from jax import lax
from jax.experimental import pallas as pl
from jax.experimental.pallas import tpu as pltpu

S, D, F = 2048, 640, 1536
KS = 4
EPS = 1e-5
C = 128
H = C // 2
NBLK = S // (2 * C)
NL = D // 128
NT = C // 8
R = 256
LR = 32
TF = 512
PW = 256
OUT_COLS = (0, 256, 512, D)
NS = S // R
NG = F // TF
RH, DH, FH = R // 2, 256, F // 2
RQ, DQ, FQ = RH // 2, DH // 2, FH // 2
BS = (4 * NT + 4) * 8
KO = (NBLK * BS + 511) // 512 * 512 + 16
DFT_SPAN = 0.9
PRE_PIECES = 5

f32, bf16, u32 = jnp.float32, jnp.bfloat16, jnp.uint32


def _scope(name):
    del name
    return contextlib.nullcontext()


def _dft_matrices():
    f = np.concatenate([np.arange(0, C, 2), np.arange(1, C, 2)])
    zeta = 2 * np.pi * (f + 0.5) / (4 * C)

    def fwd(n):
        ang = zeta[:, None] * n[None, :]
        m = np.stack([np.cos(ang), -np.sin(ang)], 0)
        return m.reshape(2, NT, 8, C).transpose(1, 0, 2, 3).reshape(2 * C, C)

    def inv(n):
        ang = n[:, None] * zeta[None, :]
        return np.stack([np.cos(ang), -np.sin(ang)], -1).reshape(C, 2 * C) / (2 * C)

    def words(m):
        b = m.astype(np.float32).astype(bf16).view(np.uint16).astype(np.uint32)
        return b[0::2] | (b[1::2] << 16)

    j = np.arange(C)
    even = (j // 2) * 2 + (j % 2) * C
    return (words(np.concatenate([fwd(even), fwd(even + 1)], 0)),
            words(np.concatenate([inv(2 * j), inv(2 * j + 1)], 0)))


def _spec_row(filt, block, tile=0, part=0):
    return filt * KO + block * BS + (2 * tile + part) * 8


def _unpack(w, i):
    return pltpu.unpack_elementwise(w, index=i, packed_dtype=bf16, unpacked_dtype=f32)


def _pack(a, b):
    return pltpu.bitcast(pltpu.pack_elementwise([a, b], packed_dtype=bf16), u32)


def _as_bf16(w):
    return pltpu.bitcast(w, bf16)


def _dot(a, b):
    return jnp.dot(a, b, preferred_element_type=f32)


def _layernorm(x):
    xc = x - jnp.sum(x, axis=-1, keepdims=True) * (1.0 / D)
    var = jnp.sum(xc * xc, axis=-1, keepdims=True) * (1.0 / D)
    return xc * lax.rsqrt(var + EPS)


def _left_factors(a11, a12, a21, a22):
    return [a11 + a22, a21 + a22, a11, a22, a11 + a12, a21 - a11, a12 - a22]


def _right_factors(b11, b12, b21, b22):
    return [b11 + b22, b11, b12 - b22, b21 - b11, b22, b11 + b12, b21 + b22]


def _factors(level, blocks):
    if len(blocks) == 2:
        yield from level(*blocks[0], *blocks[1])
        return
    outer = [level(*[blocks[2 * i + r][2 * j + c] for i in range(2) for j in range(2)])
             for r in range(2) for c in range(2)]
    for k in range(7):
        yield from level(*[o[k] for o in outer])


def _combine(m):
    return (jnp.concatenate([m[0] + m[3] - m[4] + m[6], m[1] + m[3]], axis=0),
            jnp.concatenate([m[2] + m[4], m[0] - m[1] + m[2] + m[5]], axis=0))


def _swiglu(gate, up):
    half = 0.5 * gate
    return (half * jnp.tanh(half) + half) * up


def _run_mixed(main, side):
    total, done, k = sum(w for w, _ in main), 0, 0
    for w, f in main:
        f()
        done += w
        while k < len(side) and (k + 0.5) * total <= done * len(side):
            side[k]()
            k += 1
    for f in side[k:]:
        f()


def _kernel(q_hbm, k_hbm, v_hbm, shk_hbm, ssm_hbm, d_hbm, w1_hbm, w3_hbm, w2_hbm, c_hbm, wm_hbm,
            fwd_hbm, inv_hbm, o_hbm,
            shk, dvec, cvec, fwd, inv, qb, kb, vb, sb, w1, w3, w2, wm,
            spec, zlast, kf, zb, yb, cpar, zero, par, x1b, h2b, hs, he, up_sums, down_sums, ob, sems):
    k32, v32, s32, wm32, w132, w332, w232 = (
        a.bitcast(u32) for a in (k_hbm, v_hbm, ssm_hbm, wm_hbm, w1_hbm, w3_hbm, w2_hbm))

    def conv_inputs(l, t0, n):
        cols = pl.ds(l * 128, 128)
        return [(s32.at[pl.ds(l * H, H), pl.ds(t0, n)], sb.at[l, :, pl.ds(t0, n)]),
                (k32.at[pl.ds(t0 // 2, n // 2), cols], kb.at[l, pl.ds(8 + t0 // 2, n // 2)]),
                (v32.at[pl.ds(t0 // 2, n // 2), cols], vb.at[l, pl.ds(t0 // 2, n // 2)])]

    def same(src, dst, *idx):
        return src.at[idx], dst.at[idx]

    mod_cols = lambda c0, n: same(wm32, wm, slice(None), pl.ds(c0, n))
    up_cols = lambda g: [same(w132, w1, slice(None), pl.ds(g * TF, TF)),
                         same(w332, w3, slice(None), pl.ds(g * TF, TF))]
    down_rows = lambda g: same(w232, w2, pl.ds(g * TF // 2, TF // 2))
    q_rows = lambda r0, n: same(q_hbm, qb, pl.ds(r0, n))
    groups = {
        'params': [(shk_hbm, shk), (d_hbm, dvec), (c_hbm, cvec)],
        'first': [(fwd_hbm, fwd)] + conv_inputs(0, 0, S // 2),
        0: conv_inputs(0, S // 2, S // 2),
        1: conv_inputs(1, 0, S),
        'inv': [(inv_hbm, inv)],
        **{l: conv_inputs(l, 0, S) for l in range(2, NL)},
        'mod': [mod_cols(0, 5 * D), q_rows(0, R)],
        'ffn0': [same(w132, w1, slice(None), pl.ds(0, 2 * TF)), up_cols(0)[1]],
        'ffn1': up_cols(1)[1:] + [down_rows(0)] + up_cols(2)[:1],
        'ffn2': [q_rows(R, R)] + up_cols(2)[1:] + [down_rows(1)],
        'ffn3': [mod_cols(5 * D, D), down_rows(2)],
        'q': [q_rows(2 * R, 2 * R)],
        'q_late': [q_rows(4 * R, S - 4 * R)],
    }
    named = [g for g in groups if isinstance(g, str)]
    sem_of = lambda g: sems.at[NL + named.index(g) if isinstance(g, str) else g]
    out_sem = sems.at[NL + len(named)]

    def wait(g, pairs=None):
        with _scope('wait_' + (g if isinstance(g, str) else 'slab')):
            for src, dst in (groups[g] if pairs is None else pairs):
                pltpu.make_async_copy(src, dst, sem_of(g)).wait()

    def out_copy(r0, cols=slice(None)):
        return pltpu.make_async_copy(*same(ob, o_hbm, pl.ds(r0, R), cols), out_sem)

    for g, pairs in groups.items():
        for src, dst in pairs:
            pltpu.make_async_copy(src, dst, sem_of(g)).start()

    wait('params')
    taps = shk[...].astype(f32)
    skip = dvec[...].astype(f32).reshape(1, D)
    for l in range(NL):
        kb[l, 0:8, :] = jnp.zeros((8, 128), u32)
        for j in range(KS):
            cpar[l, j] = jnp.broadcast_to(taps[j:j + 1, l * 128:(l + 1) * 128], (8, 128))
        cpar[l, KS] = jnp.broadcast_to(skip[:, l * 128:(l + 1) * 128], (8, 128))
    zero[0] = 0
    z0 = pl.multiple_of(zero[0] * 1024, 1024)

    def forward_pieces(l, buf):
        param = lambda j, rows: jnp.broadcast_to(cpar[l, j, 0:1, :], (rows, 128))
        mat = lambda i: _as_bf16(fwd[i * C:(i + 1) * C, :])

        def butterfly(filt, j, even, odd):
            r = _spec_row(filt, j)
            spec[buf][r:r + 2 * C, :] = even + odd
            spec[buf][r + 2 * C:r + 4 * C, :] = even - odd

        def signal(j):
            def f():
                kw = kb[l, j * C:j * C + C + 8, :]
                ke, ko = _unpack(kw, 0), _unpack(kw, 1)
                kf[j][0] = ke
                kf[j][1] = ko
                ke1, ko1, ko2 = kf[j][0, 7:7 + C, :], kf[j][1, 7:7 + C, :], kf[j][1, 6:6 + C, :]
                ke, ko = ke[8:], ko[8:]
                t0, t1, t2, t3 = (param(t, C) for t in range(KS))
                vw = vb[l, j * C:(j + 1) * C, :]
                xe = (t0 * ke + t1 * ko1 + t2 * ke1 + t3 * ko2) * _unpack(vw, 0)
                xo = (t0 * ko + t1 * ke + t2 * ko1 + t3 * ke1) * _unpack(vw, 1)
                butterfly(0, j, _dot(mat(0), _as_bf16(_pack(xe[:H], xe[H:]))),
                          _dot(mat(1), _as_bf16(_pack(xo[:H], xo[H:]))))
            return f

        def long_filter(j):
            def f():
                lo = sb[l, :, 2 * j * C:(2 * j + 1) * C]
                hi = sb[l, :, (2 * j + 1) * C:(2 * j + 2) * C]
                even_lane = lax.broadcasted_iota(jnp.int32, lo.shape, 1) % 2 == 0
                te = jnp.where(even_lane, lo, pltpu.roll(hi, 1, 1))
                to = jnp.where(even_lane, pltpu.roll(lo, C - 1, 1), hi)
                dims = (((1,), (1,)), ((), ()))
                pe = lax.dot_general(mat(0), _as_bf16(te), dims, preferred_element_type=f32)
                po = lax.dot_general(mat(1), _as_bf16(to), dims, preferred_element_type=f32)
                if j == 0:
                    real = lax.broadcasted_iota(jnp.int32, pe.shape, 0) % 16 < 8
                    pe = pe + jnp.where(real, param(KS, 2 * C), 0.0)
                butterfly(1, j, pe, po)
            return f
        return [piece(j) for j in range(NBLK) for piece in (signal, long_filter)]

    def product_pieces(buf):
        load = lambda filt, j, tile: [
            spec[buf][pl.ds(z0 + _spec_row(filt, j, tile, c), 8), :] for c in range(2)]

        def piece(p, t):
            def plus_tail(z, prev):
                if t < NT // 2:
                    return [z[0] - prev[1], z[1] + prev[0]]
                return [z[0] + prev[1], z[1] - prev[0]]

            def f():
                res = []
                for tile in (t, NT + t):
                    acc, xs = [None, None], {}
                    for m in range(2 * p + 2):
                        kr, ki = load(1, m, tile)
                        for i in range(2):
                            j = 2 * p + i - m
                            if j < 0:
                                continue
                            if j not in xs:
                                xs[j] = load(0, j, tile)
                            xr, xi = xs[j]
                            term = [kr * xr - ki * xi, kr * xi + ki * xr]
                            acc[i] = term if acc[i] is None else [a + b for a, b in zip(acc[i], term)]
                    row = tile * 16
                    first = acc[0]
                    if p > 0:
                        first = plus_tail(first, [zlast[p - 1][pl.ds(z0 + row + 8 * c, 8), :] for c in range(2)])
                    if 2 * p + 2 < NBLK:
                        for c in range(2):
                            zlast[p][row + 8 * c:row + 8 * c + 8, :] = acc[1][c]
                    res.append([first, plus_tail(acc[1], acc[0])])
                for i in range(2):
                    (ar, ai), (br, bi) = res[0][i], res[1][i]
                    zb[2 * p + i][0, 8 * t:8 * t + 8, :] = _pack(ar + br, ai + bi)
                    zb[2 * p + i][1, 8 * t:8 * t + 8, :] = _pack(ar - br, ai - bi)
            return f
        return [(4 * p + 5, piece(p, t)) for p in range(NBLK // 2) for t in range(NT)]

    def inverse(l, j):
        ye, yo = (_dot(_as_bf16(inv[i * H:(i + 1) * H, :]), _as_bf16(zb[j][i, pl.ds(z0, C), :]))
                  for i in range(2))
        yb[l, j * C:(j + 1) * C, :] = _pack(ye, yo)

    def conv_step(l, buf, early=0):
        products = product_pieces(buf)
        for _, f in products[:early]:
            f()
        if early:
            wait('inv')
        wait(l + 1, conv_inputs(l + 1, 0, S))
        for j in range(2 * (early // NT) - 2):
            inverse(l, j)
        ahead = forward_pieces(l + 1, 1 - buf)
        total, done, k = sum(w for w, _ in products[early:]), 0, 0
        for i, (w, f) in list(enumerate(products))[early:]:
            while k < len(ahead) and (k + 1) * total * DFT_SPAN <= done * (len(ahead) + 1):
                ahead[k]()
                k += 1
            f()
            done += w
            p, t = divmod(i, NT)
            if p > 0 and t in (NT // 4, 3 * NT // 4):
                inverse(l, 2 * p - 2 + (t > NT // 2))
        for f in ahead[k:]:
            f()
        inverse(l, NBLK - 2)
        inverse(l, NBLK - 1)

    ahead = forward_pieces(0, 0)
    wait('first')
    for f in ahead[:NBLK]:
        f()
    wait(0)
    for f in ahead[NBLK:]:
        f()
    conv_step(0, 0, early=3 * NT)
    for l in range(1, NL - 1):
        conv_step(l, l % 2)

    cond = cvec[...].astype(f32)
    cond = jnp.broadcast_to(cond * jax.nn.sigmoid(cond), (16, D)).astype(bf16)
    mod = lambda j: _dot(cond, _as_bf16(wm[:, j * D:(j + 1) * D]))[0:8]
    row = lambda j, rows, cols=slice(None): par[j, 0:1, cols]

    words = lambda x: pltpu.bitcast(x.astype(bf16), u32)

    def chunk(s):
        if isinstance(s, int):
            return s % 2, s * R
        return lax.rem(s, 2), pl.multiple_of(s * R, R)

    def norm_pieces(s):
        slot, _ = chunk(s)
        n = LR // 2

        def rows(ref_at, scale, i):
            starts = [s * (R // scale) + (half * RH + i * n) // scale for half in range(2)]
            if not isinstance(s, int):
                starts = [pl.multiple_of(r, n // scale) for r in starts]
            return jnp.concatenate([ref_at(pl.ds(r, n // scale)) for r in starts], axis=0)

        def piece(i):
            def f():
                x = rows(lambda r: qb[r, :], 1, i).astype(f32)
                y = jnp.concatenate(
                    [_as_bf16(rows(lambda r: yb[l, r, :], 2, i)).astype(f32) for l in range(NL)], axis=1)
                x = x + (_layernorm(x) * row(0, LR) + row(1, LR)) * y
                h = _layernorm(x) * row(2, LR) + row(3, LR)
                at = [slice((half * RH + i * n) // 2, (half * RH + (i + 1) * n) // 2) for half in range(2)]
                for half in range(2):
                    r = half * RH + i * n
                    x1b[slot, r:r + n, :] = x[half * n:(half + 1) * n]
                top, bottom = h[:n], h[n:]
                if isinstance(s, int) and s == 0:
                    h2b[at[0], :], h2b[at[1], :] = words(top), words(bottom)
                    return
                he[slot, at[0], :], he[slot, at[1], :] = words(top[:, 2 * DH:]), words(bottom[:, 2 * DH:])
                sums = _left_factors(top[:, :DH], top[:, DH:2 * DH], bottom[:, :DH], bottom[:, DH:2 * DH])
                for k, v in enumerate(sums):
                    hs[slot, k, at[0], :] = words(v)
            return f
        return [piece(i) for i in range(R // LR)]

    def weight_pieces(w, nb, nk, nn, out, skip=()):
        def piece(r, c):
            def f():
                blocks = [[w[i * nk + r:i * nk + r + 8, j * nn + c:j * nn + c + 128] for j in range(nb)]
                          for i in range(nb)]
                even, odd = (_factors(_right_factors, [[_unpack(b, h) for b in bs] for bs in blocks])
                             for h in range(2))
                for k, (e, o) in enumerate(zip(even, odd)):
                    if k not in skip:
                        out[k, r:r + 8, c:c + 128] = _pack(e, o)
            return f
        return [piece(r, c) for r in range(0, nk, 8) for c in range(0, nn, 128)]

    def residual(s, y, c0):
        slot, r0 = chunk(s)
        cols = slice(c0, c0 + y.shape[1])
        ob[pl.ds(r0, R), cols] = (x1b[slot, :, cols] + row(4, R, cols) * y).astype(bf16)

    def first_ffn_pieces():
        st = {}

        def gate(c):
            def f():
                st['gate', c] = _dot(_as_bf16(h2b[...]), _as_bf16(w1[:, c:c + PW]))
            return f

        def up(c):
            def f():
                u = _dot(_as_bf16(h2b[...]), _as_bf16(w3[:, c:c + PW]))
                st[c] = _swiglu(st['gate', c], u).astype(bf16)
            return f

        def down(g, c0, c1):
            def f():
                a = jnp.concatenate([st[c] for c in range(g * TF, (g + 1) * TF, PW)], axis=1)
                p = _dot(a, _as_bf16(w2[g * TF // 2:(g + 1) * TF // 2, c0:c1]))
                st['acc', c0] = p if g == 0 else st['acc', c0] + p
                if g + 1 == NG:
                    residual(0, st['acc', c0], c0)
            return f
        cols = lambda g: range(g * TF, (g + 1) * TF, PW)
        return ([[(PW, gate(c)) for c in cols(g)] for g in range(NG)],
                [[(PW, up(c)) for c in cols(g)] for g in range(NG)],
                [[(c1 - c0, down(g, c0, c1)) for c0, c1 in zip(OUT_COLS[:-1], OUT_COLS[1:])] for g in range(NG)])

    def ffn_pieces(s):
        slot, r0 = chunk(s)
        last = isinstance(s, int) and s == NS - 1
        lhs, hidden, pending = [], [[] for _ in range(4)], []

        def up(n):
            left, right = slice(n, n + 128), slice(FH + n, FH + n + 128)

            def project(i, w):
                plain = {1: w.at[0:DH // 2, left], 4: w.at[DH // 2:DH, right]}
                both = _combine([_dot(_as_bf16(hs[slot, k]),
                                      _as_bf16(plain[k][...] if k in plain else up_sums[i, k, :, left]))
                                 for k in range(7)])
                rest = _as_bf16(he[slot])
                return [p + _dot(rest, _as_bf16(w[DH:, cols])) for p, cols in zip(both, (left, right))]

            def f():
                pending.append([_swiglu(g, u) for g, u in zip(project(0, w1), project(1, w3))])
                if n >= FQ:
                    (a1, a3), (a0, a2) = pending.pop(), pending.pop()
                    a = [a0, a1, a2, a3]
                    blocks = [[v[r * RQ:(r + 1) * RQ] for v in a] for r in range(4)]
                    lhs.append([v.astype(bf16) for v in _factors(_left_factors, blocks)])
                    for j in range(4):
                        hidden[j].append(a[j].astype(bf16))
            return f

        def down():
            product = lambda k: _dot(jnp.concatenate([t[k] for t in lhs], axis=1), _as_bf16(down_sums[k]))
            inner = [_combine([product(7 * i + j) for j in range(7)]) for i in range(7)]
            for c in range(2):
                for j, y in enumerate(_combine([x[c] for x in inner])):
                    residual(s, y, (2 * j + c) * DQ)
            if last:
                out_copy(r0, pl.ds(0, 2 * DH)).start()

        def down_rest():
            a = jnp.concatenate([v for h in hidden for v in h], axis=1)
            residual(s, _dot(a, _as_bf16(w2[:, 2 * DH:])), 2 * DH)
            if last:
                out_copy(r0, pl.ds(2 * DH, D - 2 * DH)).start()
        ups = [(18, up(n + j * FQ)) for n in range(0, FQ, 128) for j in range(2)]
        downs = [(37, down)]
        return ups + [(12, down_rest)] + downs

    products = product_pieces(0)
    for _, f in products[:5 * NT // 2]:
        f()
    wait('mod')
    scale_a, gate_a, shift_a, scale_b, shift_b = (mod(j) for j in (1, 2, 0, 4, 3))
    par[0] = gate_a * (1.0 + scale_a)
    par[1] = gate_a * shift_a
    par[2] = 1.0 + scale_b
    par[3] = shift_b
    for _, f in products[5 * NT // 2:]:
        f()
    inverse(NL - 1, 0)
    inverse(NL - 1, 1)
    _run_mixed([(1, f) for f in norm_pieces(0)],
               [functools.partial(inverse, NL - 1, j) for j in range(2, NBLK)])

    gates, ups, downs = first_ffn_pieces()
    norms = norm_pieces(1)
    n = len(norms) // 2
    wait('ffn0')
    _run_mixed(gates[0] + ups[0] + gates[1], [])
    wait('ffn1')
    _run_mixed(ups[1] + downs[0] + gates[2], weight_pieces(w1, 2, DH // 2, FH, up_sums.at[0], (1, 4)))
    wait('ffn2')
    _run_mixed(ups[2] + downs[1], weight_pieces(w3, 2, DH // 2, FH, up_sums.at[1], (1, 4)) + norms[:n])
    wait('ffn3')
    par[4] = mod(5)
    _run_mixed(downs[2], weight_pieces(w2, 4, FQ // 2, DQ, down_sums) + norms[n:])
    out_copy(0).start()
    wait('q')

    def ffn_body(s, carry):
        pl.when(s == 3)(lambda: wait('q_late'))
        pieces = ffn_pieces(s)
        n = PRE_PIECES
        _run_mixed(pieces[:n], norm_pieces(s + 1))
        _run_mixed(pieces[n:], [])
        out_copy(pl.multiple_of(s * R, R)).start()
        return carry
    with _scope('ffn_loop'):
        lax.fori_loop(1, NS - 1, ffn_body, 0)
    _run_mixed(ffn_pieces(NS - 1), [])

    with _scope('wait_out'):
        for s in range(NS - 1):
            out_copy(s * R).wait()
        out_copy(S - R, pl.ds(0, 2 * DH)).wait()
        out_copy(S - R, pl.ds(2 * DH, D - 2 * DH)).wait()


@jax.jit
def pallas_adaLN_cond__ssm_conv_h3__glu_gated_swiglu__prompt_kernel(
    A_q: jax.Array,
    A_k: jax.Array,
    A_v: jax.Array,
    A_shift_k: jax.Array,
    A_ssm_k: jax.Array,
    A_ssm_D: jax.Array,
    B_x: jax.Array,
    B_w1: jax.Array,
    B_w3: jax.Array,
    B_w2: jax.Array,
    c: jax.Array,
    w_mod: jax.Array,
):
    del B_x
    fwd, inv = _dft_matrices()
    hbm = pl.BlockSpec(memory_space=pl.ANY)
    vmem = pltpu.VMEM
    out = pl.pallas_call(
        _kernel,
        in_specs=[hbm] * 13,
        out_specs=hbm,
        out_shape=jax.ShapeDtypeStruct((S, D), bf16),
        scratch_shapes=[
            vmem((KS, D), bf16), vmem((D,), bf16), vmem((1, D), bf16),
            vmem(fwd.shape, u32), vmem(inv.shape, u32),
            vmem((S, D), bf16),
            vmem((NL, S // 2 + 8, 128), u32), vmem((NL, S // 2, 128), u32),
            vmem((NL, H, S), u32),
            vmem((D // 2, F), u32), vmem((D // 2, F), u32), vmem((F // 2, D), u32),
            vmem((D // 2, 6 * D), u32),
            [vmem((2 * KO + 512, 128), f32) for _ in range(2)],
            [vmem((4 * C, 128), f32) for _ in range(NBLK // 2 - 1)],
            [vmem((2, C + 8, 128), f32) for _ in range(NBLK)],
            [vmem((2, C, 128), u32) for _ in range(NBLK)],
            vmem((NL, S // 2, 128), u32),
            vmem((NL, KS + 1, 8, 128), f32), pltpu.SMEM((1,), jnp.int32), vmem((5, 8, D), f32),
            vmem((2, R, D), f32), vmem((R // 2, D), u32),
            vmem((2, 7, RH // 2, DH), u32), vmem((2, R // 2, D - 2 * DH), u32),
            vmem((2, 7, DH // 2, FH), u32), vmem((49, FQ // 2, DQ), u32),
            vmem((S, D), bf16),
            pltpu.SemaphoreType.DMA((NL + 11,)),
        ],
        compiler_params=pltpu.CompilerParams(vmem_limit_bytes=100 * 2**20),
    )(A_q.reshape(S, D), A_k.reshape(S, D), A_v.reshape(S, D), A_shift_k.T, A_ssm_k, A_ssm_D,
      B_w1, B_w3, B_w2, c, w_mod, fwd, inv)
    return out.reshape(1, S, D)
```

```python
import functools

import jax
import jax.numpy as jnp
import numpy as np
from jax import lax
from jax.experimental import pallas as pl
from jax.experimental.pallas import tpu as pltpu

S, D, F = 2048, 640, 1536
KS = 4
EPS = 1e-5
C = 128
H = C // 2
NBLK = S // (2 * C)
NL = D // 128
NT = C // 8
R = 256
LR = 32
TF = 512
PW = 256
OUT_COLS = (0, 256, 512, D)
NS = S // R
NG = F // TF
RH, DH, FH = R // 2, 256, F // 2
RQ, DQ, FQ = RH // 2, DH // 2, FH // 2
BS = (4 * NT + 4) * 8
KO = (NBLK * BS + 511) // 512 * 512 + 16
DFT_SPAN = 0.9
PRE_PIECES = 5

f32, bf16, u32 = jnp.float32, jnp.bfloat16, jnp.uint32


def _dft_matrices():
    f = np.concatenate([np.arange(0, C, 2), np.arange(1, C, 2)])
    zeta = 2 * np.pi * (f + 0.5) / (4 * C)

    def fwd(n):
        ang = zeta[:, None] * n[None, :]
        m = np.stack([np.cos(ang), -np.sin(ang)], 0)
        return m.reshape(2, NT, 8, C).transpose(1, 0, 2, 3).reshape(2 * C, C)

    def inv(n):
        ang = n[:, None] * zeta[None, :]
        return np.stack([np.cos(ang), -np.sin(ang)], -1).reshape(C, 2 * C) / (2 * C)

    def words(m):
        b = m.astype(np.float32).astype(bf16).view(np.uint16).astype(np.uint32)
        return b[0::2] | (b[1::2] << 16)

    j = np.arange(C)
    even = (j // 2) * 2 + (j % 2) * C
    return (words(np.concatenate([fwd(even), fwd(even + 1)], 0)),
            words(np.concatenate([inv(2 * j), inv(2 * j + 1)], 0)))


def _spec_row(filt, block, tile=0, part=0):
    return filt * KO + block * BS + (2 * tile + part) * 8


def _unpack(w, i):
    return pltpu.unpack_elementwise(w, index=i, packed_dtype=bf16, unpacked_dtype=f32)


def _pack(a, b):
    return pltpu.bitcast(pltpu.pack_elementwise([a, b], packed_dtype=bf16), u32)


def _as_bf16(w):
    return pltpu.bitcast(w, bf16)


def _dot(a, b):
    return jnp.dot(a, b, preferred_element_type=f32)


def _layernorm(x):
    xc = x - jnp.sum(x, axis=-1, keepdims=True) * (1.0 / D)
    var = jnp.sum(xc * xc, axis=-1, keepdims=True) * (1.0 / D)
    return xc * lax.rsqrt(var + EPS)


def _left_factors(a11, a12, a21, a22):
    return [a11 + a22, a21 + a22, a11, a22, a11 + a12, a21 - a11, a12 - a22]


def _right_factors(b11, b12, b21, b22):
    return [b11 + b22, b11, b12 - b22, b21 - b11, b22, b11 + b12, b21 + b22]


def _factors(level, blocks):
    if len(blocks) == 2:
        yield from level(*blocks[0], *blocks[1])
        return
    outer = [level(*[blocks[2 * i + r][2 * j + c] for i in range(2) for j in range(2)])
             for r in range(2) for c in range(2)]
    for k in range(7):
        yield from level(*[o[k] for o in outer])


def _combine(m):
    return (jnp.concatenate([m[0] + m[3] - m[4] + m[6], m[1] + m[3]], axis=0),
            jnp.concatenate([m[2] + m[4], m[0] - m[1] + m[2] + m[5]], axis=0))


def _swiglu(gate, up):
    half = 0.5 * gate
    return (half * jnp.tanh(half) + half) * up


def _run_mixed(main, side):
    total, done, k = sum(w for w, _ in main), 0, 0
    for w, f in main:
        f()
        done += w
        while k < len(side) and (k + 0.5) * total <= done * len(side):
            side[k]()
            k += 1
    for f in side[k:]:
        f()


def _kernel(q_hbm, k_hbm, v_hbm, shk_hbm, ssm_hbm, d_hbm, w1_hbm, w3_hbm, w2_hbm, c_hbm, wm_hbm,
            fwd_hbm, inv_hbm, o_hbm,
            shk, dvec, cvec, fwd, inv, qb, kb, vb, sb, w1, w3, w2, wm,
            spec, zlast, kf, zb, yb, cpar, zero, par, x1b, h2b, hs, he, up_sums, down_sums, ob, sems):
    k32, v32, s32, wm32, w132, w332, w232 = (
        a.bitcast(u32) for a in (k_hbm, v_hbm, ssm_hbm, wm_hbm, w1_hbm, w3_hbm, w2_hbm))

    def conv_inputs(l, t0, n):
        cols = pl.ds(l * 128, 128)
        return [(s32.at[pl.ds(l * H, H), pl.ds(t0, n)], sb.at[l, :, pl.ds(t0, n)]),
                (k32.at[pl.ds(t0 // 2, n // 2), cols], kb.at[l, pl.ds(8 + t0 // 2, n // 2)]),
                (v32.at[pl.ds(t0 // 2, n // 2), cols], vb.at[l, pl.ds(t0 // 2, n // 2)])]

    def same(src, dst, *idx):
        return src.at[idx], dst.at[idx]

    mod_cols = lambda c0, n: same(wm32, wm, slice(None), pl.ds(c0, n))
    up_cols = lambda g: [same(w132, w1, slice(None), pl.ds(g * TF, TF)),
                         same(w332, w3, slice(None), pl.ds(g * TF, TF))]
    down_rows = lambda g: same(w232, w2, pl.ds(g * TF // 2, TF // 2))
    q_rows = lambda r0, n: same(q_hbm, qb, pl.ds(r0, n))
    groups = {
        'params': [(shk_hbm, shk), (d_hbm, dvec), (c_hbm, cvec)],
        'first': [(fwd_hbm, fwd)] + conv_inputs(0, 0, S // 2),
        0: conv_inputs(0, S // 2, S // 2),
        1: conv_inputs(1, 0, S),
        'inv': [(inv_hbm, inv)],
        **{l: conv_inputs(l, 0, S) for l in range(2, NL)},
        'mod': [mod_cols(0, 5 * D), q_rows(0, R)],
        'ffn0': [same(w132, w1, slice(None), pl.ds(0, 2 * TF)), up_cols(0)[1]],
        'ffn1': up_cols(1)[1:] + [down_rows(0)] + up_cols(2)[:1],
        'ffn2': [q_rows(R, R)] + up_cols(2)[1:] + [down_rows(1)],
        'ffn3': [mod_cols(5 * D, D), down_rows(2)],
        'q': [q_rows(2 * R, 2 * R)],
        'q_late': [q_rows(4 * R, S - 4 * R)],
    }
    sem_of = lambda g: sems.at[list(groups).index(g)]
    out_sem = sems.at[len(groups)]

    def wait(g):
        for src, dst in groups[g]:
            pltpu.make_async_copy(src, dst, sem_of(g)).wait()

    def out_copy(r0, cols=slice(None)):
        return pltpu.make_async_copy(*same(ob, o_hbm, pl.ds(r0, R), cols), out_sem)

    for g, pairs in groups.items():
        for src, dst in pairs:
            pltpu.make_async_copy(src, dst, sem_of(g)).start()

    wait('params')
    taps = shk[...].astype(f32)
    skip = dvec[...].astype(f32).reshape(1, D)
    for l in range(NL):
        kb[l, 0:8, :] = jnp.zeros((8, 128), u32)
        for j in range(KS):
            cpar[l, j] = jnp.broadcast_to(taps[j:j + 1, l * 128:(l + 1) * 128], (8, 128))
        cpar[l, KS] = jnp.broadcast_to(skip[:, l * 128:(l + 1) * 128], (8, 128))
    zero[0] = 0
    z0 = pl.multiple_of(zero[0] * 1024, 1024)

    def forward_pieces(l, buf):
        param = lambda j, rows: jnp.broadcast_to(cpar[l, j, 0:1, :], (rows, 128))
        mat = lambda i: _as_bf16(fwd[i * C:(i + 1) * C, :])

        def butterfly(filt, j, even, odd):
            r = _spec_row(filt, j)
            spec[buf][r:r + 2 * C, :] = even + odd
            spec[buf][r + 2 * C:r + 4 * C, :] = even - odd

        def signal(j):
            def f():
                kw = kb[l, j * C:j * C + C + 8, :]
                ke, ko = _unpack(kw, 0), _unpack(kw, 1)
                kf[j][0] = ke
                kf[j][1] = ko
                ke1, ko1, ko2 = kf[j][0, 7:7 + C, :], kf[j][1, 7:7 + C, :], kf[j][1, 6:6 + C, :]
                ke, ko = ke[8:], ko[8:]
                t0, t1, t2, t3 = (param(t, C) for t in range(KS))
                vw = vb[l, j * C:(j + 1) * C, :]
                xe = (t0 * ke + t1 * ko1 + t2 * ke1 + t3 * ko2) * _unpack(vw, 0)
                xo = (t0 * ko + t1 * ke + t2 * ko1 + t3 * ke1) * _unpack(vw, 1)
                butterfly(0, j, _dot(mat(0), _as_bf16(_pack(xe[:H], xe[H:]))),
                          _dot(mat(1), _as_bf16(_pack(xo[:H], xo[H:]))))
            return f

        def long_filter(j):
            def f():
                lo = sb[l, :, 2 * j * C:(2 * j + 1) * C]
                hi = sb[l, :, (2 * j + 1) * C:(2 * j + 2) * C]
                even_lane = lax.broadcasted_iota(jnp.int32, lo.shape, 1) % 2 == 0
                te = jnp.where(even_lane, lo, pltpu.roll(hi, 1, 1))
                to = jnp.where(even_lane, pltpu.roll(lo, C - 1, 1), hi)
                dims = (((1,), (1,)), ((), ()))
                pe = lax.dot_general(mat(0), _as_bf16(te), dims, preferred_element_type=f32)
                po = lax.dot_general(mat(1), _as_bf16(to), dims, preferred_element_type=f32)
                if j == 0:
                    real = lax.broadcasted_iota(jnp.int32, pe.shape, 0) % 16 < 8
                    pe = pe + jnp.where(real, param(KS, 2 * C), 0.0)
                butterfly(1, j, pe, po)
            return f
        return [piece(j) for j in range(NBLK) for piece in (signal, long_filter)]

    def product_pieces(buf):
        load = lambda filt, j, tile: [
            spec[buf][pl.ds(z0 + _spec_row(filt, j, tile, c), 8), :] for c in range(2)]

        def piece(p, t):
            def plus_tail(z, prev):
                if t < NT // 2:
                    return [z[0] - prev[1], z[1] + prev[0]]
                return [z[0] + prev[1], z[1] - prev[0]]

            def f():
                res = []
                for tile in (t, NT + t):
                    acc, xs = [None, None], {}
                    for m in range(2 * p + 2):
                        kr, ki = load(1, m, tile)
                        for i in range(2):
                            j = 2 * p + i - m
                            if j < 0:
                                continue
                            if j not in xs:
                                xs[j] = load(0, j, tile)
                            xr, xi = xs[j]
                            term = [kr * xr - ki * xi, kr * xi + ki * xr]
                            acc[i] = term if acc[i] is None else [a + b for a, b in zip(acc[i], term)]
                    row = tile * 16
                    first = acc[0]
                    if p > 0:
                        first = plus_tail(first, [zlast[p - 1][pl.ds(z0 + row + 8 * c, 8), :] for c in range(2)])
                    if 2 * p + 2 < NBLK:
                        for c in range(2):
                            zlast[p][row + 8 * c:row + 8 * c + 8, :] = acc[1][c]
                    res.append([first, plus_tail(acc[1], acc[0])])
                for i in range(2):
                    (ar, ai), (br, bi) = res[0][i], res[1][i]
                    zb[2 * p + i][0, 8 * t:8 * t + 8, :] = _pack(ar + br, ai + bi)
                    zb[2 * p + i][1, 8 * t:8 * t + 8, :] = _pack(ar - br, ai - bi)
            return f
        return [(4 * p + 5, piece(p, t)) for p in range(NBLK // 2) for t in range(NT)]

    def inverse(l, j):
        ye, yo = (_dot(_as_bf16(inv[i * H:(i + 1) * H, :]), _as_bf16(zb[j][i, pl.ds(z0, C), :]))
                  for i in range(2))
        yb[l, j * C:(j + 1) * C, :] = _pack(ye, yo)

    def conv_step(l, buf, early=0):
        products = product_pieces(buf)
        for _, f in products[:early]:
            f()
        if early:
            wait('inv')
        wait(l + 1)
        for j in range(2 * (early // NT) - 2):
            inverse(l, j)
        ahead = forward_pieces(l + 1, 1 - buf)
        total, done, k = sum(w for w, _ in products[early:]), 0, 0
        for i, (w, f) in list(enumerate(products))[early:]:
            while k < len(ahead) and (k + 1) * total * DFT_SPAN <= done * (len(ahead) + 1):
                ahead[k]()
                k += 1
            f()
            done += w
            p, t = divmod(i, NT)
            if p > 0 and t in (NT // 4, 3 * NT // 4):
                inverse(l, 2 * p - 2 + (t > NT // 2))
        for f in ahead[k:]:
            f()
        inverse(l, NBLK - 2)
        inverse(l, NBLK - 1)

    ahead = forward_pieces(0, 0)
    wait('first')
    for f in ahead[:NBLK]:
        f()
    wait(0)
    for f in ahead[NBLK:]:
        f()
    conv_step(0, 0, early=3 * NT)
    for l in range(1, NL - 1):
        conv_step(l, l % 2)

    cond = cvec[...].astype(f32)
    cond = jnp.broadcast_to(cond * jax.nn.sigmoid(cond), (16, D)).astype(bf16)
    mod = lambda j: _dot(cond, _as_bf16(wm[:, j * D:(j + 1) * D]))[0:8]
    row = lambda j, rows, cols=slice(None): par[j, 0:1, cols]

    words = lambda x: pltpu.bitcast(x.astype(bf16), u32)

    def chunk(s):
        if isinstance(s, int):
            return s % 2, s * R
        return lax.rem(s, 2), pl.multiple_of(s * R, R)

    def norm_pieces(s):
        slot, _ = chunk(s)
        n = LR // 2

        def rows(ref_at, scale, i):
            starts = [s * (R // scale) + (half * RH + i * n) // scale for half in range(2)]
            if not isinstance(s, int):
                starts = [pl.multiple_of(r, n // scale) for r in starts]
            return jnp.concatenate([ref_at(pl.ds(r, n // scale)) for r in starts], axis=0)

        def piece(i):
            def f():
                x = rows(lambda r: qb[r, :], 1, i).astype(f32)
                y = jnp.concatenate(
                    [_as_bf16(rows(lambda r: yb[l, r, :], 2, i)).astype(f32) for l in range(NL)], axis=1)
                x = x + (_layernorm(x) * row(0, LR) + row(1, LR)) * y
                h = _layernorm(x) * row(2, LR) + row(3, LR)
                at = [slice((half * RH + i * n) // 2, (half * RH + (i + 1) * n) // 2) for half in range(2)]
                for half in range(2):
                    r = half * RH + i * n
                    x1b[slot, r:r + n, :] = x[half * n:(half + 1) * n]
                top, bottom = h[:n], h[n:]
                if isinstance(s, int) and s == 0:
                    h2b[at[0], :], h2b[at[1], :] = words(top), words(bottom)
                    return
                he[slot, at[0], :], he[slot, at[1], :] = words(top[:, 2 * DH:]), words(bottom[:, 2 * DH:])
                sums = _left_factors(top[:, :DH], top[:, DH:2 * DH], bottom[:, :DH], bottom[:, DH:2 * DH])
                for k, v in enumerate(sums):
                    hs[slot, k, at[0], :] = words(v)
            return f
        return [piece(i) for i in range(R // LR)]

    def weight_pieces(w, nb, nk, nn, out, skip=()):
        def piece(r, c):
            def f():
                blocks = [[w[i * nk + r:i * nk + r + 8, j * nn + c:j * nn + c + 128] for j in range(nb)]
                          for i in range(nb)]
                even, odd = (_factors(_right_factors, [[_unpack(b, h) for b in bs] for bs in blocks])
                             for h in range(2))
                for k, (e, o) in enumerate(zip(even, odd)):
                    if k not in skip:
                        out[k, r:r + 8, c:c + 128] = _pack(e, o)
            return f
        return [piece(r, c) for r in range(0, nk, 8) for c in range(0, nn, 128)]

    def residual(s, y, c0):
        slot, r0 = chunk(s)
        cols = slice(c0, c0 + y.shape[1])
        ob[pl.ds(r0, R), cols] = (x1b[slot, :, cols] + row(4, R, cols) * y).astype(bf16)

    def first_ffn_pieces():
        st = {}

        def gate(c):
            def f():
                st['gate', c] = _dot(_as_bf16(h2b[...]), _as_bf16(w1[:, c:c + PW]))
            return f

        def up(c):
            def f():
                u = _dot(_as_bf16(h2b[...]), _as_bf16(w3[:, c:c + PW]))
                st[c] = _swiglu(st['gate', c], u).astype(bf16)
            return f

        def down(g, c0, c1):
            def f():
                a = jnp.concatenate([st[c] for c in range(g * TF, (g + 1) * TF, PW)], axis=1)
                p = _dot(a, _as_bf16(w2[g * TF // 2:(g + 1) * TF // 2, c0:c1]))
                st['acc', c0] = p if g == 0 else st['acc', c0] + p
                if g + 1 == NG:
                    residual(0, st['acc', c0], c0)
            return f
        cols = lambda g: range(g * TF, (g + 1) * TF, PW)
        return ([[(PW, gate(c)) for c in cols(g)] for g in range(NG)],
                [[(PW, up(c)) for c in cols(g)] for g in range(NG)],
                [[(c1 - c0, down(g, c0, c1)) for c0, c1 in zip(OUT_COLS[:-1], OUT_COLS[1:])] for g in range(NG)])

    def ffn_pieces(s):
        slot, r0 = chunk(s)
        last = isinstance(s, int) and s == NS - 1
        lhs, hidden, pending = [], [[] for _ in range(4)], []

        def up(n):
            left, right = slice(n, n + 128), slice(FH + n, FH + n + 128)

            def project(i, w):
                plain = {1: w.at[0:DH // 2, left], 4: w.at[DH // 2:DH, right]}
                both = _combine([_dot(_as_bf16(hs[slot, k]),
                                      _as_bf16(plain[k][...] if k in plain else up_sums[i, k, :, left]))
                                 for k in range(7)])
                rest = _as_bf16(he[slot])
                return [p + _dot(rest, _as_bf16(w[DH:, cols])) for p, cols in zip(both, (left, right))]

            def f():
                pending.append([_swiglu(g, u) for g, u in zip(project(0, w1), project(1, w3))])
                if n >= FQ:
                    (a1, a3), (a0, a2) = pending.pop(), pending.pop()
                    a = [a0, a1, a2, a3]
                    blocks = [[v[r * RQ:(r + 1) * RQ] for v in a] for r in range(4)]
                    lhs.append([v.astype(bf16) for v in _factors(_left_factors, blocks)])
                    for j in range(4):
                        hidden[j].append(a[j].astype(bf16))
            return f

        def down():
            product = lambda k: _dot(jnp.concatenate([t[k] for t in lhs], axis=1), _as_bf16(down_sums[k]))
            inner = [_combine([product(7 * i + j) for j in range(7)]) for i in range(7)]
            for c in range(2):
                for j, y in enumerate(_combine([x[c] for x in inner])):
                    residual(s, y, (2 * j + c) * DQ)
            if last:
                out_copy(r0, pl.ds(0, 2 * DH)).start()

        def down_rest():
            a = jnp.concatenate([v for h in hidden for v in h], axis=1)
            residual(s, _dot(a, _as_bf16(w2[:, 2 * DH:])), 2 * DH)
            if last:
                out_copy(r0, pl.ds(2 * DH, D - 2 * DH)).start()
        ups = [(18, up(n + j * FQ)) for n in range(0, FQ, 128) for j in range(2)]
        downs = [(37, down)]
        return ups + [(12, down_rest)] + downs

    products = product_pieces(0)
    for _, f in products[:5 * NT // 2]:
        f()
    wait('mod')
    scale_a, gate_a, shift_a, scale_b, shift_b = (mod(j) for j in (1, 2, 0, 4, 3))
    par[0] = gate_a * (1.0 + scale_a)
    par[1] = gate_a * shift_a
    par[2] = 1.0 + scale_b
    par[3] = shift_b
    for _, f in products[5 * NT // 2:]:
        f()
    inverse(NL - 1, 0)
    inverse(NL - 1, 1)
    _run_mixed([(1, f) for f in norm_pieces(0)],
               [functools.partial(inverse, NL - 1, j) for j in range(2, NBLK)])

    gates, ups, downs = first_ffn_pieces()
    norms = norm_pieces(1)
    n = len(norms) // 2
    wait('ffn0')
    _run_mixed(gates[0] + ups[0] + gates[1], [])
    wait('ffn1')
    _run_mixed(ups[1] + downs[0] + gates[2], weight_pieces(w1, 2, DH // 2, FH, up_sums.at[0], (1, 4)))
    wait('ffn2')
    _run_mixed(ups[2] + downs[1], weight_pieces(w3, 2, DH // 2, FH, up_sums.at[1], (1, 4)) + norms[:n])
    wait('ffn3')
    par[4] = mod(5)
    _run_mixed(downs[2], weight_pieces(w2, 4, FQ // 2, DQ, down_sums) + norms[n:])
    out_copy(0).start()
    wait('q')

    def ffn_body(s, carry):
        pl.when(s == 3)(lambda: wait('q_late'))
        pieces = ffn_pieces(s)
        n = PRE_PIECES
        _run_mixed(pieces[:n], norm_pieces(s + 1))
        _run_mixed(pieces[n:], [])
        out_copy(pl.multiple_of(s * R, R)).start()
        return carry
    lax.fori_loop(1, NS - 1, ffn_body, 0)
    _run_mixed(ffn_pieces(NS - 1), [])

    for s in range(NS - 1):
        out_copy(s * R).wait()
    out_copy(S - R, pl.ds(0, 2 * DH)).wait()
    out_copy(S - R, pl.ds(2 * DH, D - 2 * DH)).wait()


@jax.jit
def pallas_adaLN_cond__ssm_conv_h3__glu_gated_swiglu__prompt_kernel(
    A_q: jax.Array,
    A_k: jax.Array,
    A_v: jax.Array,
    A_shift_k: jax.Array,
    A_ssm_k: jax.Array,
    A_ssm_D: jax.Array,
    B_x: jax.Array,
    B_w1: jax.Array,
    B_w3: jax.Array,
    B_w2: jax.Array,
    c: jax.Array,
    w_mod: jax.Array,
):
    del B_x
    fwd, inv = _dft_matrices()
    hbm = pl.BlockSpec(memory_space=pl.ANY)
    vmem = pltpu.VMEM
    out = pl.pallas_call(
        _kernel,
        in_specs=[hbm] * 13,
        out_specs=hbm,
        out_shape=jax.ShapeDtypeStruct((S, D), bf16),
        scratch_shapes=[
            vmem((KS, D), bf16), vmem((D,), bf16), vmem((1, D), bf16),
            vmem(fwd.shape, u32), vmem(inv.shape, u32),
            vmem((S, D), bf16),
            vmem((NL, S // 2 + 8, 128), u32), vmem((NL, S // 2, 128), u32),
            vmem((NL, H, S), u32),
            vmem((D // 2, F), u32), vmem((D // 2, F), u32), vmem((F // 2, D), u32),
            vmem((D // 2, 6 * D), u32),
            [vmem((2 * KO + 512, 128), f32) for _ in range(2)],
            [vmem((4 * C, 128), f32) for _ in range(NBLK // 2 - 1)],
            [vmem((2, C + 8, 128), f32) for _ in range(NBLK)],
            [vmem((2, C, 128), u32) for _ in range(NBLK)],
            vmem((NL, S // 2, 128), u32),
            vmem((NL, KS + 1, 8, 128), f32), pltpu.SMEM((1,), jnp.int32), vmem((5, 8, D), f32),
            vmem((2, R, D), f32), vmem((R // 2, D), u32),
            vmem((2, 7, RH // 2, DH), u32), vmem((2, R // 2, D - 2 * DH), u32),
            vmem((2, 7, DH // 2, FH), u32), vmem((49, FQ // 2, DQ), u32),
            vmem((S, D), bf16),
            pltpu.SemaphoreType.DMA((NL + 11,)),
        ],
        compiler_params=pltpu.CompilerParams(vmem_limit_bytes=100 * 2**20),
    )(A_q.reshape(S, D), A_k.reshape(S, D), A_v.reshape(S, D), A_shift_k.T, A_ssm_k, A_ssm_D,
      B_w1, B_w3, B_w2, c, w_mod, fwd, inv)
    return out.reshape(1, S, D)
```
